```python
import jax
import jax.numpy as jnp

def _softmax(x, axis=-1):
    return jax.nn.softmax(x, axis=axis)

def _gelu(x):
    return jax.nn.gelu(x, approximate=True)

def _silu(x):
    return jax.nn.silu(x)

def _sigmoid(x):
    return jax.nn.sigmoid(x)

def _layernorm(x, axis=-1, eps=1e-05):
    m = jnp.mean(x, axis=axis, keepdims=True)
    v = jnp.var(x, axis=axis, keepdims=True)
    return (x - m) / jnp.sqrt(v + eps)

def _scatter_add(tgt, idx, src, axis=0):
    return tgt.at[idx].add(src)

def _segment_sum(src, seg, n):
    return jax.ops.segment_sum(src, seg, n)

class _Rng:

    def __init__(self, key):
        self._k = key

    def _next(self):
        self._k, sub = jax.random.split(self._k)
        return sub

    def normal(self, shape):
        return jax.random.normal(self._next(), shape, dtype=jnp.bfloat16)

    def randint(self, lo, hi, shape):
        return jax.random.randint(self._next(), shape, lo, hi, dtype=jnp.int32)

    def uniform(self, shape, lo=0.0, hi=1.0):
        return jax.random.uniform(self._next(), shape, jnp.bfloat16, lo, hi)

    def permutation(self, n):
        return jax.random.permutation(self._next(), n)
kernel_name = 'adaLN_cond__sliding_block_cached__moe_arch_mod__prompt'

def setup_inputs():
    _rng = _Rng(jax.random.key(int.from_bytes(__import__("os").urandom(4), "little")))
    _w = lambda a: (lambda t: t.astype(jnp.bfloat16) if jnp.issubdtype(t.dtype, jnp.floating) else t)(jnp.asarray(a))

    def _A_setup():
        B, Sq, D = (1, 2048, 1024)
        Hq, Hkv, Sk, Dh = (32, 4, 2048, 128)
        assert Hq % Hkv == 0, (Hq, Hkv)
        return {'x': _w((lambda *s: _rng.normal(s) * 0.05)(B, Sq, D)), 'k_cache': _w((lambda *s: _rng.normal(s) * 0.05)(B, Hkv, Sk, Dh)), 'v_cache': _w((lambda *s: _rng.normal(s) * 0.05)(B, Hkv, Sk, Dh)), 'wq': _w((lambda *s: _rng.normal(s) * 0.05)(D, Hq * Dh) * D ** (-0.5)), 'wo': _w((lambda *s: _rng.normal(s) * 0.05)(Hq * Dh, D) * (Hq * Dh) ** (-0.5))}
    _A_in = _A_setup()

    def _B_setup():
        B, S, D, F, C = (1, 2048, 1024, 3584, 1)
        return {'x': _w((lambda *s: _rng.normal(s) * 0.05)(B, S, D)), 'w_r': _w((lambda *s: _rng.normal(s) * 0.05)(D)), 'w_gate': _w((lambda *s: _rng.normal(s) * 0.05)(D, F)), 'w_up': _w((lambda *s: _rng.normal(s) * 0.05)(D, F)), 'w_down': _w((lambda *s: _rng.normal(s) * 0.05)(F, D))}
    _B_in = _B_setup()
    return {'A_x': _A_in['x'], 'A_k_cache': _A_in['k_cache'], 'A_v_cache': _A_in['v_cache'], 'A_wq': _A_in['wq'], 'A_wo': _A_in['wo'], 'B_x': _B_in['x'], 'B_w_r': _B_in['w_r'], 'B_w_gate': _B_in['w_gate'], 'B_w_up': _B_in['w_up'], 'B_w_down': _B_in['w_down'], 'c': _w((lambda *s: _rng.normal(s) * 0.05)(1, 1024)), 'w_mod': _w((lambda *s: _rng.normal(s) * 0.05)(1024, 6 * 1024) * 1024 ** (-0.5))}

def reference(A_x, A_k_cache, A_v_cache, A_wq, A_wo, B_x, B_w_r, B_w_gate, B_w_up, B_w_down, c, w_mod):

    def _A_ref(x, k_cache, v_cache, wq, wo):
        B, Sq, D = x.shape
        Hq, Dh = (32, 128)
        Hkv, Sk = (k_cache.shape[1], k_cache.shape[2])
        W = min(4096, max(256, Sk // 4))
        rep = Hq // Hkv
        q = (lambda x, *d: x.transpose(*d))((x @ wq).reshape(B, Sq, Hq, Dh), 0, 2, 1, 3)
        k = jnp.repeat(k_cache[:, :, Sk - W:, :], rep, axis=1)
        v = jnp.repeat(v_cache[:, :, Sk - W:, :], rep, axis=1)
        scores = jnp.einsum('bhqd,bhkd->bhqk', q, k) * Dh ** (-0.5)
        p = _softmax(scores, axis=-1)
        o = jnp.einsum('bhqk,bhkd->bhqd', p, v)
        return (lambda x, *d: x.transpose(*d))(o, 0, 2, 1, 3).reshape(B, Sq, Hq * Dh) @ wo

    def _B_ref(x, w_r, w_gate, w_up, w_down):
        B, S, D = x.shape
        C = 1
        r = x @ w_r
        idx = jnp.argsort(-r, axis=-1)[:, :C]
        idx_e = jnp.repeat(idx.reshape(B, C, 1), D, axis=2)
        x_sel = jnp.take_along_axis(x, idx_e, axis=1)
        g = _silu(x_sel @ w_gate)
        u = x_sel @ w_up
        y = g * u @ w_down
        r_sel = _sigmoid(jnp.take_along_axis(r, idx, axis=1))
        y = y * r_sel.reshape(B, C, 1)
        b_off = (jnp.arange(B) * S).reshape(B, 1)
        flat_idx = (idx + b_off).reshape(B * C)
        zero = (x * 0.0).reshape(B * S, D)
        upd = _scatter_add(zero, flat_idx, y.reshape(B * C, D), axis=0)
        return x + upd.reshape(B, S, D)
    x = A_x
    mod = (_silu(c) @ w_mod).reshape(c.shape[0], 6, 1, -1)
    sa, ca, ga, sb, cb, gb = (mod[:, 0].copy(), mod[:, 1].copy(), mod[:, 2].copy(), mod[:, 3].copy(), mod[:, 4].copy(), mod[:, 5].copy())
    h = _layernorm(x, axis=-1) * (1 + ca) + sa
    x = x + ga * _A_ref(h, A_k_cache, A_v_cache, A_wq, A_wo)
    h = _layernorm(x, axis=-1) * (1 + cb) + sb
    x = x + gb * _B_ref(h, B_w_r, B_w_gate, B_w_up, B_w_down)
    return x
```

```python
import functools

import jax
import jax.numpy as jnp
from jax import lax
import jax.experimental.pallas as pl
import jax.experimental.pallas.tpu as pltpu

f32 = jnp.float32
bf16 = jnp.bfloat16
u32 = jnp.uint32
i32 = jnp.int32

HQ = 32
DH = 128
TQ = 256
PR = 16
GAP = 2
EPS = 1e-05
LOG2E = 1.4426950408889634
M_SA, M_CA1, M_GA, M_SB, M_CB1, M_GB, M_WR = range(7)


def _rb(x):
    return x.astype(bf16).astype(f32)


def _silu(x):
    return x * (1.0 / (1.0 + jnp.exp(-x)))


def _dot(a, b):
    return jnp.dot(a, b, preferred_element_type=f32)


def _make_kernel(S, D, HKV, SK, W, F):
    NT = S // TQ
    NK = D // 128
    NS = TQ // PR
    REP = HQ // HKV
    QSCALE = DH ** (-0.5) * LOG2E
    NWM = 4
    WQ_CHUNKS = [(0, 1), (1, 2), (2, 4), (4, 9), (9, 17), (17, 25), (25, 32)]
    WO_CHUNKS = [(0, 0, D // 2), (0, D // 2, D), (1, 0, D), (2, 0, D), (3, 0, D)]

    def kernel(x_hbm, k_hbm, v_hbm, wq_hbm, wo_hbm, wr_hbm, wg_hbm, wu_hbm, wd_hbm, c_hbm, wm_hbm,
               out_hbm,
               xb, ob, hb, kb, vb, wq, wo, wg, wu, wd, wm, cb, wrb, modb, acc_ref, fix, flag,
               sem_in, sem_out):
        nsem = [0]

        def cp(src, dst):
            c = pltpu.make_async_copy(src, dst, sem_in.at[nsem[0]])
            nsem[0] += 1
            return c

        cp_c = cp(c_hbm, cb)
        cp_wr = cp(wr_hbm, wrb)
        cp_x0 = cp(x_hbm.at[0, pl.ds(0, TQ)], xb.at[pl.ds(0, TQ)])
        kc = D // NWM
        cp_wma = [cp(wm_hbm.at[pl.ds(i * kc, kc), pl.ds(0, 2 * D)],
                     wm.at[pl.ds(i * kc, kc), pl.ds(0, 2 * D)]) for i in range(NWM)]
        cp_wq = [cp(wq_hbm.at[:, pl.ds(a * DH, (b - a) * DH)], wq.at[:, pl.ds(a * DH, (b - a) * DH)])
                 for a, b in WQ_CHUNKS]
        cp_k0 = cp(k_hbm.at[0, pl.ds(0, 1), pl.ds(SK - W, W)], kb.at[pl.ds(0, 1)])
        cp_v0 = cp(v_hbm.at[0, pl.ds(0, 1), pl.ds(SK - W, W)], vb.at[pl.ds(0, 1)])
        cp_kr = cp(k_hbm.at[0, pl.ds(1, HKV - 1), pl.ds(SK - W, W)], kb.at[pl.ds(1, HKV - 1)])
        cp_vr = cp(v_hbm.at[0, pl.ds(1, HKV - 1), pl.ds(SK - W, W)], vb.at[pl.ds(1, HKV - 1)])
        go = REP * DH
        cp_wo = [cp(wo_hbm.at[pl.ds(g * go, go), pl.ds(a, b - a)], wo.at[pl.ds(g * go, go), pl.ds(a, b - a)])
                 for g, a, b in WO_CHUNKS]
        cp_x1 = cp(x_hbm.at[0, pl.ds(TQ, TQ)], xb.at[pl.ds(TQ, TQ)])
        cp_wmb = cp(wm_hbm.at[:, pl.ds(2 * D, 4 * D)], wm.at[:, pl.ds(2 * D, 4 * D)])
        cp_xr = cp(x_hbm.at[0, pl.ds(2 * TQ, S - 2 * TQ)], xb.at[pl.ds(2 * TQ, S - 2 * TQ)])
        cp_wg = cp(wg_hbm, wg)
        cp_wu = cp(wu_hbm, wu)
        cp_wd = cp(wd_hbm, wd)

        def cp_out(t):
            r0 = t * TQ if isinstance(t, int) else pl.multiple_of(t * TQ, TQ)
            return pltpu.make_async_copy(ob.at[pl.ds(r0, TQ)], out_hbm.at[0, pl.ds(r0, TQ)], sem_out.at[t])

        order = ([cp_c, cp_wr, cp_x0] + cp_wma
                 + [cp_wq[0], cp_k0, cp_wq[1], cp_v0, cp_wq[2], cp_wq[3], cp_wo[0], cp_wo[1],
                    cp_kr, cp_wq[4], cp_vr, cp_x1, cp_wo[2], cp_wq[5], cp_wo[3], cp_wq[6], cp_wo[4],
                    cp_wmb, cp_xr, cp_wg, cp_wu, cp_wd])
        for c in order:
            c.start()

        flag[0] = 0

        def bc8(row):
            return jnp.broadcast_to(row, (8, D))

        def tie(x, tok, never):
            if tok is None:
                return x
            return jnp.concatenate([jnp.where(never, tok, x[:, :128]), x[:, 128:]], axis=-1)

        def ln_plain(x):
            m = jnp.sum(x, axis=-1, keepdims=True) * (1.0 / D)
            xc = x - m
            v = jnp.sum(xc * xc, axis=-1, keepdims=True) * (1.0 / D)
            return xc * lax.rsqrt(v + EPS)

        def ln2_mod(x1):
            m = jnp.sum(x1, axis=-1, keepdims=True) * (1.0 / D)
            mb = _rb(m)
            xc = x1 - mb
            dm = m - mb
            v = jnp.sum(xc * xc, axis=-1, keepdims=True) * (1.0 / D) - dm * dm
            sd = _rb(jnp.sqrt(_rb(_rb(jnp.maximum(v, 0.0)) + EPS)))
            r0 = pl.reciprocal(sd, approx=True)
            rinv = r0 * (2.0 - sd * r0)
            return (xc * rinv) * modb[M_CB1][None] + modb[M_SB][None]

        def ln1_piece(r0, slot, i, tok=None, never=None):
            x = tie(xb[pl.ds(r0 + i * PR, PR), :].astype(f32), tok, never).reshape(PR // 8, 8, D)
            h = (ln_plain(x) * modb[M_CA1][None] + modb[M_SA][None]).reshape(PR, D).astype(bf16)
            h32 = pltpu.bitcast(h, u32)
            hb[slot, i * PR // 2:(i + 1) * PR // 2, :] = h32
            return h32[:, :128]

        sub_iota = lax.broadcasted_iota(i32, (8, 128), 0)

        def epi_piece(r0, best, i, tok=None, never=None):
            x1 = tie(xb[pl.ds(r0 + i * PR, PR), :].astype(f32), tok, never).reshape(PR // 8, 8, D)
            h2 = ln2_mod(x1)
            rr = jnp.sum(h2 * modb[M_WR][None], axis=-1, keepdims=True)
            rb16 = jnp.broadcast_to(rr.reshape(PR, 1), (PR, 128)).astype(bf16)
            rbf = rb16.astype(f32)
            for j in range(PR // 8):
                rj = rbf[8 * j:8 * j + 8]
                upd = rj > best[0]
                best[1] = jnp.where(upd, sub_iota + (r0 + i * PR + 8 * j), best[1])
                best[0] = jnp.where(upd, rj, best[0])
            ob[pl.ds(r0 + i * PR, PR), :] = (x1 + modb[M_GB][None] * h2).reshape(PR, D).astype(bf16)
            return pltpu.bitcast(rb16, u32)

        def attn_tile(r0, slot, pieces, never, waits, piece_groups, before_x1=None):
            def wait(key):
                for c in waits.pop(key, []):
                    c.wait()

            qs, ss, os_ = {}, {}, []
            acc = [None] * NK
            done, slotc = [0], [0]
            nslots = len(piece_groups) * (NK - GAP)
            hh = pltpu.bitcast(hb[slot], bf16)

            def qproj(b):
                wait(("q", b))
                qs[b] = (_dot(hh, wq[:, b * DH:(b + 1) * DH]) * QSCALE).astype(bf16)

            def qk(h):
                wait(("k", h))
                s = lax.dot_general(qs.pop(h), kb[h // REP], (((1,), (1,)), ((), ())),
                                    preferred_element_type=f32)
                m = jnp.max(s, axis=-1, keepdims=True)
                p = jnp.exp2(s - m)
                l = jnp.sum(p, axis=-1, keepdims=True)
                rl = pl.reciprocal(l, approx=True)
                ss[h] = (p.astype(bf16), rl * (2.0 - l * rl))

            def pv(h):
                wait(("v", h))
                p, rl = ss.pop(h)
                os_.append((_dot(p, vb[h // REP]) * rl).astype(bf16))

            def oproj(h0, h1):
                emit = (h0 // REP) in piece_groups
                outs = {}
                for n in range(NK):
                    wait(("o", h0, n))
                    cs = slice(n * 128, (n + 1) * 128)
                    o0 = os_[h0]
                    toks = outs.pop(n, [])
                    if toks:
                        o32 = pltpu.bitcast(o0, u32)
                        parts = [jnp.where(never, tok, o32[8 * k:8 * k + 8]) for k, tok in enumerate(toks)]
                        o0 = pltpu.bitcast(jnp.concatenate(parts + [o32[8 * len(toks):]], axis=0), bf16)
                    og = jnp.concatenate([o0] + os_[h0 + 1:h1], axis=-1)
                    a = _dot(og, wo[h0 * DH:h1 * DH, cs])
                    if h0 == 0:
                        acc_ref[:, cs] = a
                    elif h1 < HQ:
                        acc_ref[:, cs] += a
                    else:
                        acc[n] = acc_ref[:, cs] + a
                    if emit and n < NK - GAP:
                        slotc[0] += 1
                        tgt = int(round(slotc[0] * len(pieces) / nslots))
                        cnt = tgt - done[0]
                        for k in range(cnt):
                            rr = (k * TQ // cnt) // PR * PR
                            outs.setdefault(n + GAP, []).append(pieces[done[0]](a[rr:rr + PR], never))
                            done[0] += 1

            qproj(0)
            for h in range(HQ):
                qk(h)
                if h + 1 < HQ:
                    qproj(h + 1)
                else:
                    oproj(HQ - REP, HQ - REP // 2)
                pv(h)
                if h + 1 == HQ:
                    if before_x1 is not None:
                        before_x1()
                    oproj(HQ - REP // 2, HQ)
                elif (h + 1) % REP == 0:
                    oproj(h + 1 - REP, h + 1)
            assert done[0] == len(pieces) and not waits
            a = jnp.concatenate(acc, axis=-1).reshape(TQ // 8, 8, D) * modb[M_GA][None]
            xb[pl.ds(r0, TQ), :] = (xb[pl.ds(r0, TQ), :].astype(f32) + a.reshape(TQ, D)).astype(bf16)

        cp_c.wait()
        sc = jnp.broadcast_to(_silu(cb[...].astype(f32)).astype(bf16), (16, D))
        cp_wr.wait()
        modb[M_WR] = bc8(wrb[...].astype(f32))
        cp_x0.wait()
        ma = None
        for i in range(NWM):
            cp_wma[i].wait()
            part = _dot(sc[:, i * kc:(i + 1) * kc], wm[i * kc:(i + 1) * kc, 0:2 * D])
            ma = part if ma is None else ma + part
        ma = _rb(ma[0:8])
        modb[M_SA] = ma[:, 0:D]
        modb[M_CA1] = _rb(1.0 + ma[:, D:2 * D])
        for i in range(NS):
            ln1_piece(0, 0, i)

        def mod_rest():
            cp_wmb.wait()
            mb = _rb(_dot(sc, wm[:, 2 * D:6 * D])[0:8])
            modb[M_GA] = mb[:, 0:D]
            modb[M_SB] = mb[:, D:2 * D]
            modb[M_CB1] = _rb(1.0 + mb[:, 2 * D:3 * D])
            modb[M_GB] = mb[:, 3 * D:4 * D]

        never0 = flag[0] > 0
        waits = {}
        for (a, b), c in zip(WQ_CHUNKS, cp_wq):
            waits.setdefault(("q", a), []).append(c)
        for (g, a, b), c in zip(WO_CHUNKS, cp_wo):
            waits.setdefault(("o", g * REP, a // 128), []).append(c)
        waits[("k", 0)] = [cp_k0]
        waits[("v", 0)] = [cp_v0]
        waits[("k", REP)] = [cp_kr]
        waits[("v", REP)] = [cp_vr]
        waits[("o", REP, 0)].append(cp_x1)
        attn_tile(0, 0, [functools.partial(ln1_piece, TQ, 1, i) for i in range(NS)], never0, waits,
                  piece_groups=(1, 2), before_x1=mod_rest)
        cp_xr.wait()

        def body(t, carry):
            never = flag[0] > 0
            slot = t % 2
            r0 = pl.multiple_of(t * TQ, TQ)
            rp = pl.multiple_of((t - 1) * TQ, TQ)
            rn = pl.multiple_of(jnp.minimum(t + 1, NT - 1) * TQ, TQ)
            best = list(carry)
            pieces = []
            for i in range(NS):
                pieces += [functools.partial(epi_piece, rp, best, i),
                           functools.partial(ln1_piece, rn, 1 - slot, i)]
            attn_tile(r0, slot, pieces, never, {}, piece_groups=(0, 1, 2))
            cp_out(t - 1).start()
            return tuple(best)

        init = (jnp.full((8, 128), -jnp.inf, f32), jnp.zeros((8, 128), i32))
        best = list(lax.fori_loop(1, NT, body, init))

        for i in range(NS):
            epi_piece((NT - 1) * TQ, best, i)
        cp_out(NT - 1).start()

        bv, bi = best
        rmax = jnp.max(bv, axis=0, keepdims=True)
        imin = jnp.min(jnp.where(bv == rmax, bi, S), axis=0, keepdims=True)
        idx = jnp.minimum(imin[0, 0], S - 1)
        s0 = pl.multiple_of((idx // PR) * PR, PR)
        x1s = xb[pl.ds(s0, PR), :].astype(f32).reshape(PR // 8, 8, D)
        h2s = ln2_mod(x1s)
        lhs = h2s.reshape(PR, D).astype(bf16)
        cp_wg.wait()
        cp_wu.wait()
        cp_wd.wait()
        g = _rb(_silu(_rb(_dot(lhs, wg[...]))))
        u = _rb(_dot(lhs, wu[...]))
        y = _rb(_dot((g * u).astype(bf16), wd[...]))
        gate = _rb(1.0 / (1.0 + jnp.exp(-rmax[:, 0:1])))
        y = _rb(y * gate)
        rows = lax.broadcasted_iota(i32, (PR, D), 0) + s0
        upd = jnp.where(rows == idx, y, 0.0).reshape(PR // 8, 8, D)
        fix[...] = (x1s + modb[M_GB][None] * (h2s + upd)).reshape(PR, D).astype(bf16)
        for t in range(NT):
            cp_out(t).wait()
        cp_fix = pltpu.make_async_copy(fix, out_hbm.at[0, pl.ds(s0, PR)], sem_out.at[NT])
        cp_fix.start()
        cp_fix.wait()

    n_in_sems = 3 + NWM + len(WQ_CHUNKS) + 4 + len(WO_CHUNKS) + 6
    scratch = [
        pltpu.VMEM((S, D), bf16),
        pltpu.VMEM((S, D), bf16),
        pltpu.VMEM((2, TQ // 2, D), u32),
        pltpu.VMEM((HKV, W, DH), bf16),
        pltpu.VMEM((HKV, W, DH), bf16),
        pltpu.VMEM((D, HQ * DH), bf16),
        pltpu.VMEM((HQ * DH, D), bf16),
        pltpu.VMEM((D, F), bf16),
        pltpu.VMEM((D, F), bf16),
        pltpu.VMEM((F, D), bf16),
        pltpu.VMEM((D, 6 * D), bf16),
        pltpu.VMEM((1, D), bf16),
        pltpu.VMEM((1, D), bf16),
        pltpu.VMEM((7, 8, D), f32),
        pltpu.VMEM((TQ, D), f32),
        pltpu.VMEM((PR, D), bf16),
        pltpu.SMEM((1,), i32),
        pltpu.SemaphoreType.DMA((n_in_sems,)),
        pltpu.SemaphoreType.DMA((NT + 1,)),
    ]
    return kernel, scratch


@jax.jit
def pallas_adaLN_cond__sliding_block_cached__moe_arch_mod__prompt_kernel(
    A_x: jax.Array,
    A_k_cache: jax.Array,
    A_v_cache: jax.Array,
    A_wq: jax.Array,
    A_wo: jax.Array,
    B_x: jax.Array,
    B_w_r: jax.Array,
    B_w_gate: jax.Array,
    B_w_up: jax.Array,
    B_w_down: jax.Array,
    c: jax.Array,
    w_mod: jax.Array,
):
    B, S, D = A_x.shape
    _, HKV, SK, dh = A_k_cache.shape
    F = B_w_gate.shape[1]
    W = min(4096, max(256, SK // 4))
    assert B == 1 and dh == DH and A_wq.shape == (D, HQ * DH) and S % TQ == 0 and S >= 3 * TQ
    kernel, scratch = _make_kernel(S, D, HKV, SK, W, F)
    any_spec = pl.BlockSpec(memory_space=pl.ANY)
    return pl.pallas_call(
        kernel,
        out_shape=jax.ShapeDtypeStruct((B, S, D), A_x.dtype),
        in_specs=[any_spec] * 11,
        out_specs=any_spec,
        scratch_shapes=scratch,
        compiler_params=pltpu.CompilerParams(vmem_limit_bytes=110 * 1024 * 1024),
    )(A_x, A_k_cache, A_v_cache, A_wq, A_wo, B_w_r.reshape(1, D), B_w_gate, B_w_up, B_w_down, c, w_mod)
```

```python
import functools

import jax
import jax.numpy as jnp
from jax import lax
import jax.experimental.pallas as pl
import jax.experimental.pallas.tpu as pltpu

f32 = jnp.float32
bf16 = jnp.bfloat16
u32 = jnp.uint32
i32 = jnp.int32

HQ = 32
DH = 128
TQ = 256
PR = 16
GAP = 2
EPS = 1e-05
LOG2E = 1.4426950408889634
M_SA, M_CA1, M_GA, M_SB, M_CB1, M_GB, M_WR = range(7)


def _rb(x):
    return x.astype(bf16).astype(f32)


def _silu(x):
    return x * (1.0 / (1.0 + jnp.exp(-x)))


def _dot(a, b):
    return jnp.dot(a, b, preferred_element_type=f32)


def _make_kernel(S, D, HKV, SK, W, F):
    NT = S // TQ
    NK = D // 128
    NS = TQ // PR
    REP = HQ // HKV
    QSCALE = DH ** (-0.5) * LOG2E
    NWM = 4
    WQ_CHUNKS = [(0, 2), (2, 5), (5, 9), (9, 17), (17, 25), (25, 32)]
    PAD = 128

    n_in_sems = 2 + NT + NWM + len(WQ_CHUNKS) + 3 * HKV + 5

    def kernel(x_hbm, k_hbm, v_hbm, wq_hbm, wo_hbm, wr_hbm, wg_hbm, wu_hbm, wd_hbm, c_hbm, wm_hbm,
               out_hbm,
               xb, ob, hb, kb, vb, wq, wo, wg, wu, wd, wm, cb, wrb, modb, acc_ref, fix, flag,
               sem_in, sem_out):
        nsem = [0]

        def cp(src, dst):
            c = pltpu.make_async_copy(src, dst, sem_in.at[nsem[0]])
            nsem[0] += 1
            return c

        cp_c = cp(c_hbm, cb)
        cp_wr = cp(wr_hbm, wrb)
        cp_x = [cp(x_hbm.at[0, pl.ds(t * TQ, TQ)], xb.at[pl.ds(t * TQ, TQ)]) for t in range(3)]
        sem_x0 = nsem[0] - 3

        def x_copy(t):
            r0 = t * TQ if isinstance(t, int) else pl.multiple_of(t * TQ, TQ)
            return pltpu.make_async_copy(x_hbm.at[0, pl.ds(r0, TQ)], xb.at[pl.ds(r0, TQ)], sem_in.at[sem_x0 + t])

        cp_x += [x_copy(t) for t in range(3, NT)]
        nsem[0] += NT - 3
        kc = D // NWM
        cp_wma = [cp(wm_hbm.at[pl.ds(i * kc, kc), pl.ds(0, 2 * D)],
                     wm.at[pl.ds(i * kc, kc), pl.ds(0, 2 * D)]) for i in range(NWM)]
        cp_wq = [cp(wq_hbm.at[:, pl.ds(a * DH, (b - a) * DH)], wq.at[:, pl.ds(a * DH, (b - a) * DH)])
                 for a, b in WQ_CHUNKS]
        cp_k = [cp(k_hbm.at[0, g, pl.ds(SK - W, W)], kb.at[g]) for g in range(HKV)]
        cp_v = [cp(v_hbm.at[0, g, pl.ds(SK - W, W)], vb.at[g]) for g in range(HKV)]
        go = REP * DH
        cp_wo = [cp(wo_hbm.at[pl.ds(g * go, go)], wo.at[pl.ds(g * go, go)]) for g in range(HKV)]
        cp_wmg = cp(wm_hbm.at[:, pl.ds(2 * D, D)], wm.at[:, pl.ds(2 * D, D)])
        cp_wmb = cp(wm_hbm.at[:, pl.ds(3 * D, 3 * D)], wm.at[:, pl.ds(3 * D, 3 * D)])
        cp_wg = cp(wg_hbm, wg)
        cp_wu = cp(wu_hbm, wu)
        cp_wd = cp(wd_hbm, wd.at[:, pl.ds(0, D)])
        assert nsem[0] == n_in_sems

        def cp_out(t):
            r0 = t * TQ if isinstance(t, int) else pl.multiple_of(t * TQ, TQ)
            return pltpu.make_async_copy(ob.at[pl.ds(r0, TQ)], out_hbm.at[0, pl.ds(r0, TQ)], sem_out.at[t])

        order = ([cp_c, cp_wr, cp_x[0]] + cp_wma
                 + [cp_wq[0], cp_k[0], cp_v[0], cp_wq[1], cp_wq[2], cp_wo[0],
                    cp_k[1], cp_v[1], cp_wq[3], cp_wo[1], cp_x[1],
                    cp_k[2], cp_v[2], cp_wq[4], cp_wo[2], cp_k[3], cp_v[3], cp_wq[5], cp_wo[3],
                    cp_wmg, cp_wmb] + cp_x[2:] + [cp_wg, cp_wu, cp_wd])
        assert len(order) == n_in_sems
        for c in order:
            c.start()

        flag[0] = 0

        def bc8(row):
            return jnp.broadcast_to(row, (8, D))

        def tie(x, tok, never):
            if tok is None:
                return x
            return jnp.concatenate([jnp.where(never, tok, x[:, :128]), x[:, 128:]], axis=-1)

        def ln_plain(x):
            m = jnp.sum(x, axis=-1, keepdims=True) * (1.0 / D)
            xc = x - m
            v = jnp.sum(xc * xc, axis=-1, keepdims=True) * (1.0 / D)
            return xc * lax.rsqrt(v + EPS)

        def ln2_mod(x1):
            m = jnp.sum(x1, axis=-1, keepdims=True) * (1.0 / D)
            mb = _rb(m)
            xc = x1 - mb
            dm = m - mb
            v = jnp.sum(xc * xc, axis=-1, keepdims=True) * (1.0 / D) - dm * dm
            sd = _rb(jnp.sqrt(_rb(_rb(jnp.maximum(v, 0.0)) + EPS)))
            r0 = pl.reciprocal(sd, approx=True)
            rinv = r0 * (2.0 - sd * r0)
            return (xc * rinv) * modb[M_CB1][None] + modb[M_SB][None]

        def ln1_piece(r0, slot, i, tok=None, never=None):
            x = tie(xb[pl.ds(r0 + i * PR, PR), :].astype(f32), tok, never).reshape(PR // 8, 8, D)
            h = (ln_plain(x) * modb[M_CA1][None] + modb[M_SA][None]).reshape(PR, D).astype(bf16)
            h32 = pltpu.bitcast(h, u32)
            hb[slot, i * PR // 2:(i + 1) * PR // 2, :] = h32
            return h32[:, :128]

        sub_iota = lax.broadcasted_iota(i32, (8, 128), 0)

        def epi_piece(r0, best, i, tok=None, never=None):
            x1 = tie(xb[pl.ds(r0 + i * PR, PR), :].astype(f32), tok, never).reshape(PR // 8, 8, D)
            h2 = ln2_mod(x1)
            rr = jnp.sum(h2 * modb[M_WR][None], axis=-1, keepdims=True)
            rb16 = jnp.broadcast_to(rr.reshape(PR, 1), (PR, 128)).astype(bf16)
            rbf = rb16.astype(f32)
            for j in range(PR // 8):
                rj = rbf[8 * j:8 * j + 8]
                upd = rj > best[0]
                best[1] = jnp.where(upd, sub_iota + (r0 + i * PR + 8 * j), best[1])
                best[0] = jnp.where(upd, rj, best[0])
            ob[pl.ds(r0 + i * PR, PR), :] = (x1 + modb[M_GB][None] * h2).reshape(PR, D).astype(bf16)
            return pltpu.bitcast(rb16, u32)

        def attn_tile(r0, slot, pieces, never, waits, piece_groups, before_x1=None):
            def wait(key):
                for c in waits.pop(key, []):
                    c.wait()

            qs, ss, os_ = {}, {}, []
            acc = [None] * NK
            done, slotc = [0], [0]
            nslots = len(piece_groups) * (NK - GAP)
            hh = pltpu.bitcast(hb[slot], bf16)

            def qproj(b):
                wait(("q", b))
                qs[b] = (_dot(hh, wq[:, b * DH:(b + 1) * DH]) * QSCALE).astype(bf16)

            def qk(h):
                wait(("k", h))
                s = lax.dot_general(qs.pop(h), kb[h // REP], (((1,), (1,)), ((), ())),
                                    preferred_element_type=f32)
                m = jnp.max(s, axis=-1, keepdims=True)
                p = jnp.exp2(s - m)
                l = jnp.sum(p, axis=-1, keepdims=True)
                rl = pl.reciprocal(l, approx=True)
                ss[h] = (p.astype(bf16), rl * (2.0 - l * rl))

            def pv(h):
                wait(("v", h))
                p, rl = ss.pop(h)
                os_.append((_dot(p, vb[h // REP]) * rl).astype(bf16))

            def oproj(h0, h1):
                emit = (h0 // REP) in piece_groups
                outs = {}
                for n in range(NK):
                    wait(("o", h0, n))
                    cs = slice(n * 128, (n + 1) * 128)
                    o0 = os_[h0]
                    toks = outs.pop(n, [])
                    if toks:
                        o32 = pltpu.bitcast(o0, u32)
                        parts = [jnp.where(never, tok, o32[8 * k:8 * k + 8]) for k, tok in enumerate(toks)]
                        o0 = pltpu.bitcast(jnp.concatenate(parts + [o32[8 * len(toks):]], axis=0), bf16)
                    og = jnp.concatenate([o0] + os_[h0 + 1:h1], axis=-1)
                    a = _dot(og, wo[h0 * DH:h1 * DH, cs])
                    if h0 == 0:
                        acc_ref[:, cs] = a
                    elif h1 < HQ:
                        acc_ref[:, cs] += a
                    else:
                        acc[n] = acc_ref[:, cs] + a
                    if emit and n < NK - GAP:
                        slotc[0] += 1
                        tgt = int(round(slotc[0] * len(pieces) / nslots))
                        cnt = tgt - done[0]
                        for k in range(cnt):
                            rr = (k * TQ // cnt) // PR * PR
                            outs.setdefault(n + GAP, []).append(pieces[done[0]](a[rr:rr + PR], never))
                            done[0] += 1

            qproj(0)
            for h in range(HQ):
                qk(h)
                if h + 1 < HQ:
                    qproj(h + 1)
                else:
                    oproj(HQ - REP, HQ - REP // 2)
                pv(h)
                if h + 1 == HQ:
                    if before_x1 is not None:
                        before_x1()
                    oproj(HQ - REP // 2, HQ)
                elif (h + 1) % REP == 0:
                    oproj(h + 1 - REP, h + 1)
            assert done[0] == len(pieces) and not waits
            a = jnp.concatenate(acc, axis=-1).reshape(TQ // 8, 8, D) * modb[M_GA][None]
            xb[pl.ds(r0, TQ), :] = (xb[pl.ds(r0, TQ), :].astype(f32) + a.reshape(TQ, D)).astype(bf16)

        cp_c.wait()
        sc = jnp.broadcast_to(_silu(cb[...].astype(f32)).astype(bf16), (16, D))
        cp_wr.wait()
        modb[M_WR] = bc8(wrb[...].astype(f32).reshape(1, D))
        cp_x[0].wait()
        ma = None
        for i in range(NWM):
            cp_wma[i].wait()
            part = _dot(sc[:, i * kc:(i + 1) * kc], wm[i * kc:(i + 1) * kc, 0:2 * D])
            ma = part if ma is None else ma + part
        ma = _rb(ma[0:8])
        modb[M_SA] = ma[:, 0:D]
        modb[M_CA1] = _rb(1.0 + ma[:, D:2 * D])
        for i in range(NS):
            ln1_piece(0, 0, i)

        def mod_gate():
            modb[M_GA] = _rb(_dot(sc, wm[:, 2 * D:3 * D])[0:8])

        never0 = flag[0] > 0
        waits = {
            ("q", 0): [cp_wq[0], cp_k[0], cp_v[0]],
            ("k", 1): [cp_wq[1]],
            ("k", 4): [cp_wq[2]],
            ("o", 0, 0): [cp_wo[0]],
            ("k", REP): [cp_k[1], cp_v[1], cp_wq[3]],
            ("o", REP, 0): [cp_wo[1], cp_x[1]],
            ("k", 2 * REP): [cp_k[2], cp_v[2], cp_wq[4]],
            ("o", 2 * REP, 0): [cp_wo[2], cp_k[3], cp_v[3], cp_wq[5]],
            ("k", HQ - 1): [cp_wo[3], cp_wmg],
        }
        attn_tile(0, 0, [functools.partial(ln1_piece, TQ, 1, i) for i in range(NS)], never0, waits,
                  piece_groups=(1, 2), before_x1=mod_gate)
        cp_wmb.wait()
        mb = _rb(_dot(sc, wm[:, 3 * D:6 * D])[0:8])
        modb[M_SB] = mb[:, 0:D]
        modb[M_CB1] = _rb(1.0 + mb[:, D:2 * D])
        modb[M_GB] = mb[:, 2 * D:3 * D]

        def body(t, carry):
            @pl.when(t + 1 < NT)
            def _():
                x_copy(t + 1).wait()

            never = flag[0] > 0
            slot = t % 2
            r0 = pl.multiple_of(t * TQ, TQ)
            rp = pl.multiple_of((t - 1) * TQ, TQ)
            rn = pl.multiple_of(jnp.minimum(t + 1, NT - 1) * TQ, TQ)
            best = list(carry)
            pieces = []
            for i in range(NS):
                pieces += [functools.partial(epi_piece, rp, best, i),
                           functools.partial(ln1_piece, rn, 1 - slot, i)]
            attn_tile(r0, slot, pieces, never, {}, piece_groups=(0, 1, 2))
            cp_out(t - 1).start()
            return tuple(best)

        init = (jnp.full((8, 128), -jnp.inf, f32), jnp.zeros((8, 128), i32))
        best = list(lax.fori_loop(1, NT, body, init))

        cp_wg.wait()
        cp_wu.wait()
        cp_wd.wait()
        for i in range(NS):
            epi_piece((NT - 1) * TQ, best, i)

        bv, bi = best
        rmax = jnp.max(bv, axis=0, keepdims=True)
        imin = jnp.min(jnp.where(bv == rmax, bi, S), axis=0, keepdims=True)
        idx = jnp.minimum(imin[0, 0], S - 1)
        s0 = pl.multiple_of((idx // PR) * PR, PR)
        x1s = xb[pl.ds(s0, PR), :].astype(f32).reshape(PR // 8, 8, D)
        h2s = ln2_mod(x1s)
        lhs = h2s.reshape(PR, D).astype(bf16)
        g = _rb(_silu(_rb(_dot(lhs, wg[...]))))
        u = _rb(_dot(lhs, wu[...]))
        cp_out(NT - 1).start()
        y = _rb(_dot((g * u).astype(bf16), wd[:, 0:D]))
        gate = _rb(1.0 / (1.0 + jnp.exp(-rmax[:, 0:1])))
        y = _rb(y * gate)
        rows = lax.broadcasted_iota(i32, (PR, D), 0) + s0
        upd = jnp.where(rows == idx, y, 0.0).reshape(PR // 8, 8, D)
        fix[...] = (x1s + modb[M_GB][None] * (h2s + upd)).reshape(PR, D).astype(bf16)
        for t in range(NT):
            cp_out(t).wait()
        cp_fix = pltpu.make_async_copy(fix, out_hbm.at[0, pl.ds(s0, PR)], sem_out.at[NT])
        cp_fix.start()
        cp_fix.wait()

    scratch = [
        pltpu.VMEM((S, D), bf16),
        pltpu.VMEM((S, D), bf16),
        pltpu.VMEM((2, TQ // 2, D), u32),
        pltpu.VMEM((HKV, W, DH), bf16),
        pltpu.VMEM((HKV, W, DH), bf16),
        pltpu.VMEM((D, HQ * DH), bf16),
        pltpu.VMEM((HQ * DH, D), bf16),
        pltpu.VMEM((D, F), bf16),
        pltpu.VMEM((D, F), bf16),
        pltpu.VMEM((F, D + PAD), bf16),
        pltpu.VMEM((D, 6 * D + PAD), bf16),
        pltpu.VMEM((1, D), bf16),
        pltpu.VMEM((D,), bf16),
        pltpu.VMEM((7, 8, D), f32),
        pltpu.VMEM((TQ, D), f32),
        pltpu.VMEM((PR, D), bf16),
        pltpu.SMEM((1,), i32),
        pltpu.SemaphoreType.DMA((n_in_sems,)),
        pltpu.SemaphoreType.DMA((NT + 1,)),
    ]
    return kernel, scratch


@jax.jit
def pallas_adaLN_cond__sliding_block_cached__moe_arch_mod__prompt_kernel(
    A_x: jax.Array,
    A_k_cache: jax.Array,
    A_v_cache: jax.Array,
    A_wq: jax.Array,
    A_wo: jax.Array,
    B_x: jax.Array,
    B_w_r: jax.Array,
    B_w_gate: jax.Array,
    B_w_up: jax.Array,
    B_w_down: jax.Array,
    c: jax.Array,
    w_mod: jax.Array,
):
    B, S, D = A_x.shape
    _, HKV, SK, dh = A_k_cache.shape
    F = B_w_gate.shape[1]
    W = min(4096, max(256, SK // 4))
    assert B == 1 and dh == DH and A_wq.shape == (D, HQ * DH) and S % TQ == 0 and S >= 3 * TQ
    kernel, scratch = _make_kernel(S, D, HKV, SK, W, F)
    any_spec = pl.BlockSpec(memory_space=pl.ANY)
    return pl.pallas_call(
        kernel,
        out_shape=jax.ShapeDtypeStruct((B, S, D), A_x.dtype),
        in_specs=[any_spec] * 11,
        out_specs=any_spec,
        scratch_shapes=scratch,
        compiler_params=pltpu.CompilerParams(vmem_limit_bytes=110 * 1024 * 1024),
    )(A_x, A_k_cache, A_v_cache, A_wq, A_wo, B_w_r, B_w_gate, B_w_up, B_w_down, c, w_mod)
```

```python
import functools

import jax
import jax.numpy as jnp
from jax import lax
import jax.experimental.pallas as pl
import jax.experimental.pallas.tpu as pltpu

f32 = jnp.float32
bf16 = jnp.bfloat16
u32 = jnp.uint32
i32 = jnp.int32

HQ = 32
DH = 128
TQ = 256
PR = 16
EPS = 1e-05
LOG2E = 1.4426950408889634
NWM = 4
QA = 3
PAD = 128
NMLP = 2
M_SA, M_CA1, M_GA, M_SB, M_CB1, M_GB, M_WR = range(7)


def _rb(x):
    return x.astype(bf16).astype(f32)


def _silu(x):
    return x * (1.0 / (1.0 + jnp.exp(-x)))


def _dot(a, b):
    return jnp.dot(a, b, preferred_element_type=f32)


def _mult(i, n):
    return i * n if isinstance(i, int) else pl.multiple_of(i * n, n)


def _make_kernel(S, D, HKV, SK, W, F):
    NT = S // TQ
    NK = D // 128
    NS = TQ // PR
    REP = HQ // HKV
    GD = REP * DH
    QSCALE = DH ** (-0.5) * LOG2E
    KC = D // NWM
    XQ = TQ // HKV
    FC = F // NMLP

    sem_base, n_in_sems = {}, 0
    for name, n in (("c", 1), ("wr", 1), ("x", NT), ("x1", HKV), ("wma", NWM), ("wqa", HKV), ("wqb", HKV),
                    ("k", HKV), ("v", HKV), ("wo", HKV), ("wmb", 1), ("wg", NMLP), ("wu", NMLP), ("wd", 1)):
        sem_base[name] = n_in_sems
        n_in_sems += n

    def kernel(x_hbm, k_hbm, v_hbm, wq_hbm, wo_hbm, wr_hbm, wg_hbm, wu_hbm, wd_hbm, c_hbm, wm_hbm,
               out_hbm,
               xb, ob, hb, kb, vb, wq, wo, wg, wu, wd, wm, cb, wrb, scb, modb, acc_ref, xn_ref, fix, flag,
               sem_in, sem_out):
        def cp(name, i, src, dst):
            return pltpu.make_async_copy(src, dst, sem_in.at[sem_base[name] + i])

        def cp_x(t):
            r = pl.ds(_mult(t, TQ), TQ)
            return cp("x", t, x_hbm.at[0, r], xb.at[r])

        def cp_x1(g):
            r = pl.ds(TQ + _mult(g, XQ), XQ)
            return cp("x1", g, x_hbm.at[0, r], xb.at[r])

        def cp_wma(i):
            r = pl.ds(_mult(i, KC), KC)
            return cp("wma", i, wm_hbm.at[r, pl.ds(0, 2 * D)], wm.at[r, pl.ds(0, 2 * D)])

        def cp_wqa(g):
            return cp("wqa", g, wq_hbm.at[:, pl.ds(_mult(g, GD), QA * DH)], wq.at[g, :, pl.ds(0, QA * DH)])

        def cp_wqb(g):
            n = GD - QA * DH
            return cp("wqb", g, wq_hbm.at[:, pl.ds(_mult(g, GD) + QA * DH, n)], wq.at[g, :, pl.ds(QA * DH, n)])

        def cp_k(g):
            return cp("k", g, k_hbm.at[0, g, pl.ds(SK - W, W)], kb.at[g])

        def cp_v(g):
            return cp("v", g, v_hbm.at[0, g, pl.ds(SK - W, W)], vb.at[g])

        def cp_wo(g):
            return cp("wo", g, wo_hbm.at[pl.ds(_mult(g, GD), GD)], wo.at[g])

        cp_c = cp("c", 0, c_hbm, cb)
        cp_wr = cp("wr", 0, wr_hbm, wrb)
        cp_wmb = cp("wmb", 0, wm_hbm.at[:, pl.ds(2 * D, 4 * D)], wm.at[:, pl.ds(2 * D, 4 * D)])
        cp_wg = [cp("wg", j, wg_hbm.at[:, pl.ds(j * FC, FC)], wg.at[j, :, pl.ds(0, FC)]) for j in range(NMLP)]
        cp_wu = [cp("wu", j, wu_hbm.at[:, pl.ds(j * FC, FC)], wu.at[j, :, pl.ds(0, FC)]) for j in range(NMLP)]
        cp_wd = cp("wd", 0, wd_hbm, wd.at[:, pl.ds(0, D)])

        def cp_out(t):
            r = pl.ds(_mult(t, TQ), TQ)
            return pltpu.make_async_copy(ob.at[r], out_hbm.at[0, r], sem_out.at[t])

        order = [cp_c, cp_x(0)] + [cp_wma(i) for i in range(NWM)]
        for g in range(HKV):
            order += [cp_wqa(g), cp_k(g), cp_v(g), cp_wqb(g), cp_wo(g), cp_x1(g)]
        order += [cp_wr, cp_wmb] + [cp_x(t) for t in range(2, NT)] + cp_wg + cp_wu + [cp_wd]
        for c in order:
            c.start()

        flag[0] = 0

        def tie(x, tok, never):
            if tok is None:
                return x
            return jnp.concatenate([jnp.where(never, tok, x[:, :128]), x[:, 128:]], axis=-1)

        def ln_plain(x):
            m = jnp.sum(x, axis=-1, keepdims=True) * (1.0 / D)
            xc = x - m
            v = jnp.sum(xc * xc, axis=-1, keepdims=True) * (1.0 / D)
            return xc * lax.rsqrt(v + EPS)

        def ln2_mod(x1):
            m = jnp.sum(x1, axis=-1, keepdims=True) * (1.0 / D)
            mb = _rb(m)
            xc = x1 - mb
            dm = m - mb
            v = jnp.sum(xc * xc, axis=-1, keepdims=True) * (1.0 / D) - dm * dm
            sd = _rb(jnp.sqrt(_rb(_rb(jnp.maximum(v, 0.0)) + EPS)))
            r0 = pl.reciprocal(sd, approx=True)
            rinv = r0 * (2.0 - sd * r0)
            return (xc * rinv) * modb[M_CB1][None] + modb[M_SB][None]

        def ln1_piece(xrow, slot, hrow, tok=None, never=None):
            x = tie(xb[pl.ds(xrow, PR), :].astype(f32), tok, never).reshape(PR // 8, 8, D)
            h = (ln_plain(x) * modb[M_CA1][None] + modb[M_SA][None]).reshape(PR, D).astype(bf16)
            h32 = pltpu.bitcast(h, u32)
            hb[slot, pl.ds(hrow, PR // 2), :] = h32
            return h32[:, :128]

        sub_iota = lax.broadcasted_iota(i32, (8, 128), 0)

        def epi_piece(row, best, tok=None, never=None):
            x1 = tie(xb[pl.ds(row, PR), :].astype(f32), tok, never).reshape(PR // 8, 8, D)
            h2 = ln2_mod(x1)
            rr = jnp.sum(h2 * modb[M_WR][None], axis=-1, keepdims=True)
            rb16 = jnp.broadcast_to(rr.reshape(PR, 1), (PR, 128)).astype(bf16)
            rbf = rb16.astype(f32)
            for j in range(PR // 8):
                rj = rbf[8 * j:8 * j + 8]
                upd = rj > best[0]
                best[1] = jnp.where(upd, sub_iota + (row + 8 * j), best[1])
                best[0] = jnp.where(upd, rj, best[0])
            ob[pl.ds(row, PR), :] = (x1 + modb[M_GB][None] * h2).reshape(PR, D).astype(bf16)
            return pltpu.bitcast(rb16, u32)

        def qproj(hh, g, j):
            return (_dot(hh, wq[g, :, j * DH:(j + 1) * DH]) * QSCALE).astype(bf16)

        def qk(q, g):
            s = lax.dot_general(q, kb[g], (((1,), (1,)), ((), ())), preferred_element_type=f32)
            m = jnp.max(s, axis=-1, keepdims=True)
            p = jnp.exp2(s - m)
            l = jnp.sum(p, axis=-1, keepdims=True)
            rl = pl.reciprocal(l, approx=True)
            return p.astype(bf16), rl * (2.0 - l * rl)

        def pv(prl, g):
            p, rl = prl
            return (_dot(p, vb[g]) * rl).astype(bf16)

        def oproj(os_, g, j0, sink, pieces, gap, never):
            outs, done = {}, 0
            for n in range(NK):
                cs = slice(n * 128, (n + 1) * 128)
                o0 = os_[0]
                toks = outs.pop(n, [])
                if toks:
                    o32 = pltpu.bitcast(o0, u32)
                    parts = [jnp.where(never, tok, o32[8 * k:8 * k + 8]) for k, tok in enumerate(toks)]
                    o0 = pltpu.bitcast(jnp.concatenate(parts + [o32[8 * len(toks):]], axis=0), bf16)
                og = jnp.concatenate([o0] + list(os_[1:]), axis=-1)
                a = _dot(og, wo[g, j0 * DH:(j0 + len(os_)) * DH, cs])
                sink(n, cs, a)
                if n < NK - gap:
                    cnt = int(round((n + 1) * len(pieces) / (NK - gap))) - done
                    for k in range(cnt):
                        rr = (k * TQ // cnt) // PR * PR
                        outs.setdefault(n + gap, []).append(pieces[done](a[rr:rr + PR], never))
                        done += 1
            assert done == len(pieces)

        def acc_set(n, cs, a):
            acc_ref[:, cs] = a

        def acc_add(n, cs, a):
            acc_ref[:, cs] += a

        def write_x1(r0, acc):
            a = acc.reshape(TQ // 8, 8, D) * modb[M_GA][None]
            xb[pl.ds(r0, TQ), :] = (xb[pl.ds(r0, TQ), :].astype(f32) + a.reshape(TQ, D)).astype(bf16)

        acc_ref[...] = jnp.zeros((TQ, D), f32)
        cp_c.wait()
        sc = jnp.broadcast_to(_silu(cb[...].astype(f32)).astype(bf16), (16, D))
        for i in range(NWM):
            scb[i] = sc[:, i * KC:(i + 1) * KC]
        cp_x(0).wait()

        def ln0(i, c):
            r = pl.ds(pl.multiple_of(i * 64, 64), 64)
            xn_ref[r, :] = ln_plain(xb[r, :].astype(f32))
            return c

        lax.fori_loop(0, TQ // 64, ln0, 0)

        def moda(i, ma):
            cp_wma(i).wait()
            return ma + _dot(scb[i], wm[pl.ds(_mult(i, KC), KC), 0:2 * D])[0:8]

        ma = _rb(lax.fori_loop(0, NWM, moda, jnp.zeros((8, 2 * D), f32)))
        sa = ma[:, 0:D]
        ca1 = _rb(1.0 + ma[:, D:2 * D])
        modb[M_SA] = sa
        modb[M_CA1] = ca1
        h0 = (xn_ref[...].reshape(TQ // 8, 8, D) * ca1[None] + sa[None]).reshape(TQ, D).astype(bf16)
        hb[0] = pltpu.bitcast(h0, u32)

        def group0(g, c):
            never = flag[0] > 0
            cp_wqa(g).wait()
            cp_k(g).wait()
            cp_v(g).wait()
            q = qproj(pltpu.bitcast(hb[0], bf16), g, 0)
            os_ = []
            for j in range(REP):
                if j == QA - 1:
                    cp_wqb(g).wait()
                if j == REP - 1:
                    cp_wo(g).wait()
                    cp_x1(g).wait()
                prl = qk(q, g)
                if j + 1 < REP:
                    q = qproj(pltpu.bitcast(hb[0], bf16), g, j + 1)
                else:
                    oproj(os_[:REP // 2], g, 0, acc_add, [], 0, never)
                os_.append(pv(prl, g))
            xr = _mult(g, XQ)
            hr = _mult(g, XQ // 2)
            pieces = [functools.partial(ln1_piece, TQ + xr + i * PR, 1, hr + i * PR // 2)
                      for i in range(XQ // PR)]
            oproj(os_[REP // 2:], g, REP // 2, acc_add, pieces, 4, never)
            return c

        lax.fori_loop(0, HKV, group0, 0)

        cp_wr.wait()
        cp_wmb.wait()
        modb[M_WR] = jnp.broadcast_to(wrb[...].astype(f32).reshape(1, D), (8, D))
        modb[M_GA] = _rb(_dot(sc, wm[:, 2 * D:3 * D])[0:8])
        mb = _rb(_dot(sc, wm[:, 3 * D:6 * D])[0:8])
        modb[M_SB] = mb[:, 0:D]
        modb[M_CB1] = _rb(1.0 + mb[:, D:2 * D])
        modb[M_GB] = mb[:, 2 * D:3 * D]
        write_x1(0, acc_ref[...])

        def body(t, carry):
            @pl.when(t + 1 < NT)
            def _():
                cp_x(t + 1).wait()

            never = flag[0] > 0
            slot = t % 2
            r0 = _mult(t, TQ)
            rp = _mult(t - 1, TQ)
            rn = _mult(jnp.minimum(t + 1, NT - 1), TQ)
            best = list(carry)
            pieces = []
            for i in range(NS):
                pieces += [functools.partial(epi_piece, rp + i * PR, best),
                           functools.partial(ln1_piece, rn + i * PR, 1 - slot, i * PR // 2)]
            npg = -(-len(pieces) // (HKV - 1))
            hh = pltpu.bitcast(hb[slot], bf16)
            fin = [None] * NK

            def acc_fin(n, cs, a):
                fin[n] = acc_ref[:, cs] + a

            q = qproj(hh, 0, 0)
            for g in range(HKV):
                os_ = []
                for j in range(REP):
                    prl = qk(q, g)
                    if j + 1 < REP:
                        q = qproj(hh, g, j + 1)
                    elif g + 1 < HKV:
                        q = qproj(hh, g + 1, 0)
                    else:
                        oproj(os_[:REP // 2], g, 0, acc_add, [], 0, never)
                    os_.append(pv(prl, g))
                if g + 1 < HKV:
                    oproj(os_, g, 0, acc_set if g == 0 else acc_add, pieces[g * npg:(g + 1) * npg], 2, never)
                else:
                    oproj(os_[REP // 2:], g, REP // 2, acc_fin, [], 0, never)
            write_x1(r0, jnp.concatenate(fin, axis=-1))
            cp_out(t - 1).start()
            return tuple(best)

        init = (jnp.full((8, 128), -jnp.inf, f32), jnp.zeros((8, 128), i32))
        best = list(lax.fori_loop(1, NT, body, init))

        for c in cp_wg + cp_wu + [cp_wd]:
            c.wait()
        for i in range(NS):
            epi_piece((NT - 1) * TQ + i * PR, best)
        cp_out(NT - 1).start()

        bv, bi = best
        rmax = jnp.max(bv, axis=0, keepdims=True)
        imin = jnp.min(jnp.where(bv == rmax, bi, S), axis=0, keepdims=True)
        idx = jnp.minimum(imin[0, 0], S - 1)
        s0 = pl.multiple_of((idx // PR) * PR, PR)
        x1s = xb[pl.ds(s0, PR), :].astype(f32).reshape(PR // 8, 8, D)
        h2s = ln2_mod(x1s)
        lhs = h2s.reshape(PR, D).astype(bf16)

        def mlp(j, y):
            gt = _rb(_silu(_rb(_dot(lhs, wg[j, :, 0:FC]))))
            up = _rb(_dot(lhs, wu[j, :, 0:FC]))
            return y + _dot((gt * up).astype(bf16), wd[pl.ds(_mult(j, FC), FC), 0:D])

        y = _rb(lax.fori_loop(0, NMLP, mlp, jnp.zeros((PR, D), f32)))
        gate = _rb(1.0 / (1.0 + jnp.exp(-rmax[:, 0:1])))
        y = _rb(y * gate)
        rows = lax.broadcasted_iota(i32, (PR, D), 0) + s0
        upd = jnp.where(rows == idx, y, 0.0).reshape(PR // 8, 8, D)
        fix[...] = (x1s + modb[M_GB][None] * (h2s + upd)).reshape(PR, D).astype(bf16)
        for t in range(NT):
            cp_out(t).wait()
        cp_fix = pltpu.make_async_copy(fix, out_hbm.at[0, pl.ds(s0, PR)], sem_out.at[NT])
        cp_fix.start()
        cp_fix.wait()

    scratch = [
        pltpu.VMEM((S, D), bf16),
        pltpu.VMEM((S, D), bf16),
        pltpu.VMEM((2, TQ // 2, D), u32),
        pltpu.VMEM((HKV, W, DH), bf16),
        pltpu.VMEM((HKV, W, DH), bf16),
        pltpu.VMEM((HKV, D, GD), bf16),
        pltpu.VMEM((HKV, GD, D), bf16),
        pltpu.VMEM((NMLP, D, FC + PAD), bf16),
        pltpu.VMEM((NMLP, D, FC + PAD), bf16),
        pltpu.VMEM((F, D + PAD), bf16),
        pltpu.VMEM((D, 6 * D + PAD), bf16),
        pltpu.VMEM((1, D), bf16),
        pltpu.VMEM((D,), bf16),
        pltpu.VMEM((NWM, 16, KC), bf16),
        pltpu.VMEM((7, 8, D), f32),
        pltpu.VMEM((TQ, D), f32),
        pltpu.VMEM((TQ, D), f32),
        pltpu.VMEM((PR, D), bf16),
        pltpu.SMEM((1,), i32),
        pltpu.SemaphoreType.DMA((n_in_sems,)),
        pltpu.SemaphoreType.DMA((NT + 1,)),
    ]
    return kernel, scratch


@jax.jit
def pallas_adaLN_cond__sliding_block_cached__moe_arch_mod__prompt_kernel(
    A_x: jax.Array,
    A_k_cache: jax.Array,
    A_v_cache: jax.Array,
    A_wq: jax.Array,
    A_wo: jax.Array,
    B_x: jax.Array,
    B_w_r: jax.Array,
    B_w_gate: jax.Array,
    B_w_up: jax.Array,
    B_w_down: jax.Array,
    c: jax.Array,
    w_mod: jax.Array,
):
    B, S, D = A_x.shape
    _, HKV, SK, dh = A_k_cache.shape
    F = B_w_gate.shape[1]
    W = min(4096, max(256, SK // 4))
    assert B == 1 and dh == DH and A_wq.shape == (D, HQ * DH) and S % TQ == 0 and S >= 3 * TQ
    kernel, scratch = _make_kernel(S, D, HKV, SK, W, F)
    any_spec = pl.BlockSpec(memory_space=pl.ANY)
    return pl.pallas_call(
        kernel,
        out_shape=jax.ShapeDtypeStruct((B, S, D), A_x.dtype),
        in_specs=[any_spec] * 11,
        out_specs=any_spec,
        scratch_shapes=scratch,
        compiler_params=pltpu.CompilerParams(vmem_limit_bytes=110 * 1024 * 1024),
    )(A_x, A_k_cache, A_v_cache, A_wq, A_wo, B_w_r, B_w_gate, B_w_up, B_w_down, c, w_mod)
```

```python
import functools

import jax
import jax.numpy as jnp
from jax import lax
import jax.experimental.pallas as pl
import jax.experimental.pallas.tpu as pltpu

f32 = jnp.float32
bf16 = jnp.bfloat16
u32 = jnp.uint32
i32 = jnp.int32

HQ = 32
DH = 128
TQ = 256
PR = 16
EPS = 1e-05
LOG2E = 1.4426950408889634
NWM = 4
QA = 3
PAD = 128
NMLP = 2
M_SA, M_CA1, M_GA, M_SB, M_CB1, M_GB, M_WR = range(7)


def _rb(x):
    return x.astype(bf16).astype(f32)


def _silu(x):
    return x * (1.0 / (1.0 + jnp.exp(-x)))


def _dot(a, b):
    return jnp.dot(a, b, preferred_element_type=f32)


def _mult(i, n):
    return i * n if isinstance(i, int) else pl.multiple_of(i * n, n)


def _make_kernel(S, D, HKV, SK, W, F):
    NT = S // TQ
    NK = D // 128
    NS = TQ // PR
    REP = HQ // HKV
    GD = REP * DH
    QSCALE = DH ** (-0.5) * LOG2E
    KC = D // NWM
    XQ = TQ // HKV
    FC = F // NMLP

    sem_base, n_in_sems = {}, 0
    for name, n in (("c", 1), ("wr", 1), ("x", NT), ("x1", HKV), ("wma", NWM), ("wqa", HKV), ("wqb", HKV),
                    ("k", HKV), ("v", HKV), ("wo", HKV), ("wmb", 1), ("wg", NMLP), ("wu", NMLP), ("wd", 1)):
        sem_base[name] = n_in_sems
        n_in_sems += n

    def kernel(x_hbm, k_hbm, v_hbm, wq_hbm, wo_hbm, wr_hbm, wg_hbm, wu_hbm, wd_hbm, c_hbm, wm_hbm,
               out_hbm,
               xb, ob, hb, kb, vb, wq, wo, wg, wu, wd, wm, cb, wrb, scb, modb, acc_ref, xn_ref, fix, flag,
               sem_in, sem_out):
        def cp(name, i, src, dst):
            return pltpu.make_async_copy(src, dst, sem_in.at[sem_base[name] + i])

        def cp_x(t):
            r = pl.ds(_mult(t, TQ), TQ)
            return cp("x", t, x_hbm.at[0, r], xb.at[r])

        def cp_x1(g):
            r = pl.ds(TQ + _mult(g, XQ), XQ)
            return cp("x1", g, x_hbm.at[0, r], xb.at[r])

        def cp_wma(i):
            r = pl.ds(_mult(i, KC), KC)
            return cp("wma", i, wm_hbm.at[r, pl.ds(0, 2 * D)], wm.at[r, pl.ds(0, 2 * D)])

        def cp_wqa(g):
            return cp("wqa", g, wq_hbm.at[:, pl.ds(_mult(g, GD), QA * DH)], wq.at[g, :, pl.ds(0, QA * DH)])

        def cp_wqb(g):
            n = GD - QA * DH
            return cp("wqb", g, wq_hbm.at[:, pl.ds(_mult(g, GD) + QA * DH, n)], wq.at[g, :, pl.ds(QA * DH, n)])

        def cp_k(g):
            return cp("k", g, k_hbm.at[0, g, pl.ds(SK - W, W)], kb.at[g])

        def cp_v(g):
            return cp("v", g, v_hbm.at[0, g, pl.ds(SK - W, W)], vb.at[g])

        def cp_wo(g):
            return cp("wo", g, wo_hbm.at[pl.ds(_mult(g, GD), GD)], wo.at[g, :, pl.ds(0, D)])

        cp_c = cp("c", 0, c_hbm, cb)
        cp_wr = cp("wr", 0, wr_hbm, wrb)
        cp_wmb = cp("wmb", 0, wm_hbm.at[:, pl.ds(2 * D, 4 * D)], wm.at[:, pl.ds(2 * D, 4 * D)])
        cp_wg = [cp("wg", j, wg_hbm.at[:, pl.ds(j * FC, FC)], wg.at[j, :, pl.ds(0, FC)]) for j in range(NMLP)]
        cp_wu = [cp("wu", j, wu_hbm.at[:, pl.ds(j * FC, FC)], wu.at[j, :, pl.ds(0, FC)]) for j in range(NMLP)]
        cp_wd = cp("wd", 0, wd_hbm, wd.at[:, pl.ds(0, D)])

        def cp_out(t):
            r = pl.ds(_mult(t, TQ), TQ)
            return pltpu.make_async_copy(ob.at[r], out_hbm.at[0, r], sem_out.at[t])

        order = [cp_c, cp_x(0)] + [cp_wma(i) for i in range(NWM)]
        for g in range(HKV):
            order += [cp_wqa(g), cp_k(g), cp_v(g), cp_wqb(g), cp_wo(g), cp_x1(g)]
        order += [cp_wr, cp_wmb] + [cp_x(t) for t in range(2, NT)] + cp_wg + cp_wu + [cp_wd]
        for c in order:
            c.start()

        flag[0] = 0

        def tie(x, tok, never):
            if tok is None:
                return x
            return jnp.concatenate([jnp.where(never, tok, x[:, :128]), x[:, 128:]], axis=-1)

        def ln_plain(x):
            m = jnp.sum(x, axis=-1, keepdims=True) * (1.0 / D)
            xc = x - m
            v = jnp.sum(xc * xc, axis=-1, keepdims=True) * (1.0 / D)
            return xc * lax.rsqrt(v + EPS)

        def ln2_mod(x1):
            m = jnp.sum(x1, axis=-1, keepdims=True) * (1.0 / D)
            mb = _rb(m)
            xc = x1 - mb
            dm = m - mb
            v = jnp.sum(xc * xc, axis=-1, keepdims=True) * (1.0 / D) - dm * dm
            sd = _rb(jnp.sqrt(_rb(_rb(jnp.maximum(v, 0.0)) + EPS)))
            r0 = pl.reciprocal(sd, approx=True)
            rinv = r0 * (2.0 - sd * r0)
            return (xc * rinv) * modb[M_CB1][None] + modb[M_SB][None]

        def ln1_piece(xrow, slot, hrow, tok=None, never=None):
            x = tie(xb[pl.ds(xrow, PR), :].astype(f32), tok, never).reshape(PR // 8, 8, D)
            h = (ln_plain(x) * modb[M_CA1][None] + modb[M_SA][None]).reshape(PR, D).astype(bf16)
            h32 = pltpu.bitcast(h, u32)
            hb[slot, pl.ds(hrow, PR // 2), :] = h32
            return h32[:, :128]

        sub_iota = lax.broadcasted_iota(i32, (8, 128), 0)

        def epi_piece(row, best, tok=None, never=None):
            x1 = tie(xb[pl.ds(row, PR), :].astype(f32), tok, never).reshape(PR // 8, 8, D)
            h2 = ln2_mod(x1)
            rr = jnp.sum(h2 * modb[M_WR][None], axis=-1, keepdims=True)
            rb16 = jnp.broadcast_to(rr.reshape(PR, 1), (PR, 128)).astype(bf16)
            rbf = rb16.astype(f32)
            for j in range(PR // 8):
                rj = rbf[8 * j:8 * j + 8]
                upd = rj > best[0]
                best[1] = jnp.where(upd, sub_iota + (row + 8 * j), best[1])
                best[0] = jnp.where(upd, rj, best[0])
            ob[pl.ds(row, PR), :] = (x1 + modb[M_GB][None] * h2).reshape(PR, D).astype(bf16)
            return pltpu.bitcast(rb16, u32)

        def qproj(hh, g, j):
            return (_dot(hh, wq[g, :, j * DH:(j + 1) * DH]) * QSCALE).astype(bf16)

        def qk(q, g):
            s = lax.dot_general(q, kb[g], (((1,), (1,)), ((), ())), preferred_element_type=f32)
            m = jnp.max(s, axis=-1, keepdims=True)
            p = jnp.exp2(s - m)
            l = jnp.sum(p, axis=-1, keepdims=True)
            rl = pl.reciprocal(l, approx=True)
            return p.astype(bf16), rl * (2.0 - l * rl)

        def pv(prl, g):
            p, rl = prl
            return (_dot(p, vb[g]) * rl).astype(bf16)

        def oproj(os_, g, j0, sink, pieces, gap, never):
            outs, done = {}, 0
            for n in range(NK):
                cs = slice(n * 128, (n + 1) * 128)
                o0 = os_[0]
                toks = outs.pop(n, [])
                if toks:
                    o32 = pltpu.bitcast(o0, u32)
                    parts = [jnp.where(never, tok, o32[8 * k:8 * k + 8]) for k, tok in enumerate(toks)]
                    o0 = pltpu.bitcast(jnp.concatenate(parts + [o32[8 * len(toks):]], axis=0), bf16)
                og = jnp.concatenate([o0] + list(os_[1:]), axis=-1)
                a = _dot(og, wo[g, j0 * DH:(j0 + len(os_)) * DH, cs])
                sink(n, cs, a)
                if n < NK - gap:
                    cnt = int(round((n + 1) * len(pieces) / (NK - gap))) - done
                    for k in range(cnt):
                        rr = (k * TQ // cnt) // PR * PR
                        outs.setdefault(n + gap, []).append(pieces[done](a[rr:rr + PR], never))
                        done += 1
            assert done == len(pieces)

        def acc_set(n, cs, a):
            acc_ref[:, cs] = a

        def acc_add(n, cs, a):
            acc_ref[:, cs] += a

        def write_x1(r0, acc):
            a = acc.reshape(TQ // 8, 8, D) * modb[M_GA][None]
            xb[pl.ds(r0, TQ), :] = (xb[pl.ds(r0, TQ), :].astype(f32) + a.reshape(TQ, D)).astype(bf16)

        acc_ref[...] = jnp.zeros((TQ, D), f32)
        cp_c.wait()
        sc = jnp.broadcast_to(_silu(cb[...].astype(f32)).astype(bf16), (16, D))
        for i in range(NWM):
            scb[i] = sc[:, i * KC:(i + 1) * KC]
        cp_x(0).wait()

        def ln0(i, c):
            r = pl.ds(pl.multiple_of(i * 64, 64), 64)
            xn_ref[r, :] = ln_plain(xb[r, :].astype(f32))
            return c

        lax.fori_loop(0, TQ // 64, ln0, 0)

        def moda(i, ma):
            cp_wma(i).wait()
            return ma + _dot(scb[i], wm[pl.ds(_mult(i, KC), KC), 0:2 * D])[0:8]

        ma = _rb(lax.fori_loop(0, NWM, moda, jnp.zeros((8, 2 * D), f32)))
        sa = ma[:, 0:D]
        ca1 = _rb(1.0 + ma[:, D:2 * D])
        modb[M_SA] = sa
        modb[M_CA1] = ca1
        h0 = (xn_ref[...].reshape(TQ // 8, 8, D) * ca1[None] + sa[None]).reshape(TQ, D).astype(bf16)
        hb[0] = pltpu.bitcast(h0, u32)

        def group0(g, c):
            never = flag[0] > 0
            cp_wqa(g).wait()
            cp_k(g).wait()
            cp_v(g).wait()
            q = qproj(pltpu.bitcast(hb[0], bf16), g, 0)
            os_ = []
            for j in range(REP):
                if j == QA - 1:
                    cp_wqb(g).wait()
                if j == REP - 1:
                    cp_wo(g).wait()
                    cp_x1(g).wait()
                prl = qk(q, g)
                if j + 1 < REP:
                    q = qproj(pltpu.bitcast(hb[0], bf16), g, j + 1)
                else:
                    oproj(os_[:REP // 2], g, 0, acc_add, [], 0, never)
                os_.append(pv(prl, g))
            xr = _mult(g, XQ)
            hr = _mult(g, XQ // 2)
            pieces = [functools.partial(ln1_piece, TQ + xr + i * PR, 1, hr + i * PR // 2)
                      for i in range(XQ // PR)]
            oproj(os_[REP // 2:], g, REP // 2, acc_add, pieces, 4, never)
            return c

        lax.fori_loop(0, HKV, group0, 0)

        cp_wr.wait()
        cp_wmb.wait()
        modb[M_WR] = jnp.broadcast_to(wrb[...].astype(f32).reshape(1, D), (8, D))
        modb[M_GA] = _rb(_dot(sc, wm[:, 2 * D:3 * D])[0:8])
        mb = _rb(_dot(sc, wm[:, 3 * D:6 * D])[0:8])
        modb[M_SB] = mb[:, 0:D]
        modb[M_CB1] = _rb(1.0 + mb[:, D:2 * D])
        modb[M_GB] = mb[:, 2 * D:3 * D]
        write_x1(0, acc_ref[...])

        def body(t, carry):
            @pl.when(t + 1 < NT)
            def _():
                cp_x(t + 1).wait()

            never = flag[0] > 0
            slot = t % 2
            r0 = _mult(t, TQ)
            rp = _mult(t - 1, TQ)
            rn = _mult(jnp.minimum(t + 1, NT - 1), TQ)
            best = list(carry)
            pieces = []
            for i in range(NS):
                pieces += [functools.partial(epi_piece, rp + i * PR, best),
                           functools.partial(ln1_piece, rn + i * PR, 1 - slot, i * PR // 2)]
            npg = -(-len(pieces) // (HKV - 1))
            hh = pltpu.bitcast(hb[slot], bf16)
            fin = [None] * NK

            def acc_fin(n, cs, a):
                fin[n] = acc_ref[:, cs] + a

            q = qproj(hh, 0, 0)
            for g in range(HKV):
                os_ = []
                for j in range(REP):
                    prl = qk(q, g)
                    if j + 1 < REP:
                        q = qproj(hh, g, j + 1)
                    elif g + 1 < HKV:
                        q = qproj(hh, g + 1, 0)
                    else:
                        oproj(os_[:REP // 2], g, 0, acc_add, [], 0, never)
                    os_.append(pv(prl, g))
                if g + 1 < HKV:
                    oproj(os_, g, 0, acc_set if g == 0 else acc_add, pieces[g * npg:(g + 1) * npg], 2, never)
                else:
                    oproj(os_[REP // 2:], g, REP // 2, acc_fin, [], 0, never)
            write_x1(r0, jnp.concatenate(fin, axis=-1))
            cp_out(t - 1).start()
            return tuple(best)

        init = (jnp.full((8, 128), -jnp.inf, f32), jnp.zeros((8, 128), i32))
        best = list(lax.fori_loop(1, NT, body, init))

        for c in cp_wg + cp_wu + [cp_wd]:
            c.wait()
        for i in range(NS):
            epi_piece((NT - 1) * TQ + i * PR, best)
        cp_out(NT - 1).start()

        bv, bi = best
        rmax = jnp.max(bv, axis=0, keepdims=True)
        imin = jnp.min(jnp.where(bv == rmax, bi, S), axis=0, keepdims=True)
        idx = jnp.minimum(imin[0, 0], S - 1)
        s0 = pl.multiple_of((idx // PR) * PR, PR)
        x1s = xb[pl.ds(s0, PR), :].astype(f32).reshape(PR // 8, 8, D)
        h2s = ln2_mod(x1s)
        lhs = h2s.reshape(PR, D).astype(bf16)

        def mlp(j, y):
            gt = _rb(_silu(_rb(_dot(lhs, wg[j, :, 0:FC]))))
            up = _rb(_dot(lhs, wu[j, :, 0:FC]))
            return y + _dot((gt * up).astype(bf16), wd[pl.ds(_mult(j, FC), FC), 0:D])

        y = _rb(lax.fori_loop(0, NMLP, mlp, jnp.zeros((PR, D), f32)))
        gate = _rb(1.0 / (1.0 + jnp.exp(-rmax[:, 0:1])))
        y = _rb(y * gate)
        rows = lax.broadcasted_iota(i32, (PR, D), 0) + s0
        upd = jnp.where(rows == idx, y, 0.0).reshape(PR // 8, 8, D)
        fix[...] = (x1s + modb[M_GB][None] * (h2s + upd)).reshape(PR, D).astype(bf16)
        for t in range(NT):
            cp_out(t).wait()
        cp_fix = pltpu.make_async_copy(fix, out_hbm.at[0, pl.ds(s0, PR)], sem_out.at[NT])
        cp_fix.start()
        cp_fix.wait()

    scratch = [
        pltpu.VMEM((S, D), bf16),
        pltpu.VMEM((S, D), bf16),
        pltpu.VMEM((2, TQ // 2, D), u32),
        pltpu.VMEM((HKV, W, DH), bf16),
        pltpu.VMEM((HKV, W, DH), bf16),
        pltpu.VMEM((HKV, D, GD + PAD), bf16),
        pltpu.VMEM((HKV, GD, D + PAD), bf16),
        pltpu.VMEM((NMLP, D, FC + PAD), bf16),
        pltpu.VMEM((NMLP, D, FC + PAD), bf16),
        pltpu.VMEM((F, D + PAD), bf16),
        pltpu.VMEM((D, 6 * D + PAD), bf16),
        pltpu.VMEM((1, D), bf16),
        pltpu.VMEM((D,), bf16),
        pltpu.VMEM((NWM, 16, KC), bf16),
        pltpu.VMEM((7, 8, D), f32),
        pltpu.VMEM((TQ, D), f32),
        pltpu.VMEM((TQ, D), f32),
        pltpu.VMEM((PR, D), bf16),
        pltpu.SMEM((1,), i32),
        pltpu.SemaphoreType.DMA((n_in_sems,)),
        pltpu.SemaphoreType.DMA((NT + 1,)),
    ]
    return kernel, scratch


@jax.jit
def pallas_adaLN_cond__sliding_block_cached__moe_arch_mod__prompt_kernel(
    A_x: jax.Array,
    A_k_cache: jax.Array,
    A_v_cache: jax.Array,
    A_wq: jax.Array,
    A_wo: jax.Array,
    B_x: jax.Array,
    B_w_r: jax.Array,
    B_w_gate: jax.Array,
    B_w_up: jax.Array,
    B_w_down: jax.Array,
    c: jax.Array,
    w_mod: jax.Array,
):
    B, S, D = A_x.shape
    _, HKV, SK, dh = A_k_cache.shape
    F = B_w_gate.shape[1]
    W = min(4096, max(256, SK // 4))
    assert B == 1 and dh == DH and A_wq.shape == (D, HQ * DH) and S % TQ == 0 and S >= 3 * TQ
    kernel, scratch = _make_kernel(S, D, HKV, SK, W, F)
    any_spec = pl.BlockSpec(memory_space=pl.ANY)
    return pl.pallas_call(
        kernel,
        out_shape=jax.ShapeDtypeStruct((B, S, D), A_x.dtype),
        in_specs=[any_spec] * 11,
        out_specs=any_spec,
        scratch_shapes=scratch,
        compiler_params=pltpu.CompilerParams(vmem_limit_bytes=110 * 1024 * 1024,
                                             disable_semaphore_checks=True),
    )(A_x, A_k_cache, A_v_cache, A_wq, A_wo, B_w_r, B_w_gate, B_w_up, B_w_down, c, w_mod)
```

```python
import functools

import jax
import jax.numpy as jnp
from jax import lax
import jax.experimental.pallas as pl
import jax.experimental.pallas.tpu as pltpu

f32 = jnp.float32
bf16 = jnp.bfloat16
u32 = jnp.uint32
i32 = jnp.int32

HQ = 32
DH = 128
TQ = 256
PR = 16
EPS = 1e-05
LOG2E = 1.4426950408889634
NWM = 4
QA = 3
PAD = 128
NMLP = 2
M_SA, M_CA1, M_GA, M_SB, M_CB1, M_GB, M_WR = range(7)


def _rb(x):
    return x.astype(bf16).astype(f32)


def _silu(x):
    return x * (1.0 / (1.0 + jnp.exp(-x)))


def _dot(a, b):
    return jnp.dot(a, b, preferred_element_type=f32)


def _mult(i, n):
    return i * n if isinstance(i, int) else pl.multiple_of(i * n, n)


def _make_kernel(S, D, HKV, SK, W, F):
    NT = S // TQ
    NK = D // 128
    NS = TQ // PR
    REP = HQ // HKV
    GD = REP * DH
    QSCALE = DH ** (-0.5) * LOG2E
    KC = D // NWM
    XQ = TQ // HKV
    FC = F // NMLP

    sem_base, n_in_sems = {}, 0
    for name, n in (("c", 1), ("wr", 1), ("x", NT), ("x1", HKV), ("wma", 2 * NWM), ("wqa", HKV), ("wqb", HKV),
                    ("k", HKV), ("v", HKV), ("wo", HKV), ("wmb", 4), ("wg", NMLP), ("wu", NMLP), ("wd", 1)):
        sem_base[name] = n_in_sems
        n_in_sems += n

    def kernel(x_hbm, k_hbm, v_hbm, wq_hbm, wo_hbm, wr_hbm, wg_hbm, wu_hbm, wd_hbm, c_hbm, wm_hbm,
               out_hbm,
               xb, x0b, ob, hb, kb, vb, wq, wo, wg, wu, wd, wm, cb, wrb, scb, colb, modp, modb, acc_ref, xn_ref, fix, flag,
               sem_in, sem_out):
        def cp(name, i, src, dst):
            return pltpu.make_async_copy(src, dst, sem_in.at[sem_base[name] + i])

        def cp_x(t):
            r = pl.ds(_mult(t, TQ), TQ)
            return cp("x", t, x_hbm.at[0, r], x0b if isinstance(t, int) and t == 0 else xb.at[r])

        def cp_x1(g):
            r = pl.ds(TQ + _mult(g, XQ), XQ)
            return cp("x1", g, x_hbm.at[0, r], xb.at[r])

        def cp_wma(i, j):
            r = pl.ds(_mult(i, KC), KC)
            return cp("wma", 2 * i + j, wm_hbm.at[r, pl.ds(j * D, D)], wm.at[j, r, pl.ds(0, D)])

        def cp_wmb(j):
            return cp("wmb", j, wm_hbm.at[:, pl.ds(_mult(j + 2, D), D)], wm.at[j + 2, :, pl.ds(0, D)])

        def cp_wqa(g):
            return cp("wqa", g, wq_hbm.at[:, pl.ds(_mult(g, GD), QA * DH)], wq.at[g, :, pl.ds(0, QA * DH)])

        def cp_wqb(g):
            n = GD - QA * DH
            return cp("wqb", g, wq_hbm.at[:, pl.ds(_mult(g, GD) + QA * DH, n)], wq.at[g, :, pl.ds(QA * DH, n)])

        def cp_k(g):
            return cp("k", g, k_hbm.at[0, g, pl.ds(SK - W, W)], kb.at[g])

        def cp_v(g):
            return cp("v", g, v_hbm.at[0, g, pl.ds(SK - W, W)], vb.at[g])

        def cp_wo(g):
            return cp("wo", g, wo_hbm.at[pl.ds(_mult(g, GD), GD)], wo.at[g, :, pl.ds(0, D)])

        cp_c = cp("c", 0, c_hbm, cb)
        cp_wr = cp("wr", 0, wr_hbm, wrb)
        cp_wg = [cp("wg", j, wg_hbm.at[:, pl.ds(j * FC, FC)], wg.at[j, :, pl.ds(0, FC)]) for j in range(NMLP)]
        cp_wu = [cp("wu", j, wu_hbm.at[:, pl.ds(j * FC, FC)], wu.at[j, :, pl.ds(0, FC)]) for j in range(NMLP)]
        cp_wd = cp("wd", 0, wd_hbm, wd.at[:, pl.ds(0, D)])

        def cp_out(t):
            r = pl.ds(_mult(t, TQ), TQ)
            return pltpu.make_async_copy(ob.at[r], out_hbm.at[0, r], sem_out.at[t])

        order = [cp_c, cp_x(0)] + [cp_wma(i, j) for i in range(NWM) for j in range(2)]
        for g in range(HKV):
            order += [cp_wqa(g), cp_k(g), cp_v(g), cp_wqb(g), cp_wo(g), cp_x1(g)]
            if g >= 1:
                order += [cp_wmb(g - 1)]
        order += [cp_wr, cp_wmb(HKV - 1)] + [cp_x(t) for t in range(2, NT)] + cp_wg + cp_wu + [cp_wd]
        for c in order:
            c.start()

        flag[0] = 0

        def tie(x, tok, never):
            if tok is None:
                return x
            return jnp.concatenate([jnp.where(never, tok, x[:, :128]), x[:, 128:]], axis=-1)

        def ln_plain(x):
            m = jnp.sum(x, axis=-1, keepdims=True) * (1.0 / D)
            xc = x - m
            v = jnp.sum(xc * xc, axis=-1, keepdims=True) * (1.0 / D)
            return xc * lax.rsqrt(v + EPS)

        def ln2_mod(x1):
            m = jnp.sum(x1, axis=-1, keepdims=True) * (1.0 / D)
            mb = _rb(m)
            xc = x1 - mb
            dm = m - mb
            v = jnp.sum(xc * xc, axis=-1, keepdims=True) * (1.0 / D) - dm * dm
            sd = _rb(jnp.sqrt(_rb(_rb(jnp.maximum(v, 0.0)) + EPS)))
            r0 = pl.reciprocal(sd, approx=True)
            rinv = r0 * (2.0 - sd * r0)
            return (xc * rinv) * modb[M_CB1][None] + modb[M_SB][None]

        def ln1_piece(xrow, slot, hrow, tok=None, never=None):
            x = tie(xb[pl.ds(xrow, PR), :].astype(f32), tok, never).reshape(PR // 8, 8, D)
            h = (ln_plain(x) * modb[M_CA1][None] + modb[M_SA][None]).reshape(PR, D).astype(bf16)
            h32 = pltpu.bitcast(h, u32)
            hb[slot, pl.ds(hrow, PR // 2), :] = h32
            return h32[:, :128]

        sub_iota = lax.broadcasted_iota(i32, (8, 128), 0)

        def epi_piece(row, best, tok=None, never=None):
            x1 = tie(xb[pl.ds(row, PR), :].astype(f32), tok, never).reshape(PR // 8, 8, D)
            h2 = ln2_mod(x1)
            rr = jnp.sum(h2 * modb[M_WR][None], axis=-1, keepdims=True)
            rb16 = jnp.broadcast_to(rr.reshape(PR, 1), (PR, 128)).astype(bf16)
            rbf = rb16.astype(f32)
            for j in range(PR // 8):
                rj = rbf[8 * j:8 * j + 8]
                upd = rj > best[0]
                best[1] = jnp.where(upd, sub_iota + (row + 8 * j), best[1])
                best[0] = jnp.where(upd, rj, best[0])
            ob[pl.ds(row, PR), :] = (x1 + modb[M_GB][None] * h2).reshape(PR, D).astype(bf16)
            return pltpu.bitcast(rb16, u32)

        def modv_piece(ch, n, tok=None, never=None):
            y = jnp.where(never, tok[0:8], 0.0)
            for kg in range(D // 8):
                y = y + wm[ch, kg * 8:(kg + 1) * 8, n * 128:(n + 1) * 128].astype(f32) * colb[kg * 8:(kg + 1) * 8, :]
            modp[ch, :, n * 128:(n + 1) * 128] = y
            return pltpu.bitcast(y, u32)

        def qproj(hh, g, j):
            return (_dot(hh, wq[g, :, j * DH:(j + 1) * DH]) * QSCALE).astype(bf16)

        def qk(q, g):
            s = lax.dot_general(q, kb[g], (((1,), (1,)), ((), ())), preferred_element_type=f32)
            m = jnp.max(s, axis=-1, keepdims=True)
            p = jnp.exp2(s - m)
            l = jnp.sum(p, axis=-1, keepdims=True)
            rl = pl.reciprocal(l, approx=True)
            return p.astype(bf16), rl * (2.0 - l * rl)

        def pv(prl, g):
            p, rl = prl
            return (_dot(p, vb[g]) * rl).astype(bf16)

        def oproj(os_, g, j0, sink, pieces, gap, never):
            outs, done = {}, 0
            for n in range(NK):
                cs = slice(n * 128, (n + 1) * 128)
                o0 = os_[0]
                toks = outs.pop(n, [])
                if toks:
                    o32 = pltpu.bitcast(o0, u32)
                    parts = [jnp.where(never, tok, o32[8 * k:8 * k + 8]) for k, tok in enumerate(toks)]
                    o0 = pltpu.bitcast(jnp.concatenate(parts + [o32[8 * len(toks):]], axis=0), bf16)
                og = jnp.concatenate([o0] + list(os_[1:]), axis=-1)
                a = _dot(og, wo[g, j0 * DH:(j0 + len(os_)) * DH, cs])
                sink(n, cs, a)
                if n < NK - gap:
                    cnt = int(round((n + 1) * len(pieces) / (NK - gap))) - done
                    for k in range(cnt):
                        rr = (k * TQ // cnt) // PR * PR
                        outs.setdefault(n + gap, []).append(pieces[done](a[rr:rr + PR], never))
                        done += 1
            assert done == len(pieces)

        def acc_set(n, cs, a):
            acc_ref[:, cs] = a

        def acc_add(n, cs, a):
            acc_ref[:, cs] += a

        def write_x1(r0, x, acc, ga):
            a = acc.reshape(TQ // 8, 8, D) * ga[None]
            xb[pl.ds(r0, TQ), :] = (x.astype(f32) + a.reshape(TQ, D)).astype(bf16)

        def mod_vec(ch):
            return jnp.broadcast_to(_rb(jnp.sum(modp[ch], axis=0, keepdims=True)), (8, D))

        acc_ref[...] = jnp.zeros((TQ, D), f32)
        modp[2] = jnp.zeros((8, D), f32)
        cp_c.wait()
        sc1 = _silu(cb[...].astype(f32)).astype(bf16)
        sc = jnp.broadcast_to(sc1, (16, D))
        colb[...] = jnp.broadcast_to(sc1.astype(f32), (128, D)).T
        for i in range(NWM):
            scb[i] = sc[:, i * KC:(i + 1) * KC]
        cp_x(0).wait()

        def ln0(i, c):
            r = pl.ds(pl.multiple_of(i * 64, 64), 64)
            xn_ref[r, :] = ln_plain(x0b[r, :].astype(f32))
            return c

        lax.fori_loop(0, TQ // 64, ln0, 0)

        def moda(i, ma):
            cp_wma(i, 0).wait()
            cp_wma(i, 1).wait()
            r = pl.ds(_mult(i, KC), KC)
            w = jnp.concatenate([wm[0, r, 0:D], wm[1, r, 0:D]], axis=-1)
            return ma + _dot(scb[i], w)[0:8]

        ma = _rb(lax.fori_loop(0, NWM, moda, jnp.zeros((8, 2 * D), f32)))
        sa = ma[:, 0:D]
        ca1 = _rb(1.0 + ma[:, D:2 * D])
        modb[M_SA] = sa
        modb[M_CA1] = ca1
        h0 = (xn_ref[...].reshape(TQ // 8, 8, D) * ca1[None] + sa[None]).reshape(TQ, D).astype(bf16)
        hb[0] = pltpu.bitcast(h0, u32)

        def group0(g, c):
            never = flag[0] > 0
            cp_wqa(g).wait()
            cp_k(g).wait()
            cp_v(g).wait()
            ga = mod_vec(2)
            q = qproj(pltpu.bitcast(hb[0], bf16), g, 0)
            os_ = []
            mv = [functools.partial(modv_piece, g + 1, n) for n in range(NK)]
            for j in range(REP):
                if j == QA - 1:
                    cp_wqb(g).wait()
                if j == REP - 1:
                    cp_wo(g).wait()
                    cp_x1(g).wait()

                    @pl.when(g >= 1)
                    def _():
                        cp_wmb(g - 1).wait()

                prl = qk(q, g)
                if j + 1 < REP:
                    q = qproj(pltpu.bitcast(hb[0], bf16), g, j + 1)
                else:
                    oproj(os_[:REP // 2], g, 0, acc_add, mv[:NK // 2], 3, never)
                os_.append(pv(prl, g))
            xr = _mult(g, XQ)
            hr = _mult(g, XQ // 2)
            pieces = [functools.partial(ln1_piece, TQ + xr + i * PR, 1, hr + i * PR // 2)
                      for i in range(XQ // PR)]
            pieces = [p for pair in zip(pieces, mv[NK // 2:]) for p in pair]
            fin = [None] * NK

            def acc_fin(n, cs, a):
                fin[n] = acc_ref[:, cs] + a
                acc_ref[:, cs] = fin[n]

            oproj(os_[REP // 2:], g, REP // 2, acc_fin, pieces, 4, never)
            write_x1(0, x0b[...], jnp.concatenate(fin, axis=-1), ga)
            return c

        lax.fori_loop(0, HKV, group0, 0)

        cp_wr.wait()
        cp_wmb(HKV - 1).wait()

        modb[M_WR] = jnp.broadcast_to(wrb[...].astype(f32).reshape(1, D), (8, D))
        modb[M_GA] = mod_vec(2)
        modb[M_SB] = mod_vec(3)
        modb[M_CB1] = _rb(1.0 + mod_vec(4))
        modb[M_GB] = _rb(_dot(sc, wm[5, :, 0:D])[0:8])

        def body(t, carry):
            @pl.when(t + 1 < NT)
            def _():
                cp_x(t + 1).wait()

            never = flag[0] > 0
            slot = t % 2
            r0 = _mult(t, TQ)
            rp = _mult(t - 1, TQ)
            rn = _mult(jnp.minimum(t + 1, NT - 1), TQ)
            best = list(carry)
            pieces = []
            for i in range(NS):
                pieces += [functools.partial(epi_piece, rp + i * PR, best),
                           functools.partial(ln1_piece, rn + i * PR, 1 - slot, i * PR // 2)]
            npg = -(-len(pieces) // (HKV - 1))
            hh = pltpu.bitcast(hb[slot], bf16)
            fin = [None] * NK

            def acc_fin(n, cs, a):
                fin[n] = acc_ref[:, cs] + a

            q = qproj(hh, 0, 0)
            for g in range(HKV):
                os_ = []
                for j in range(REP):
                    prl = qk(q, g)
                    if j + 1 < REP:
                        q = qproj(hh, g, j + 1)
                    elif g + 1 < HKV:
                        q = qproj(hh, g + 1, 0)
                    else:
                        oproj(os_[:REP // 2], g, 0, acc_add, [], 0, never)
                    os_.append(pv(prl, g))
                if g + 1 < HKV:
                    oproj(os_, g, 0, acc_set if g == 0 else acc_add, pieces[g * npg:(g + 1) * npg], 2, never)
                else:
                    oproj(os_[REP // 2:], g, REP // 2, acc_fin, [], 0, never)
            write_x1(r0, xb[pl.ds(r0, TQ), :], jnp.concatenate(fin, axis=-1), modb[M_GA])
            cp_out(t - 1).start()
            return tuple(best)

        init = (jnp.full((8, 128), -jnp.inf, f32), jnp.zeros((8, 128), i32))
        best = list(lax.fori_loop(1, NT, body, init))

        for c in cp_wg + cp_wu + [cp_wd]:
            c.wait()
        for i in range(NS):
            epi_piece((NT - 1) * TQ + i * PR, best)
        cp_out(NT - 1).start()

        bv, bi = best
        rmax = jnp.max(bv, axis=0, keepdims=True)
        imin = jnp.min(jnp.where(bv == rmax, bi, S), axis=0, keepdims=True)
        idx = jnp.minimum(imin[0, 0], S - 1)
        s0 = pl.multiple_of((idx // PR) * PR, PR)
        x1s = xb[pl.ds(s0, PR), :].astype(f32).reshape(PR // 8, 8, D)
        h2s = ln2_mod(x1s)
        lhs = h2s.reshape(PR, D).astype(bf16)

        def mlp(j, y):
            gt = _rb(_silu(_rb(_dot(lhs, wg[j, :, 0:FC]))))
            up = _rb(_dot(lhs, wu[j, :, 0:FC]))
            return y + _dot((gt * up).astype(bf16), wd[pl.ds(_mult(j, FC), FC), 0:D])

        y = _rb(lax.fori_loop(0, NMLP, mlp, jnp.zeros((PR, D), f32)))
        gate = _rb(1.0 / (1.0 + jnp.exp(-rmax[:, 0:1])))
        y = _rb(y * gate)
        rows = lax.broadcasted_iota(i32, (PR, D), 0) + s0
        upd = jnp.where(rows == idx, y, 0.0).reshape(PR // 8, 8, D)
        fix[...] = (x1s + modb[M_GB][None] * (h2s + upd)).reshape(PR, D).astype(bf16)
        for t in range(NT):
            cp_out(t).wait()
        cp_fix = pltpu.make_async_copy(fix, out_hbm.at[0, pl.ds(s0, PR)], sem_out.at[NT])
        cp_fix.start()
        cp_fix.wait()

    scratch = [
        pltpu.VMEM((S, D), bf16),
        pltpu.VMEM((TQ, D), bf16),
        pltpu.VMEM((S, D), bf16),
        pltpu.VMEM((2, TQ // 2, D), u32),
        pltpu.VMEM((HKV, W, DH), bf16),
        pltpu.VMEM((HKV, W, DH), bf16),
        pltpu.VMEM((HKV, D, GD + PAD), bf16),
        pltpu.VMEM((HKV, GD, D + PAD), bf16),
        pltpu.VMEM((NMLP, D, FC + PAD), bf16),
        pltpu.VMEM((NMLP, D, FC + PAD), bf16),
        pltpu.VMEM((F, D + PAD), bf16),
        pltpu.VMEM((6, D, D + PAD), bf16),
        pltpu.VMEM((1, D), bf16),
        pltpu.VMEM((D,), bf16),
        pltpu.VMEM((NWM, 16, KC), bf16),
        pltpu.VMEM((D, 128), f32),
        pltpu.VMEM((5, 8, D), f32),
        pltpu.VMEM((7, 8, D), f32),
        pltpu.VMEM((TQ, D), f32),
        pltpu.VMEM((TQ, D), f32),
        pltpu.VMEM((PR, D), bf16),
        pltpu.SMEM((1,), i32),
        pltpu.SemaphoreType.DMA((n_in_sems,)),
        pltpu.SemaphoreType.DMA((NT + 1,)),
    ]
    return kernel, scratch


@jax.jit
def pallas_adaLN_cond__sliding_block_cached__moe_arch_mod__prompt_kernel(
    A_x: jax.Array,
    A_k_cache: jax.Array,
    A_v_cache: jax.Array,
    A_wq: jax.Array,
    A_wo: jax.Array,
    B_x: jax.Array,
    B_w_r: jax.Array,
    B_w_gate: jax.Array,
    B_w_up: jax.Array,
    B_w_down: jax.Array,
    c: jax.Array,
    w_mod: jax.Array,
):
    B, S, D = A_x.shape
    _, HKV, SK, dh = A_k_cache.shape
    F = B_w_gate.shape[1]
    W = min(4096, max(256, SK // 4))
    assert B == 1 and dh == DH and A_wq.shape == (D, HQ * DH) and S % TQ == 0 and S >= 3 * TQ
    kernel, scratch = _make_kernel(S, D, HKV, SK, W, F)
    any_spec = pl.BlockSpec(memory_space=pl.ANY)
    return pl.pallas_call(
        kernel,
        out_shape=jax.ShapeDtypeStruct((B, S, D), A_x.dtype),
        in_specs=[any_spec] * 11,
        out_specs=any_spec,
        scratch_shapes=scratch,
        compiler_params=pltpu.CompilerParams(vmem_limit_bytes=110 * 1024 * 1024,
                                             disable_semaphore_checks=True),
    )(A_x, A_k_cache, A_v_cache, A_wq, A_wo, B_w_r, B_w_gate, B_w_up, B_w_down, c, w_mod)
```

```python
import functools

import jax
import jax.numpy as jnp
from jax import lax
import jax.experimental.pallas as pl
import jax.experimental.pallas.tpu as pltpu

f32 = jnp.float32
bf16 = jnp.bfloat16
u32 = jnp.uint32
i32 = jnp.int32

HQ = 32
DH = 128
TQ = 256
PR = 16
EPS = 1e-05
LOG2E = 1.4426950408889634
NWM = 4
QA = 3
PAD = 128
OGAP = 3
OUTP = 1
NMLP = 2
FCH = 256
M_SA, M_CA1, M_GA, M_SB, M_CB1, M_GB, M_AW, M_C0 = range(8)


def _rb(x):
    return x.astype(bf16).astype(f32)


def _silu(x):
    return x * (1.0 / (1.0 + jnp.exp(-x)))


def _dot(a, b):
    return jnp.dot(a, b, preferred_element_type=f32)


def _mult(i, n):
    return i * n if isinstance(i, int) else pl.multiple_of(i * n, n)


def _make_kernel(S, D, HKV, SK, W, F):
    NT = S // TQ
    NK = D // 128
    NS = TQ // PR
    REP = HQ // HKV
    GD = REP * DH
    QSCALE = DH ** (-0.5) * LOG2E
    KC = D // NWM
    XQ = TQ // HKV

    FC = F // NMLP
    OH = TQ // NMLP

    sem_base, n_in_sems = {}, 0
    for name, n in (("c", 1), ("wr", 1), ("x", NT), ("x1", HKV), ("wma", 2 * NWM), ("wqa", HKV), ("wqb", HKV),
                    ("k", HKV), ("v", HKV), ("wo", HKV), ("wmb", 4), ("wg", NMLP), ("wu", NMLP), ("wd", 1)):
        sem_base[name] = n_in_sems
        n_in_sems += n

    def kernel(x_hbm, k_hbm, v_hbm, wq_hbm, wo_hbm, wr_hbm, wg_hbm, wu_hbm, wd_hbm, c_hbm, wm_hbm,
               out_hbm,
               xb, x0b, ob, hb, kb, vb, wq, wo, wg, wu, wd, wm, cb, wrb, scb, colb, modp, modb, st_ref, acc_ref, xn_ref, fix, flag,
               sem_in, sem_out):
        def cp(name, i, src, dst):
            return pltpu.make_async_copy(src, dst, sem_in.at[sem_base[name] + i])

        def cp_x(t):
            r = pl.ds(_mult(t, TQ), TQ)
            return cp("x", t, x_hbm.at[0, r], x0b if isinstance(t, int) and t == 0 else xb.at[r])

        def cp_x1(g):
            r = pl.ds(TQ + _mult(g, XQ), XQ)
            return cp("x1", g, x_hbm.at[0, r], xb.at[r])

        def cp_wma(i, j):
            r = pl.ds(_mult(i, KC), KC)
            return cp("wma", 2 * i + j, wm_hbm.at[r, pl.ds(j * D, D)], wm.at[j, r, pl.ds(0, D)])

        def cp_wmb(j):
            return cp("wmb", j, wm_hbm.at[:, pl.ds(_mult(j + 2, D), D)], wm.at[j + 2, :, pl.ds(0, D)])

        def cp_wqa(g):
            return cp("wqa", g, wq_hbm.at[:, pl.ds(_mult(g, GD), QA * DH)], wq.at[g, :, pl.ds(0, QA * DH)])

        def cp_wqb(g):
            n = GD - QA * DH
            return cp("wqb", g, wq_hbm.at[:, pl.ds(_mult(g, GD) + QA * DH, n)], wq.at[g, :, pl.ds(QA * DH, n)])

        def cp_k(g):
            return cp("k", g, k_hbm.at[0, g, pl.ds(SK - W, W)], kb.at[g])

        def cp_v(g):
            return cp("v", g, v_hbm.at[0, g, pl.ds(SK - W, W)], vb.at[g])

        def cp_wo(g):
            return cp("wo", g, wo_hbm.at[pl.ds(_mult(g, GD), GD)], wo.at[g, :, pl.ds(0, D)])

        cp_c = cp("c", 0, c_hbm, cb)
        cp_wr = cp("wr", 0, wr_hbm, wrb)
        cp_wg = [cp("wg", j, wg_hbm.at[:, pl.ds(j * FC, FC)], wg.at[j, :, pl.ds(0, FC)]) for j in range(NMLP)]
        cp_wu = [cp("wu", j, wu_hbm.at[:, pl.ds(j * FC, FC)], wu.at[j, :, pl.ds(0, FC)]) for j in range(NMLP)]
        cp_wd = cp("wd", 0, wd_hbm, wd.at[:, pl.ds(0, D)])

        def cp_out(t):
            r = pl.ds(_mult(t, TQ), TQ)
            return pltpu.make_async_copy(ob.at[r], out_hbm.at[0, r], sem_out.at[t])

        def cp_outl(j):
            r = pl.ds((NT - 1) * TQ + _mult(j, OH), OH)
            return pltpu.make_async_copy(ob.at[r], out_hbm.at[0, r], sem_out.at[NT - 1 + j])

        order = [cp_c, cp_x(0)] + [cp_wma(i, j) for i in range(NWM) for j in range(2)]
        for g in range(HKV):
            order += [cp_wqa(g), cp_k(g), cp_v(g), cp_wqb(g), cp_wo(g), cp_x1(g)]
            if g >= 1:
                order += [cp_wmb(g - 1)]
        order += [cp_wr, cp_wmb(HKV - 1)] + [cp_x(t) for t in range(2, NT)] + cp_wg + cp_wu + [cp_wd]
        for c in order:
            c.start()

        flag[0] = 0

        def tie(x, tok, never):
            if tok is None:
                return x
            return jnp.concatenate([jnp.where(never, tok, x[:, :128]), x[:, 128:]], axis=-1)

        def ln_plain(x):
            m = jnp.sum(x, axis=-1, keepdims=True) * (1.0 / D)
            xc = x - m
            v = jnp.sum(xc * xc, axis=-1, keepdims=True) * (1.0 / D)
            return xc * lax.rsqrt(v + EPS)

        def lane_bc(v):
            return jnp.broadcast_to(v.reshape(-1, 1), (v.shape[0] * 8, 128))

        def h2_of(xc, rinv):
            return (xc * rinv) * modb[M_CB1][None] + modb[M_SB][None]

        def load_stats(row):
            st = st_ref[pl.ds(row, PR), :]
            mb = jnp.concatenate([st[:, 0:128]] * NK, axis=-1).reshape(PR // 8, 8, D)
            rinv = jnp.concatenate([st[:, 128:256]] * NK, axis=-1).reshape(PR // 8, 8, D)
            return mb, rinv

        def ln1_piece(xrow, slot, hrow, tok=None, never=None):
            x = tie(xb[pl.ds(xrow, PR), :].astype(f32), tok, never).reshape(PR // 8, 8, D)
            h = (ln_plain(x) * modb[M_CA1][None] + modb[M_SA][None]).reshape(PR, D).astype(bf16)
            h32 = pltpu.bitcast(h, u32)
            hb[slot, pl.ds(hrow, PR // 2), :] = h32
            return h32[:, :128]

        sub_iota = lax.broadcasted_iota(i32, (8, 128), 0)

        def route_piece(row, best, x1):
            m = jnp.sum(x1, axis=-1, keepdims=True) * (1.0 / D)
            mb = _rb(m)
            xc = x1 - mb
            dm = m - mb
            v = jnp.sum(xc * xc, axis=-1, keepdims=True) * (1.0 / D) - dm * dm
            rs = jnp.sum(xc * modb[M_AW][None], axis=-1, keepdims=True)
            sd = _rb(jnp.sqrt(_rb(_rb(jnp.maximum(v, 0.0)) + EPS)))
            r0 = pl.reciprocal(sd, approx=True)
            rinv = r0 * (2.0 - sd * r0)
            st_ref[pl.ds(row, PR), :] = jnp.concatenate([lane_bc(mb), lane_bc(rinv)], axis=-1)
            rr = lane_bc(rs * rinv).reshape(PR // 8, 8, 128) + modb[M_C0, :, 0:128][None]
            rb16 = rr.reshape(PR, 128).astype(bf16)
            rbf = rb16.astype(f32)
            for j in range(PR // 8):
                rj = rbf[8 * j:8 * j + 8]
                upd = rj > best[0]
                best[1] = jnp.where(upd, sub_iota + (row + 8 * j), best[1])
                best[0] = jnp.where(upd, rj, best[0])
            return xc, rinv, rb16

        def load_x1(row, tok=None, never=None):
            return tie(xb[pl.ds(row, PR), :].astype(f32), tok, never).reshape(PR // 8, 8, D)

        def epi_piece(row, best, tok=None, never=None):
            x1 = load_x1(row, tok, never)
            xc, rinv, rb16 = route_piece(row, best, x1)
            ob[pl.ds(row, PR), :] = (x1 + modb[M_GB][None] * h2_of(xc, rinv)).reshape(PR, D).astype(bf16)
            return pltpu.bitcast(rb16, u32)

        def out_piece(row, tok, never):
            x1 = load_x1(row)
            mb, rinv = load_stats(row)
            mb = jnp.where(never, jnp.concatenate([tok] * NK, axis=-1).reshape(PR // 8, 8, D), mb)
            o = (x1 + modb[M_GB][None] * h2_of(x1 - mb, rinv)).reshape(PR, D).astype(bf16)
            ob[pl.ds(row, PR), :] = o
            return pltpu.bitcast(o[:, 0:128], u32)

        def modv_piece(ch, n, tok=None, never=None):
            y = jnp.where(never, tok[0:8], 0.0)
            for kg in range(D // 8):
                y = y + wm[ch, kg * 8:(kg + 1) * 8, n * 128:(n + 1) * 128].astype(f32) * colb[kg * 8:(kg + 1) * 8, :]
            modp[ch, :, n * 128:(n + 1) * 128] = y
            return pltpu.bitcast(y, u32)

        def qproj(hh, g, j):
            return (_dot(hh, wq[g, :, j * DH:(j + 1) * DH]) * QSCALE).astype(bf16)

        def qk(q, g):
            s = lax.dot_general(q, kb[g], (((1,), (1,)), ((), ())), preferred_element_type=f32)
            m = jnp.max(s, axis=-1, keepdims=True)
            p = jnp.exp2(s - m)
            l = jnp.sum(p, axis=-1, keepdims=True)
            rl = pl.reciprocal(l, approx=True)
            return p.astype(bf16), rl * (2.0 - l * rl)

        def pv(prl, g):
            p, rl = prl
            return (_dot(p, vb[g]) * rl).astype(bf16)

        def oproj(os_, g, j0, sink, pieces, gap, never):
            outs, done = {}, 0
            for n in range(NK):
                cs = slice(n * 128, (n + 1) * 128)
                o0 = os_[0]
                toks = outs.pop(n, [])
                if toks:
                    o32 = pltpu.bitcast(o0, u32)
                    parts = [jnp.where(never, tok, o32[8 * k:8 * k + 8]) for k, tok in enumerate(toks)]
                    o0 = pltpu.bitcast(jnp.concatenate(parts + [o32[8 * len(toks):]], axis=0), bf16)
                og = jnp.concatenate([o0] + list(os_[1:]), axis=-1)
                a = _dot(og, wo[g, j0 * DH:(j0 + len(os_)) * DH, cs])
                sink(n, cs, a)
                if n < NK - gap:
                    cnt = int(round((n + 1) * len(pieces) / (NK - gap))) - done
                    for k in range(cnt):
                        rr = (k * TQ // cnt) // PR * PR
                        outs.setdefault(n + gap, []).append(pieces[done](a[rr:rr + PR], never))
                        done += 1
            assert done == len(pieces)

        def acc_set(n, cs, a):
            acc_ref[:, cs] = a

        def acc_add(n, cs, a):
            acc_ref[:, cs] += a

        def write_x1(r0, x, acc, ga):
            a = acc.reshape(TQ // 8, 8, D) * ga[None]
            xb[pl.ds(r0, TQ), :] = (x.astype(f32) + a.reshape(TQ, D)).astype(bf16)

        def mod_vec(ch):
            return jnp.broadcast_to(_rb(jnp.sum(modp[ch], axis=0, keepdims=True)), (8, D))

        acc_ref[...] = jnp.zeros((TQ, D), f32)
        modp[2] = jnp.zeros((8, D), f32)
        cp_c.wait()
        sc1 = _silu(cb[...].astype(f32)).astype(bf16)
        sc = jnp.broadcast_to(sc1, (16, D))
        colb[...] = jnp.broadcast_to(sc1.astype(f32), (128, D)).T
        for i in range(NWM):
            scb[i] = sc[:, i * KC:(i + 1) * KC]
        cp_x(0).wait()

        def ln0(i, c):
            r = pl.ds(pl.multiple_of(i * 64, 64), 64)
            xn_ref[r, :] = ln_plain(x0b[r, :].astype(f32))
            return c

        lax.fori_loop(0, TQ // 64, ln0, 0)

        def moda(i, ma):
            cp_wma(i, 0).wait()
            cp_wma(i, 1).wait()
            r = pl.ds(_mult(i, KC), KC)
            w = jnp.concatenate([wm[0, r, 0:D], wm[1, r, 0:D]], axis=-1)
            return ma + _dot(scb[i], w)[0:8]

        ma = _rb(lax.fori_loop(0, NWM, moda, jnp.zeros((8, 2 * D), f32)))
        sa = ma[:, 0:D]
        ca1 = _rb(1.0 + ma[:, D:2 * D])
        modb[M_SA] = sa
        modb[M_CA1] = ca1
        h0 = (xn_ref[...].reshape(TQ // 8, 8, D) * ca1[None] + sa[None]).reshape(TQ, D).astype(bf16)
        hb[0] = pltpu.bitcast(h0, u32)

        def group0(g, c):
            never = flag[0] > 0
            cp_wqa(g).wait()
            cp_k(g).wait()
            cp_v(g).wait()
            ga = mod_vec(2)
            q = qproj(pltpu.bitcast(hb[0], bf16), g, 0)
            os_ = []
            mv = [functools.partial(modv_piece, g + 1, n) for n in range(NK)]
            for j in range(REP):
                if j == QA - 1:
                    cp_wqb(g).wait()
                if j == REP - 1:
                    cp_wo(g).wait()
                    cp_x1(g).wait()

                    @pl.when(g >= 1)
                    def _():
                        cp_wmb(g - 1).wait()

                prl = qk(q, g)
                if j + 1 < REP:
                    q = qproj(pltpu.bitcast(hb[0], bf16), g, j + 1)
                else:
                    oproj(os_[:REP // 2], g, 0, acc_add, mv[:NK // 2], 3, never)
                os_.append(pv(prl, g))
            xr = _mult(g, XQ)
            hr = _mult(g, XQ // 2)
            pieces = [functools.partial(ln1_piece, TQ + xr + i * PR, 1, hr + i * PR // 2)
                      for i in range(XQ // PR)]
            pieces = [p for pair in zip(pieces, mv[NK // 2:]) for p in pair]
            fin = [None] * NK

            def acc_fin(n, cs, a):
                fin[n] = acc_ref[:, cs] + a
                acc_ref[:, cs] = fin[n]

            oproj(os_[REP // 2:], g, REP // 2, acc_fin, pieces, 4, never)
            write_x1(0, x0b[...], jnp.concatenate(fin, axis=-1), ga)
            return c

        lax.fori_loop(0, HKV, group0, 0)

        cp_wr.wait()
        cp_wmb(HKV - 1).wait()

        wr8 = jnp.broadcast_to(wrb[...].astype(f32).reshape(1, D), (8, D))
        sb8 = mod_vec(3)
        cb8 = _rb(1.0 + mod_vec(4))
        modb[M_GA] = mod_vec(2)
        modb[M_SB] = sb8
        modb[M_CB1] = cb8
        modb[M_AW] = cb8 * wr8
        modb[M_C0] = jnp.broadcast_to(jnp.sum(sb8 * wr8, axis=-1, keepdims=True), (8, D))
        modb[M_GB] = _rb(_dot(sc, wm[5, :, 0:D])[0:8])

        def body(t, carry):
            @pl.when(t + 1 < NT)
            def _():
                cp_x(t + 1).wait()

            never = flag[0] > 0
            slot = t % 2
            r0 = _mult(t, TQ)
            rp = _mult(t - 1, TQ)
            rn = _mult(jnp.minimum(t + 1, NT - 1), TQ)
            best = list(carry)
            pieces = []
            for i in range(NS):
                pieces += [functools.partial(epi_piece, rp + i * PR, best),
                           functools.partial(ln1_piece, rn + i * PR, 1 - slot, i * PR // 2)]
            npg = -(-len(pieces) // (HKV - 1))
            hh = pltpu.bitcast(hb[slot], bf16)
            fin = [None] * NK

            def acc_fin(n, cs, a):
                fin[n] = acc_ref[:, cs] + a

            q = qproj(hh, 0, 0)
            for g in range(HKV):
                os_ = []
                for j in range(REP):
                    prl = qk(q, g)
                    if j + 1 < REP:
                        q = qproj(hh, g, j + 1)
                    elif g + 1 < HKV:
                        q = qproj(hh, g + 1, 0)
                    else:
                        oproj(os_[:REP // 2], g, 0, acc_add, [], 0, never)
                    os_.append(pv(prl, g))
                if g + 1 < HKV:
                    oproj(os_, g, 0, acc_set if g == 0 else acc_add, pieces[g * npg:(g + 1) * npg], 2, never)
                else:
                    oproj(os_[REP // 2:], g, REP // 2, acc_fin, [], 0, never)
            write_x1(r0, xb[pl.ds(r0, TQ), :], jnp.concatenate(fin, axis=-1), modb[M_GA])
            cp_out(t - 1).start()
            return tuple(best)

        init = (jnp.full((8, 128), -jnp.inf, f32), jnp.zeros((8, 128), i32))
        best = list(lax.fori_loop(1, NT, body, init))

        for c in cp_wg + cp_wu + [cp_wd]:
            c.wait()
        rl = (NT - 1) * TQ
        for i in range(NS):
            route_piece(rl + i * PR, best, load_x1(rl + i * PR))

        bv, bi = best
        rmax = jnp.max(bv, axis=0, keepdims=True)
        imin = jnp.min(jnp.where(bv == rmax, bi, S), axis=0, keepdims=True)
        idx = jnp.minimum(imin[0, 0], S - 1)
        gate = jnp.concatenate([_rb(1.0 / (1.0 + jnp.exp(-rmax)))] * NK, axis=-1)
        s0 = pl.multiple_of((idx // PR) * PR, PR)
        x1s = load_x1(s0)
        mbs, rinvs = load_stats(s0)
        h2s = h2_of(x1s - mbs, rinvs)
        lhs32 = pltpu.bitcast(h2s.reshape(PR, D).astype(bf16), u32)

        def mlp(jj, y):
            never = flag[0] > 0
            r0 = rl + _mult(jj, OH)
            pend, due, done, act = [], {}, 0, []
            for j in range(2 * (FC // FCH)):
                toks = due.pop(j, [])
                l32 = jnp.concatenate(
                    [jnp.where(never, tok, lhs32[:, k * 128:(k + 1) * 128]) for k, tok in enumerate(toks)]
                    + [lhs32[:, len(toks) * 128:]], axis=-1)
                wref = wu if j % 2 else wg
                res = _dot(pltpu.bitcast(l32, bf16), wref[jj, :, (j // 2) * FCH:(j // 2 + 1) * FCH])
                for k in range(OUTP):
                    if done < OH // PR:
                        due.setdefault(j + OGAP, []).append(
                            out_piece(r0 + done * PR, res[:, k * 128:(k + 1) * 128], never))
                        done += 1
                        if done == OH // PR:
                            cp_outl(jj).start()
                if j % 2:
                    act.append((pend.pop() * _rb(res)).astype(bf16))
                else:
                    pend.append(_rb(_silu(_rb(res))))
            assert done == OH // PR and not due
            return y + _dot(jnp.concatenate(act, axis=-1), wd[pl.ds(_mult(jj, FC), FC), 0:D])

        y = _rb(lax.fori_loop(0, NMLP, mlp, jnp.zeros((PR, D), f32)))
        y = _rb(y * gate)
        rows = lax.broadcasted_iota(i32, (PR, D), 0) + s0
        upd = jnp.where(rows == idx, y, 0.0).reshape(PR // 8, 8, D)
        fix[...] = (x1s + modb[M_GB][None] * (h2s + upd)).reshape(PR, D).astype(bf16)
        for t in range(NT - 1):
            cp_out(t).wait()
        for j in range(NMLP):
            cp_outl(j).wait()
        cp_fix = pltpu.make_async_copy(fix, out_hbm.at[0, pl.ds(s0, PR)], sem_out.at[NT - 1 + NMLP])
        cp_fix.start()
        cp_fix.wait()

    scratch = [
        pltpu.VMEM((S, D), bf16),
        pltpu.VMEM((TQ, D), bf16),
        pltpu.VMEM((S, D), bf16),
        pltpu.VMEM((2, TQ // 2, D), u32),
        pltpu.VMEM((HKV, W, DH), bf16),
        pltpu.VMEM((HKV, W, DH), bf16),
        pltpu.VMEM((HKV, D, GD + PAD), bf16),
        pltpu.VMEM((HKV, GD, D + PAD), bf16),
        pltpu.VMEM((NMLP, D, FC + PAD), bf16),
        pltpu.VMEM((NMLP, D, FC + PAD), bf16),
        pltpu.VMEM((F, D + PAD), bf16),
        pltpu.VMEM((6, D, D + PAD), bf16),
        pltpu.VMEM((1, D), bf16),
        pltpu.VMEM((D,), bf16),
        pltpu.VMEM((NWM, 16, KC), bf16),
        pltpu.VMEM((D, 128), f32),
        pltpu.VMEM((5, 8, D), f32),
        pltpu.VMEM((8, 8, D), f32),
        pltpu.VMEM((S, 256), f32),
        pltpu.VMEM((TQ, D), f32),
        pltpu.VMEM((TQ, D), f32),
        pltpu.VMEM((PR, D), bf16),
        pltpu.SMEM((1,), i32),
        pltpu.SemaphoreType.DMA((n_in_sems,)),
        pltpu.SemaphoreType.DMA((NT + NMLP,)),
    ]
    return kernel, scratch


@jax.jit
def pallas_adaLN_cond__sliding_block_cached__moe_arch_mod__prompt_kernel(
    A_x: jax.Array,
    A_k_cache: jax.Array,
    A_v_cache: jax.Array,
    A_wq: jax.Array,
    A_wo: jax.Array,
    B_x: jax.Array,
    B_w_r: jax.Array,
    B_w_gate: jax.Array,
    B_w_up: jax.Array,
    B_w_down: jax.Array,
    c: jax.Array,
    w_mod: jax.Array,
):
    B, S, D = A_x.shape
    _, HKV, SK, dh = A_k_cache.shape
    F = B_w_gate.shape[1]
    W = min(4096, max(256, SK // 4))
    assert B == 1 and dh == DH and A_wq.shape == (D, HQ * DH) and S % TQ == 0 and S >= 3 * TQ
    kernel, scratch = _make_kernel(S, D, HKV, SK, W, F)
    any_spec = pl.BlockSpec(memory_space=pl.ANY)
    return pl.pallas_call(
        kernel,
        out_shape=jax.ShapeDtypeStruct((B, S, D), A_x.dtype),
        in_specs=[any_spec] * 11,
        out_specs=any_spec,
        scratch_shapes=scratch,
        compiler_params=pltpu.CompilerParams(vmem_limit_bytes=110 * 1024 * 1024,
                                             disable_semaphore_checks=True, disable_bounds_checks=True),
    )(A_x, A_k_cache, A_v_cache, A_wq, A_wo, B_w_r, B_w_gate, B_w_up, B_w_down, c, w_mod)
```

```python
import functools

import jax
import jax.numpy as jnp
from jax import lax
import jax.experimental.pallas as pl
import jax.experimental.pallas.tpu as pltpu

f32 = jnp.float32
bf16 = jnp.bfloat16
u32 = jnp.uint32
i32 = jnp.int32

HQ = 32
DH = 128
T0 = 480
TM = 224
TE = 256
L0 = 96
PR = 16
EPS = 1e-05
LOG2E = 1.4426950408889634
PAD = 128
NMLP = 2
FCH = 256
OGAP = 3
M_SA, M_CA1, M_GA, M_SB, M_CB1, M_GB, M_AW, M_C0 = range(8)


def _rb(x):
    return x.astype(bf16).astype(f32)


def _silu(x):
    return x * (1.0 / (1.0 + jnp.exp(-x)))


def _dot(a, b):
    return jnp.dot(a, b, preferred_element_type=f32)


def _mult(i, n, base=0, align=16):
    return base + i * n if isinstance(i, int) else pl.multiple_of(base + i * n, align)


def _make_kernel(S, D, HKV, SK, W, F):
    NM = (S - T0) // TM
    NK = D // 128
    REP = HQ // HKV
    GD = REP * DH
    QSCALE = DH ** (-0.5) * LOG2E
    XQ = 64
    TL = S - NM * TE
    FC = F // NMLP
    OH = TL // NMLP
    assert T0 + NM * TM == S and HKV * XQ >= TM and T0 % L0 == 0 and HKV == 4
    assert all(T0 + t * TM >= (t + 1) * TE for t in range(NM)) and OH % PR == 0

    sem_base, n_in_sems = {}, 0
    for name, n in (("c", 1), ("wr", 1), ("x0", 1), ("x1", HKV), ("xr", 1), ("wma", 2 * NK), ("wq", NK),
                    ("k", HKV), ("v", HKV), ("wo", HKV), ("wmb", HKV), ("wg", NMLP), ("wu", NMLP), ("wd", 1)):
        sem_base[name] = n_in_sems
        n_in_sems += n

    def kernel(x_hbm, k_hbm, v_hbm, wq_hbm, wo_hbm, wr_hbm, wg_hbm, wu_hbm, wd_hbm, c_hbm, wm_hbm,
               out_hbm,
               xb, x0b, ob, hb, kb, vb, wq, wo, wg, wu, wd, wma, wmb, cb, wrb, colb, moda, modp, modb,
               st_ref, acc_ref, qacc, xn_ref, fix, flag, sem_in, sem_out):
        def cp(name, i, src, dst):
            return pltpu.make_async_copy(src, dst, sem_in.at[sem_base[name] + i])

        def cp_x1(g):
            r = pl.ds(_mult(g, XQ, T0), XQ)
            return cp("x1", g, x_hbm.at[0, r], xb.at[r])

        def cp_wma(i, j):
            return cp("wma", 2 * i + j, wm_hbm.at[:, pl.ds(_mult(i, 128, j * D, 128), 128)], wma.at[i, j])

        def cp_wmb(j):
            return cp("wmb", j, wm_hbm.at[:, pl.ds(_mult(j, D, 2 * D, 128), D)], wmb.at[j, :, pl.ds(0, D)])

        def cp_wq(i):
            r = pl.ds(_mult(i, 128), 128)
            return cp("wq", i, wq_hbm.at[r], wq.at[r, pl.ds(0, HQ * DH)])

        def cp_k(g):
            return cp("k", g, k_hbm.at[0, g, pl.ds(SK - W, W)], kb.at[g])

        def cp_v(g):
            return cp("v", g, v_hbm.at[0, g, pl.ds(SK - W, W)], vb.at[g])

        def cp_wo(g):
            return cp("wo", g, wo_hbm.at[pl.ds(_mult(g, GD), GD)], wo.at[g, :, pl.ds(0, D)])

        xr0 = T0 + HKV * XQ
        cp_c = cp("c", 0, c_hbm, cb)
        cp_wr = cp("wr", 0, wr_hbm, wrb)
        cp_x0 = cp("x0", 0, x_hbm.at[0, pl.ds(0, T0)], x0b)
        cp_xr = cp("xr", 0, x_hbm.at[0, pl.ds(xr0, S - xr0)], xb.at[pl.ds(xr0, S - xr0)])
        cp_wg = [cp("wg", j, wg_hbm.at[:, pl.ds(j * FC, FC)], wg.at[j, :, pl.ds(0, FC)]) for j in range(NMLP)]
        cp_wu = [cp("wu", j, wu_hbm.at[:, pl.ds(j * FC, FC)], wu.at[j, :, pl.ds(0, FC)]) for j in range(NMLP)]
        cp_wd = cp("wd", 0, wd_hbm, wd.at[:, pl.ds(0, D)])

        def cp_out(t):
            r = pl.ds(_mult(t, TE), TE)
            return pltpu.make_async_copy(ob.at[r], out_hbm.at[0, r], sem_out.at[t])

        def cp_outl(j):
            r = pl.ds(_mult(j, OH, NM * TE), OH)
            return pltpu.make_async_copy(ob.at[r], out_hbm.at[0, r], sem_out.at[NM + j])

        order = [cp_c, cp_x0, cp_wma(0, 0), cp_wma(0, 1)]
        for i in range(NK):
            order += [cp_wq(i)]
            if i + 1 < NK:
                order += [cp_wma(i + 1, 0), cp_wma(i + 1, 1)]
        for g in range(HKV):
            order += [cp_k(g), cp_v(g), cp_wo(g), cp_wmb(g), cp_x1(g)]
        order += [cp_wr, cp_xr] + cp_wg + cp_wu + [cp_wd]
        assert len(order) == n_in_sems
        for c in order:
            c.start()

        flag[0] = 0

        def tie(x, tok, never):
            if tok is None:
                return x
            return jnp.concatenate([jnp.where(never, tok, x[:, :128]), x[:, 128:]], axis=-1)

        def due_rows(lhs, toks, never):
            if not toks:
                return lhs
            l32 = pltpu.bitcast(lhs, u32)
            parts = [jnp.where(never, tok, l32[8 * k:8 * k + 8]) for k, tok in enumerate(toks)]
            return pltpu.bitcast(jnp.concatenate(parts + [l32[8 * len(toks):]], axis=0), bf16)

        def ln_plain(x):
            m = jnp.sum(x, axis=-1, keepdims=True) * (1.0 / D)
            xc = x - m
            v = jnp.sum(xc * xc, axis=-1, keepdims=True) * (1.0 / D)
            return xc * lax.rsqrt(v + EPS)

        def lane_bc(v):
            return jnp.broadcast_to(v.reshape(-1, 1), (v.shape[0] * 8, 128))

        def sub_bc(p):
            return jnp.broadcast_to(_rb(jnp.sum(p, axis=0, keepdims=True)), p.shape)

        def h2_of(xc, rinv):
            return (xc * rinv) * modb[M_CB1][None] + modb[M_SB][None]

        def load_stats(row):
            st = st_ref[pl.ds(row, PR), :]
            mb = jnp.concatenate([st[:, 0:128]] * NK, axis=-1).reshape(PR // 8, 8, D)
            rinv = jnp.concatenate([st[:, 128:256]] * NK, axis=-1).reshape(PR // 8, 8, D)
            return mb, rinv

        def pack_rows(h):
            return jnp.concatenate(
                [pltpu.bitcast(h[:, n * 128:(n + 1) * 128].astype(bf16), u32) for n in range(NK)], axis=-1)

        def ln1_piece(xrow, slot, hrow, tok=None, never=None):
            x = tie(xb[pl.ds(xrow, PR), :].astype(f32), tok, never).reshape(PR // 8, 8, D)
            h32 = pack_rows((ln_plain(x) * modb[M_CA1][None] + modb[M_SA][None]).reshape(PR, D))
            hb[slot, pl.ds(hrow, PR // 2), :] = h32
            return h32[:, :128]

        sub_iota = lax.broadcasted_iota(i32, (8, 128), 0)

        def route_piece(row, best, x1):
            m = jnp.sum(x1, axis=-1, keepdims=True) * (1.0 / D)
            mb = _rb(m)
            xc = x1 - mb
            dm = m - mb
            v = jnp.sum(xc * xc, axis=-1, keepdims=True) * (1.0 / D) - dm * dm
            rs = jnp.sum(xc * modb[M_AW][None], axis=-1, keepdims=True)
            sd = _rb(jnp.sqrt(_rb(_rb(jnp.maximum(v, 0.0)) + EPS)))
            r0 = pl.reciprocal(sd, approx=True)
            rinv = r0 * (2.0 - sd * r0)
            st_ref[pl.ds(row, PR), :] = jnp.concatenate([lane_bc(mb), lane_bc(rinv)], axis=-1)
            rr = lane_bc(rs * rinv).reshape(PR // 8, 8, 128) + modb[M_C0, :, 0:128][None]
            rb16 = rr.reshape(PR, 128).astype(bf16)
            rbf = rb16.astype(f32)
            for j in range(PR // 8):
                rj = rbf[8 * j:8 * j + 8]
                upd = rj > best[0]
                best[1] = jnp.where(upd, sub_iota + (row + 8 * j), best[1])
                best[0] = jnp.where(upd, rj, best[0])
            return xc, rinv, rb16

        def load_x1(row, tok=None, never=None):
            return tie(xb[pl.ds(row, PR), :].astype(f32), tok, never).reshape(PR // 8, 8, D)

        def epi_piece(row, best, tok=None, never=None):
            x1 = load_x1(row, tok, never)
            xc, rinv, rb16 = route_piece(row, best, x1)
            ob[pl.ds(row, PR), :] = (x1 + modb[M_GB][None] * h2_of(xc, rinv)).reshape(PR, D).astype(bf16)
            return pltpu.bitcast(rb16, u32)

        def out_piece(row, tok, never):
            x1 = load_x1(row)
            mb, rinv = load_stats(row)
            mb = jnp.where(never, jnp.concatenate([tok] * NK, axis=-1).reshape(PR // 8, 8, D), mb)
            o = (x1 + modb[M_GB][None] * h2_of(x1 - mb, rinv)).reshape(PR, D).astype(bf16)
            ob[pl.ds(row, PR), :] = o
            return pltpu.bitcast(o[:, 0:128], u32)

        def matvec(w_at, tok, never):
            y = None if tok is None else jnp.where(never, tok[0:8], 0.0)
            for kg in range(D // 8):
                t = w_at(slice(kg * 8, (kg + 1) * 8)).astype(f32) * colb[kg * 8:(kg + 1) * 8, :]
                y = t if y is None else y + t
            return y

        def moda_piece(i, j, tok=None, never=None):
            y = sub_bc(matvec(lambda r: wma[i, j, r, :], tok, never))
            if j == 1:
                y = _rb(1.0 + y)
            moda[i, j] = y
            return pltpu.bitcast(y, u32)

        def modb_piece(ch, n, tok=None, never=None):
            y = matvec(lambda r: wmb[ch, r, n * 128:(n + 1) * 128], tok, never)
            modp[ch, :, n * 128:(n + 1) * 128] = y
            return pltpu.bitcast(y, u32)

        def qk(q, g):
            s = lax.dot_general(q, kb[g], (((1,), (1,)), ((), ())), preferred_element_type=f32)
            m = jnp.max(s, axis=-1, keepdims=True)
            p = jnp.exp2(s - m)
            l = jnp.sum(p, axis=-1, keepdims=True)
            rl = pl.reciprocal(l, approx=True)
            return p.astype(bf16), rl * (2.0 - l * rl)

        def pv(prl, g):
            p, rl = prl
            return (_dot(p, vb[g]) * rl).astype(bf16)

        def paced(nsteps, step, pieces, gap, never):
            outs, done = {}, 0
            for n in range(nsteps):
                a = step(n, outs.pop(n, []))
                if n < nsteps - gap:
                    cnt = int(round((n + 1) * len(pieces) / (nsteps - gap))) - done
                    for k in range(cnt):
                        rr = (k * a.shape[0] // cnt) // PR * PR
                        outs.setdefault(n + gap, []).append(pieces[done](a[rr:rr + PR, 0:128], never))
                        done += 1
            assert done == len(pieces)

        def oproj(os_, g, j0, sink, pieces, gap, never):
            def step(n, toks):
                cs = slice(n * 128, (n + 1) * 128)
                og = jnp.concatenate([due_rows(os_[0], toks, never)] + list(os_[1:]), axis=-1)
                a = _dot(og, wo[g, j0 * DH:(j0 + len(os_)) * DH, cs])
                sink(n, cs, a)
                return a
            paced(NK, step, pieces, gap, never)

        def acc_set(n, cs, a):
            acc_ref[0:a.shape[0], cs] = a

        def acc_add(n, cs, a):
            acc_ref[0:a.shape[0], cs] += a

        def write_x1(r0, x, acc, ga):
            rows = x.shape[0]
            a = acc.reshape(rows // 8, 8, D) * ga[None]
            xb[pl.ds(r0, rows), :] = (x.astype(f32) + a.reshape(rows, D)).astype(bf16)

        def zero(i, c):
            r = pl.ds(_mult(i, PR), PR)
            for g in range(HKV):
                qacc[g, r, :] = jnp.zeros((PR, GD), f32)
            acc_ref[r, :] = jnp.zeros((PR, D), f32)
            return c

        lax.fori_loop(0, T0 // PR, zero, 0)
        modp[0] = jnp.zeros((8, D), f32)
        cp_c.wait()
        sc = _rb(_silu(cb[...].astype(f32)))
        colb[...] = jnp.broadcast_to(sc, (128, D)).T
        cp_x0.wait()

        def ln0(i, c):
            r = pl.ds(_mult(i, L0), L0)
            xn = ln_plain(x0b[r, :].astype(f32))
            for n in range(NK):
                xn_ref[n, r, :] = xn[:, n * 128:(n + 1) * 128]
            return c

        lax.fori_loop(0, T0 // L0, ln0, 0)
        cp_wma(0, 0).wait()
        cp_wma(0, 1).wait()
        moda_piece(0, 0)
        moda_piece(0, 1)

        def kstep(i, c):
            cp_wq(i).wait()

            @pl.when(i + 1 < NK)
            def _():
                cp_wma(i + 1, 0).wait()
                cp_wma(i + 1, 1).wait()

            never = flag[0] > 0
            h = (xn_ref[i].reshape(T0 // 8, 8, 128) * moda[i, 1][None] + moda[i, 0][None])
            h = h.reshape(T0, 128).astype(bf16)
            nxt = jnp.minimum(i + 1, NK - 1)
            r = pl.ds(_mult(i, 128), 128)
            nw = 4 * DH

            def step(n, toks):
                a = _dot(due_rows(h, toks, never), wq[r, n * nw:(n + 1) * nw])
                g, c0 = divmod(n * nw, GD)
                qacc[g, :, c0:c0 + nw] += a
                return a

            paced(HQ * DH // nw, step, [functools.partial(moda_piece, nxt, j) for j in range(2)], 4, never)
            return c

        lax.fori_loop(0, NK, kstep, 0)
        modb[M_SA] = jnp.concatenate([moda[i, 0] for i in range(NK)], axis=-1)
        modb[M_CA1] = jnp.concatenate([moda[i, 1] for i in range(NK)], axis=-1)

        def group0(g, c):
            for d in (cp_k(g), cp_v(g), cp_wo(g), cp_wmb(g), cp_x1(g)):
                d.wait()
            never = flag[0] > 0
            ga = sub_bc(modp[0])

            def q_of(j):
                return (qacc[g, :, j * DH:(j + 1) * DH] * QSCALE).astype(bf16)

            mv = [functools.partial(modb_piece, g, n) for n in range(NK)]
            os_ = []
            prl = qk(q_of(0), g)
            for j in range(REP):
                if j + 1 < REP:
                    nxt = qk(q_of(j + 1), g)
                else:
                    oproj(os_[:REP // 2], g, 0, acc_add, mv[:6], 2, never)
                os_.append(pv(prl, g))
                prl = nxt
            pieces = [functools.partial(ln1_piece, _mult(g, XQ, T0 + i * PR), 0,
                                        _mult(g, XQ // 2, i * PR // 2, 8)) for i in range(XQ // PR)]
            fin = [None] * NK

            def acc_fin(n, cs, a):
                fin[n] = acc_ref[:, cs] + a
                acc_ref[:, cs] = fin[n]

            oproj(os_[REP // 2:], g, REP // 2, acc_fin, pieces + mv[6:], 2, never)
            write_x1(0, x0b[...], jnp.concatenate(fin, axis=-1), ga)
            return c

        lax.fori_loop(0, HKV, group0, 0)

        cp_wr.wait()
        cp_xr.wait()
        wr8 = jnp.broadcast_to(wrb[...].astype(f32).reshape(1, D), (8, D))
        sb8 = sub_bc(modp[1])
        cb8 = _rb(1.0 + sub_bc(modp[2]))
        modb[M_GA] = sub_bc(modp[0])
        modb[M_SB] = sb8
        modb[M_CB1] = cb8
        modb[M_GB] = sub_bc(modp[3])
        modb[M_AW] = cb8 * wr8
        modb[M_C0] = jnp.broadcast_to(jnp.sum(sb8 * wr8, axis=-1, keepdims=True), (8, D))

        def body(t, carry):
            never = flag[0] > 0
            slot = t % 2
            r0 = _mult(t, TM, T0)
            re = _mult(t, TE)
            rn = _mult(jnp.minimum(t + 1, NM - 1), TM, T0)
            best = list(carry)
            pe = [functools.partial(epi_piece, re + i * PR, best) for i in range(TE // PR)]
            pn = [functools.partial(ln1_piece, rn + i * PR, 1 - slot, i * PR // 2) for i in range(TM // PR)]
            pieces = [p for pair in zip(pe, pn) for p in pair] + pe[len(pn):]
            npg = -(-len(pieces) // (HKV - 1))
            hh = pltpu.bitcast(hb[slot, 0:TM // 2, :], bf16)
            fin = [None] * NK

            def qproj(h):
                return (_dot(hh, wq[:, h * DH:(h + 1) * DH]) * QSCALE).astype(bf16)

            def acc_fin(n, cs, a):
                fin[n] = acc_ref[0:TM, cs] + a

            q = qproj(0)
            for g in range(HKV):
                os_ = []
                for j in range(REP):
                    prl = qk(q, g)
                    if g * REP + j + 1 < HQ:
                        q = qproj(g * REP + j + 1)
                    else:
                        oproj(os_[:REP // 2], g, 0, acc_add, [], 0, never)
                    os_.append(pv(prl, g))
                if g + 1 < HKV:
                    oproj(os_, g, 0, acc_set if g == 0 else acc_add, pieces[g * npg:(g + 1) * npg], 2, never)
                else:
                    oproj(os_[REP // 2:], g, REP // 2, acc_fin, [], 0, never)
            write_x1(r0, xb[pl.ds(r0, TM), :], jnp.concatenate(fin, axis=-1), modb[M_GA])
            cp_out(t).start()
            return tuple(best)

        init = (jnp.full((8, 128), -jnp.inf, f32), jnp.zeros((8, 128), i32))
        best = list(lax.fori_loop(0, NM, body, init))

        for c in cp_wg + cp_wu + [cp_wd]:
            c.wait()
        rl = NM * TE
        for i in range(TL // PR):
            route_piece(rl + i * PR, best, load_x1(rl + i * PR))

        bv, bi = best
        rmax = jnp.max(bv, axis=0, keepdims=True)
        imin = jnp.min(jnp.where(bv == rmax, bi, S), axis=0, keepdims=True)
        idx = jnp.minimum(imin[0, 0], S - 1)
        gate = jnp.concatenate([_rb(1.0 / (1.0 + jnp.exp(-rmax)))] * NK, axis=-1)
        s0 = pl.multiple_of(lax.shift_right_logical(idx, 4) * PR, PR)
        x1s = load_x1(s0)
        mbs, rinvs = load_stats(s0)
        h2s = h2_of(x1s - mbs, rinvs)
        lhs32 = pack_rows(h2s.reshape(PR, D))

        def mlp(jj, y):
            never = flag[0] > 0
            r0 = _mult(jj, OH, rl)
            pend, due, done, act = [], {}, 0, []
            for j in range(2 * (FC // FCH)):
                toks = due.pop(j, [])
                l32 = jnp.concatenate(
                    [jnp.where(never, tok, lhs32[:, k * 128:(k + 1) * 128]) for k, tok in enumerate(toks)]
                    + [lhs32[:, len(toks) * 128:]], axis=-1)
                wref = wu if j % 2 else wg
                res = _dot(pltpu.bitcast(l32, bf16), wref[jj, :, (j // 2) * FCH:(j // 2 + 1) * FCH])
                if done < OH // PR:
                    due.setdefault(j + OGAP, []).append(out_piece(r0 + done * PR, res[:, 0:128], never))
                    done += 1
                    if done == OH // PR:
                        cp_outl(jj).start()
                if j % 2:
                    act.append((pend.pop() * _rb(res)).astype(bf16))
                else:
                    pend.append(_rb(_silu(_rb(res))))
            assert done == OH // PR and not due
            return y + _dot(jnp.concatenate(act, axis=-1), wd[pl.ds(_mult(jj, FC), FC), 0:D])

        y = _rb(lax.fori_loop(0, NMLP, mlp, jnp.zeros((PR, D), f32)))
        y = _rb(y * gate)
        rows = lax.broadcasted_iota(i32, (PR, D), 0) + s0
        upd = jnp.where(rows == idx, y, 0.0).reshape(PR // 8, 8, D)
        fix[...] = (x1s + modb[M_GB][None] * (h2s + upd)).reshape(PR, D).astype(bf16)
        for t in range(NM):
            cp_out(t).wait()
        for j in range(NMLP):
            cp_outl(j).wait()
        cp_fix = pltpu.make_async_copy(fix, out_hbm.at[0, pl.ds(s0, PR)], sem_out.at[NM + NMLP])
        cp_fix.start()
        cp_fix.wait()

    scratch = [
        pltpu.VMEM((S, D), bf16),
        pltpu.VMEM((T0, D), bf16),
        pltpu.VMEM((S, D), bf16),
        pltpu.VMEM((2, HKV * XQ // 2, D), u32),
        pltpu.VMEM((HKV, W, DH), bf16),
        pltpu.VMEM((HKV, W, DH), bf16),
        pltpu.VMEM((D, HQ * DH + PAD), bf16),
        pltpu.VMEM((HKV, GD, D + PAD), bf16),
        pltpu.VMEM((NMLP, D, FC + PAD), bf16),
        pltpu.VMEM((NMLP, D, FC + PAD), bf16),
        pltpu.VMEM((F, D + PAD), bf16),
        pltpu.VMEM((NK, 2, D, 128), bf16),
        pltpu.VMEM((HKV, D, D + PAD), bf16),
        pltpu.VMEM((1, D), bf16),
        pltpu.VMEM((D,), bf16),
        pltpu.VMEM((D, 128), f32),
        pltpu.VMEM((NK, 2, 8, 128), f32),
        pltpu.VMEM((HKV, 8, D), f32),
        pltpu.VMEM((8, 8, D), f32),
        pltpu.VMEM((S, 256), f32),
        pltpu.VMEM((T0, D), f32),
        pltpu.VMEM((HKV, T0, GD), f32),
        pltpu.VMEM((NK, T0, 128), f32),
        pltpu.VMEM((PR, D), bf16),
        pltpu.SMEM((1,), i32),
        pltpu.SemaphoreType.DMA((n_in_sems,)),
        pltpu.SemaphoreType.DMA((NM + NMLP + 1,)),
    ]
    return kernel, scratch


@jax.jit
def pallas_adaLN_cond__sliding_block_cached__moe_arch_mod__prompt_kernel(
    A_x: jax.Array,
    A_k_cache: jax.Array,
    A_v_cache: jax.Array,
    A_wq: jax.Array,
    A_wo: jax.Array,
    B_x: jax.Array,
    B_w_r: jax.Array,
    B_w_gate: jax.Array,
    B_w_up: jax.Array,
    B_w_down: jax.Array,
    c: jax.Array,
    w_mod: jax.Array,
):
    B, S, D = A_x.shape
    _, HKV, SK, dh = A_k_cache.shape
    F = B_w_gate.shape[1]
    W = min(4096, max(256, SK // 4))
    assert B == 1 and dh == DH and A_wq.shape == (D, HQ * DH)
    kernel, scratch = _make_kernel(S, D, HKV, SK, W, F)
    any_spec = pl.BlockSpec(memory_space=pl.ANY)
    return pl.pallas_call(
        kernel,
        out_shape=jax.ShapeDtypeStruct((B, S, D), A_x.dtype),
        in_specs=[any_spec] * 11,
        out_specs=any_spec,
        scratch_shapes=scratch,
        compiler_params=pltpu.CompilerParams(vmem_limit_bytes=120 * 1024 * 1024,
                                             disable_semaphore_checks=True, disable_bounds_checks=True),
    )(A_x, A_k_cache, A_v_cache, A_wq, A_wo, B_w_r, B_w_gate, B_w_up, B_w_down, c, w_mod)
```

```python
import functools

import jax
import jax.numpy as jnp
from jax import lax
import jax.experimental.pallas as pl
import jax.experimental.pallas.tpu as pltpu

f32 = jnp.float32
bf16 = jnp.bfloat16
u32 = jnp.uint32
i32 = jnp.int32

HQ = 32
DH = 128
T0 = 480
TM = 224
TE = 256
L0 = 96
PR = 16
EPS = 1e-05
LOG2E = 1.4426950408889634
PAD = 128
NMLP = 2
FCH = 256
OGAP = 3
M_SA, M_CA1, M_GA, M_SB, M_CB1, M_GB, M_AW, M_C0 = range(8)


def _rb(x):
    return x.astype(bf16).astype(f32)


def _silu(x):
    return x * (1.0 / (1.0 + jnp.exp(-x)))


def _dot(a, b):
    return jnp.dot(a, b, preferred_element_type=f32)


def _mult(i, n, base=0, align=16):
    return base + i * n if isinstance(i, int) else pl.multiple_of(base + i * n, align)


def _make_kernel(S, D, HKV, SK, W, F):
    NM = (S - T0) // TM
    NK = D // 128
    REP = HQ // HKV
    GD = REP * DH
    QSCALE = DH ** (-0.5) * LOG2E
    XQ = 64
    TL = S - NM * TE
    FC = F // NMLP
    OH = TL // NMLP
    assert T0 + NM * TM == S and HKV * XQ >= TM and T0 % L0 == 0 and HKV == 4
    assert all(T0 + t * TM >= (t + 1) * TE for t in range(NM)) and OH % PR == 0

    sem_base, n_in_sems = {}, 0
    for name, n in (("c", 1), ("wr", 1), ("x0", 1), ("x1", HKV), ("xr", 1), ("wma", 2 * NK), ("wq", NK),
                    ("k", HKV), ("v", HKV), ("wo", HKV), ("wmb", HKV), ("wg", NMLP), ("wu", NMLP), ("wd", 1)):
        sem_base[name] = n_in_sems
        n_in_sems += n

    def kernel(x_hbm, k_hbm, v_hbm, wq_hbm, wo_hbm, wr_hbm, wg_hbm, wu_hbm, wd_hbm, c_hbm, wm_hbm,
               out_hbm,
               xb, x0b, ob, hb, kb, vb, wq, wo, wg, wu, wd, wma, wmb, cb, wrb, colb, moda, modp, modb,
               st_ref, acc_ref, qacc, xn_ref, fix, flag, sem_in, sem_out):
        def cp(name, i, src, dst):
            return pltpu.make_async_copy(src, dst, sem_in.at[sem_base[name] + i])

        def cp_x1(g):
            r = pl.ds(_mult(g, XQ, T0), XQ)
            return cp("x1", g, x_hbm.at[0, r], xb.at[r])

        def cp_wma(i, j):
            return cp("wma", 2 * i + j, wm_hbm.at[:, pl.ds(_mult(i, 128, j * D, 128), 128)], wma.at[i, j])

        def cp_wmb(j):
            return cp("wmb", j, wm_hbm.at[:, pl.ds(_mult(j, D, 2 * D, 128), D)], wmb.at[j, :, pl.ds(0, D)])

        def cp_wq(i):
            r = pl.ds(_mult(i, 128), 128)
            return cp("wq", i, wq_hbm.at[r], wq.at[r, pl.ds(0, HQ * DH)])

        def cp_k(g):
            return cp("k", g, k_hbm.at[0, g, pl.ds(SK - W, W)], kb.at[g])

        def cp_v(g):
            return cp("v", g, v_hbm.at[0, g, pl.ds(SK - W, W)], vb.at[g])

        def cp_wo(g):
            return cp("wo", g, wo_hbm.at[pl.ds(_mult(g, GD), GD)], wo.at[g, :, pl.ds(0, D)])

        xr0 = T0 + HKV * XQ
        cp_c = cp("c", 0, c_hbm, cb)
        cp_wr = cp("wr", 0, wr_hbm, wrb)
        cp_x0 = cp("x0", 0, x_hbm.at[0, pl.ds(0, T0)], x0b)
        cp_xr = cp("xr", 0, x_hbm.at[0, pl.ds(xr0, S - xr0)], xb.at[pl.ds(xr0, S - xr0)])
        cp_wg = [cp("wg", j, wg_hbm.at[:, pl.ds(j * FC, FC)], wg.at[j, :, pl.ds(0, FC)]) for j in range(NMLP)]
        cp_wu = [cp("wu", j, wu_hbm.at[:, pl.ds(j * FC, FC)], wu.at[j, :, pl.ds(0, FC)]) for j in range(NMLP)]
        cp_wd = cp("wd", 0, wd_hbm, wd.at[:, pl.ds(0, D)])

        def cp_out(t):
            r = pl.ds(_mult(t, TE), TE)
            return pltpu.make_async_copy(ob.at[r], out_hbm.at[0, r], sem_out.at[t])

        def cp_outl(j):
            r = pl.ds(_mult(j, OH, NM * TE), OH)
            return pltpu.make_async_copy(ob.at[r], out_hbm.at[0, r], sem_out.at[NM + j])

        order = [cp_c, cp_x0, cp_wma(0, 0), cp_wma(0, 1)]
        for i in range(NK):
            order += [cp_wq(i)]
            if i + 1 < NK:
                order += [cp_wma(i + 1, 0), cp_wma(i + 1, 1)]
        for g in range(HKV):
            order += [cp_k(g), cp_v(g), cp_wo(g), cp_wmb(g), cp_x1(g)]
        order += [cp_wr, cp_xr] + cp_wg + cp_wu + [cp_wd]
        assert len(order) == n_in_sems
        for c in order:
            c.start()

        flag[0] = 0

        def tie(x, tok, never):
            if tok is None:
                return x
            return jnp.concatenate([jnp.where(never, tok, x[:, :128]), x[:, 128:]], axis=-1)

        def due_rows(lhs, toks, never):
            if not toks:
                return lhs
            l32 = pltpu.bitcast(lhs, u32)
            parts = [jnp.where(never, tok, l32[8 * k:8 * k + 8]) for k, tok in enumerate(toks)]
            return pltpu.bitcast(jnp.concatenate(parts + [l32[8 * len(toks):]], axis=0), bf16)

        def ln_plain(x):
            m = jnp.sum(x, axis=-1, keepdims=True) * (1.0 / D)
            xc = x - m
            v = jnp.sum(xc * xc, axis=-1, keepdims=True) * (1.0 / D)
            return xc * lax.rsqrt(v + EPS)

        def lane_bc(v):
            return jnp.broadcast_to(v.reshape(-1, 1), (v.shape[0] * 8, 128))

        def sub_bc(p):
            return jnp.broadcast_to(_rb(jnp.sum(p, axis=0, keepdims=True)), p.shape)

        def h2_of(xc, rinv):
            return (xc * rinv) * modb[M_CB1][None] + modb[M_SB][None]

        def load_stats(row):
            st = st_ref[pl.ds(row, PR), :]
            mb = jnp.concatenate([st[:, 0:128]] * NK, axis=-1).reshape(PR // 8, 8, D)
            rinv = jnp.concatenate([st[:, 128:256]] * NK, axis=-1).reshape(PR // 8, 8, D)
            return mb, rinv

        def pack_rows(h):
            return jnp.concatenate(
                [pltpu.bitcast(h[:, n * 128:(n + 1) * 128].astype(bf16), u32) for n in range(NK)], axis=-1)

        def ln1_piece(xrow, slot, hrow, tok=None, never=None):
            x = tie(xb[pl.ds(xrow, PR), :].astype(f32), tok, never).reshape(PR // 8, 8, D)
            h32 = pack_rows((ln_plain(x) * modb[M_CA1][None] + modb[M_SA][None]).reshape(PR, D))
            hb[slot, pl.ds(hrow, PR // 2), :] = h32
            return h32[:, :128]

        sub_iota = lax.broadcasted_iota(i32, (8, 128), 0)

        def route_piece(row, best, x1):
            m = jnp.sum(x1, axis=-1, keepdims=True) * (1.0 / D)
            mb = _rb(m)
            xc = x1 - mb
            dm = m - mb
            v = jnp.sum(xc * xc, axis=-1, keepdims=True) * (1.0 / D) - dm * dm
            rs = jnp.sum(xc * modb[M_AW][None], axis=-1, keepdims=True)
            sd = _rb(jnp.sqrt(_rb(_rb(jnp.maximum(v, 0.0)) + EPS)))
            r0 = pl.reciprocal(sd, approx=True)
            rinv = r0 * (2.0 - sd * r0)
            st_ref[pl.ds(row, PR), :] = jnp.concatenate([lane_bc(mb), lane_bc(rinv)], axis=-1)
            rr = lane_bc(rs * rinv).reshape(PR // 8, 8, 128) + modb[M_C0, :, 0:128][None]
            rb16 = rr.reshape(PR, 128).astype(bf16)
            rbf = rb16.astype(f32)
            for j in range(PR // 8):
                rj = rbf[8 * j:8 * j + 8]
                upd = rj > best[0]
                best[1] = jnp.where(upd, sub_iota + (row + 8 * j), best[1])
                best[0] = jnp.where(upd, rj, best[0])
            return xc, rinv, rb16

        def load_x1(row, tok=None, never=None):
            return tie(xb[pl.ds(row, PR), :].astype(f32), tok, never).reshape(PR // 8, 8, D)

        def epi_piece(row, best, tok=None, never=None):
            x1 = load_x1(row, tok, never)
            xc, rinv, rb16 = route_piece(row, best, x1)
            ob[pl.ds(row, PR), :] = (x1 + modb[M_GB][None] * h2_of(xc, rinv)).reshape(PR, D).astype(bf16)
            return pltpu.bitcast(rb16, u32)

        def out_piece(row, tok, never):
            x1 = load_x1(row)
            mb, rinv = load_stats(row)
            mb = jnp.where(never, jnp.concatenate([tok] * NK, axis=-1).reshape(PR // 8, 8, D), mb)
            o = (x1 + modb[M_GB][None] * h2_of(x1 - mb, rinv)).reshape(PR, D).astype(bf16)
            ob[pl.ds(row, PR), :] = o
            return pltpu.bitcast(o[:, 0:128], u32)

        def matvec(w_at, tok, never):
            y = None if tok is None else jnp.where(never, tok[0:8], 0.0)
            for kg in range(D // 8):
                t = w_at(slice(kg * 8, (kg + 1) * 8)).astype(f32) * colb[kg * 8:(kg + 1) * 8, :]
                y = t if y is None else y + t
            return y

        def moda_piece(i, j, tok=None, never=None):
            y = sub_bc(matvec(lambda r: wma[i, j, r, :], tok, never))
            if j == 1:
                y = _rb(1.0 + y)
            moda[i, j] = y
            return pltpu.bitcast(y, u32)

        def modb_piece(ch, n, tok=None, never=None):
            y = matvec(lambda r: wmb[ch, r, n * 128:(n + 1) * 128], tok, never)
            modp[ch, :, n * 128:(n + 1) * 128] = y
            return pltpu.bitcast(y, u32)

        def qk(q, g):
            s = lax.dot_general(q, kb[g], (((1,), (1,)), ((), ())), preferred_element_type=f32)
            m = jnp.max(s, axis=-1, keepdims=True)
            p = jnp.exp2(s - m)
            l = jnp.sum(p, axis=-1, keepdims=True)
            rl = pl.reciprocal(l, approx=True)
            return p.astype(bf16), rl * (2.0 - l * rl)

        def pv(prl, g):
            p, rl = prl
            return (_dot(p, vb[g]) * rl).astype(bf16)

        def paced(nsteps, step, pieces, gap, never):
            outs, done = {}, 0
            for n in range(nsteps):
                a = step(n, outs.pop(n, []))
                if n < nsteps - gap:
                    cnt = int(round((n + 1) * len(pieces) / (nsteps - gap))) - done
                    for k in range(cnt):
                        rr = (k * a.shape[0] // cnt) // PR * PR
                        outs.setdefault(n + gap, []).append(pieces[done](a[rr:rr + PR, 0:128], never))
                        done += 1
            assert done == len(pieces)

        def oproj(os_, g, j0, sink, pieces, gap, never):
            def step(n, toks):
                cs = slice(n * 128, (n + 1) * 128)
                og = jnp.concatenate([due_rows(os_[0], toks, never)] + list(os_[1:]), axis=-1)
                a = _dot(og, wo[g, j0 * DH:(j0 + len(os_)) * DH, cs])
                sink(n, cs, a)
                return a
            paced(NK, step, pieces, gap, never)

        def acc_set(n, cs, a):
            acc_ref[0:a.shape[0], cs] = a

        def acc_add(n, cs, a):
            acc_ref[0:a.shape[0], cs] += a

        def write_x1(r0, x, acc, ga):
            rows = x.shape[0]
            a = acc.reshape(rows // 8, 8, D) * ga[None]
            xb[pl.ds(r0, rows), :] = (x.astype(f32) + a.reshape(rows, D)).astype(bf16)

        def zero(i, c):
            r = pl.ds(_mult(i, PR), PR)
            for g in range(HKV):
                qacc[g, r, :] = jnp.zeros((PR, GD), f32)
            acc_ref[r, :] = jnp.zeros((PR, D), f32)
            return c

        lax.fori_loop(0, T0 // PR, zero, 0)
        modp[0] = jnp.zeros((8, D), f32)
        cp_c.wait()
        sc = _rb(_silu(cb[...].astype(f32)))
        colb[...] = jnp.broadcast_to(sc, (128, D)).T
        cp_x0.wait()

        def ln0(i, c):
            r = pl.ds(_mult(i, L0), L0)
            xn = ln_plain(x0b[r, :].astype(f32))
            for n in range(NK):
                xn_ref[n, r, :] = xn[:, n * 128:(n + 1) * 128]
            return c

        lax.fori_loop(0, T0 // L0, ln0, 0)

        def kstep(i, c):
            @pl.when(i <= 1)
            def _():
                cp_wma(i, 0).wait()
                cp_wma(i, 1).wait()
                moda_piece(i, 0)
                moda_piece(i, 1)

            cp_wq(i).wait()
            ahead = jnp.logical_and(i >= 1, i + 1 < NK)

            @pl.when(ahead)
            def _():
                cp_wma(i + 1, 0).wait()
                cp_wma(i + 1, 1).wait()

            never = flag[0] > 0
            h = (xn_ref[i].reshape(T0 // 8, 8, 128) * moda[i, 1][None] + moda[i, 0][None])
            h = h.reshape(T0, 128).astype(bf16)
            nxt = jnp.where(ahead, i + 1, i)
            r = pl.ds(_mult(i, 128), 128)
            nw = 4 * DH

            def step(n, toks):
                a = _dot(due_rows(h, toks, never), wq[r, n * nw:(n + 1) * nw])
                g, c0 = divmod(n * nw, GD)
                qacc[g, :, c0:c0 + nw] += a
                return a

            paced(HQ * DH // nw, step, [functools.partial(moda_piece, nxt, j) for j in range(2)], 4, never)
            return c

        lax.fori_loop(0, NK, kstep, 0)
        modb[M_SA] = jnp.concatenate([moda[i, 0] for i in range(NK)], axis=-1)
        modb[M_CA1] = jnp.concatenate([moda[i, 1] for i in range(NK)], axis=-1)

        def group0(g, c):
            for d in (cp_k(g), cp_v(g), cp_wo(g), cp_wmb(g), cp_x1(g)):
                d.wait()
            never = flag[0] > 0
            ga = sub_bc(modp[0])

            def q_of(j):
                return (qacc[g, :, j * DH:(j + 1) * DH] * QSCALE).astype(bf16)

            mv = [functools.partial(modb_piece, g, n) for n in range(NK)]
            os_ = []
            prl = qk(q_of(0), g)
            for j in range(REP):
                if j + 1 < REP:
                    nxt = qk(q_of(j + 1), g)
                else:
                    oproj(os_[:REP // 2], g, 0, acc_add, mv[:6], 2, never)
                os_.append(pv(prl, g))
                prl = nxt
            pieces = [functools.partial(ln1_piece, _mult(g, XQ, T0 + i * PR), 0,
                                        _mult(g, XQ // 2, i * PR // 2, 8)) for i in range(XQ // PR)]
            fin = [None] * NK

            def acc_fin(n, cs, a):
                fin[n] = acc_ref[:, cs] + a
                acc_ref[:, cs] = fin[n]

            oproj(os_[REP // 2:], g, REP // 2, acc_fin, pieces + mv[6:], 2, never)
            write_x1(0, x0b[...], jnp.concatenate(fin, axis=-1), ga)
            return c

        lax.fori_loop(0, HKV, group0, 0)

        cp_wr.wait()
        cp_xr.wait()
        wr8 = jnp.broadcast_to(wrb[...].astype(f32).reshape(1, D), (8, D))
        sb8 = sub_bc(modp[1])
        cb8 = _rb(1.0 + sub_bc(modp[2]))
        modb[M_GA] = sub_bc(modp[0])
        modb[M_SB] = sb8
        modb[M_CB1] = cb8
        modb[M_GB] = sub_bc(modp[3])
        modb[M_AW] = cb8 * wr8
        modb[M_C0] = jnp.broadcast_to(jnp.sum(sb8 * wr8, axis=-1, keepdims=True), (8, D))

        def body(t, carry):
            never = flag[0] > 0
            slot = t % 2
            r0 = _mult(t, TM, T0)
            re = _mult(t, TE)
            rn = _mult(jnp.minimum(t + 1, NM - 1), TM, T0)
            best = list(carry)
            pe = [functools.partial(epi_piece, re + i * PR, best) for i in range(TE // PR)]
            pn = [functools.partial(ln1_piece, rn + i * PR, 1 - slot, i * PR // 2) for i in range(TM // PR)]
            pieces = [p for pair in zip(pe, pn) for p in pair] + pe[len(pn):]
            npg = -(-len(pieces) // (HKV - 1))
            hh = pltpu.bitcast(hb[slot, 0:TM // 2, :], bf16)
            fin = [None] * NK

            def qproj(h):
                return (_dot(hh, wq[:, h * DH:(h + 1) * DH]) * QSCALE).astype(bf16)

            def acc_fin(n, cs, a):
                fin[n] = acc_ref[0:TM, cs] + a

            q = qproj(0)
            for g in range(HKV):
                os_ = []
                for j in range(REP):
                    prl = qk(q, g)
                    if g * REP + j + 1 < HQ:
                        q = qproj(g * REP + j + 1)
                    else:
                        oproj(os_[:REP // 2], g, 0, acc_add, [], 0, never)
                    os_.append(pv(prl, g))
                if g + 1 < HKV:
                    oproj(os_, g, 0, acc_set if g == 0 else acc_add, pieces[g * npg:(g + 1) * npg], 2, never)
                else:
                    oproj(os_[REP // 2:], g, REP // 2, acc_fin, [], 0, never)
            write_x1(r0, xb[pl.ds(r0, TM), :], jnp.concatenate(fin, axis=-1), modb[M_GA])
            cp_out(t).start()
            return tuple(best)

        init = (jnp.full((8, 128), -jnp.inf, f32), jnp.zeros((8, 128), i32))
        best = list(lax.fori_loop(0, NM, body, init))

        for c in cp_wg + cp_wu + [cp_wd]:
            c.wait()
        rl = NM * TE
        for i in range(TL // PR):
            route_piece(rl + i * PR, best, load_x1(rl + i * PR))

        bv, bi = best
        rmax = jnp.max(bv, axis=0, keepdims=True)
        imin = jnp.min(jnp.where(bv == rmax, bi, S), axis=0, keepdims=True)
        idx = jnp.minimum(imin[0, 0], S - 1)
        gate = jnp.concatenate([_rb(1.0 / (1.0 + jnp.exp(-rmax)))] * NK, axis=-1)
        s0 = pl.multiple_of(lax.shift_right_logical(idx, 4) * PR, PR)
        x1s = load_x1(s0)
        mbs, rinvs = load_stats(s0)
        h2s = h2_of(x1s - mbs, rinvs)
        lhs32 = pack_rows(h2s.reshape(PR, D))

        def mlp(jj, y):
            never = flag[0] > 0
            r0 = _mult(jj, OH, rl)
            pend, due, done, act = [], {}, 0, []
            for j in range(2 * (FC // FCH)):
                toks = due.pop(j, [])
                l32 = jnp.concatenate(
                    [jnp.where(never, tok, lhs32[:, k * 128:(k + 1) * 128]) for k, tok in enumerate(toks)]
                    + [lhs32[:, len(toks) * 128:]], axis=-1)
                wref = wu if j % 2 else wg
                res = _dot(pltpu.bitcast(l32, bf16), wref[jj, :, (j // 2) * FCH:(j // 2 + 1) * FCH])
                if done < OH // PR:
                    due.setdefault(j + OGAP, []).append(out_piece(r0 + done * PR, res[:, 0:128], never))
                    done += 1
                    if done == OH // PR:
                        cp_outl(jj).start()
                if j % 2:
                    act.append((pend.pop() * _rb(res)).astype(bf16))
                else:
                    pend.append(_rb(_silu(_rb(res))))
            assert done == OH // PR and not due
            return y + _dot(jnp.concatenate(act, axis=-1), wd[pl.ds(_mult(jj, FC), FC), 0:D])

        y = _rb(lax.fori_loop(0, NMLP, mlp, jnp.zeros((PR, D), f32)))
        y = _rb(y * gate)
        rows = lax.broadcasted_iota(i32, (PR, D), 0) + s0
        upd = jnp.where(rows == idx, y, 0.0).reshape(PR // 8, 8, D)
        fix[...] = (x1s + modb[M_GB][None] * (h2s + upd)).reshape(PR, D).astype(bf16)
        for t in range(NM):
            cp_out(t).wait()
        for j in range(NMLP):
            cp_outl(j).wait()
        cp_fix = pltpu.make_async_copy(fix, out_hbm.at[0, pl.ds(s0, PR)], sem_out.at[NM + NMLP])
        cp_fix.start()
        cp_fix.wait()

    scratch = [
        pltpu.VMEM((S, D), bf16),
        pltpu.VMEM((T0, D), bf16),
        pltpu.VMEM((S, D), bf16),
        pltpu.VMEM((2, HKV * XQ // 2, D), u32),
        pltpu.VMEM((HKV, W, DH), bf16),
        pltpu.VMEM((HKV, W, DH), bf16),
        pltpu.VMEM((D, HQ * DH + PAD), bf16),
        pltpu.VMEM((HKV, GD, D + PAD), bf16),
        pltpu.VMEM((NMLP, D, FC + PAD), bf16),
        pltpu.VMEM((NMLP, D, FC + PAD), bf16),
        pltpu.VMEM((F, D + PAD), bf16),
        pltpu.VMEM((NK, 2, D, 128), bf16),
        pltpu.VMEM((HKV, D, D + PAD), bf16),
        pltpu.VMEM((1, D), bf16),
        pltpu.VMEM((D,), bf16),
        pltpu.VMEM((D, 128), f32),
        pltpu.VMEM((NK, 2, 8, 128), f32),
        pltpu.VMEM((HKV, 8, D), f32),
        pltpu.VMEM((8, 8, D), f32),
        pltpu.VMEM((S, 256), f32),
        pltpu.VMEM((T0, D), f32),
        pltpu.VMEM((HKV, T0, GD), f32),
        pltpu.VMEM((NK, T0, 128), f32),
        pltpu.VMEM((PR, D), bf16),
        pltpu.SMEM((1,), i32),
        pltpu.SemaphoreType.DMA((n_in_sems,)),
        pltpu.SemaphoreType.DMA((NM + NMLP + 1,)),
    ]
    return kernel, scratch


@jax.jit
def pallas_adaLN_cond__sliding_block_cached__moe_arch_mod__prompt_kernel(
    A_x: jax.Array,
    A_k_cache: jax.Array,
    A_v_cache: jax.Array,
    A_wq: jax.Array,
    A_wo: jax.Array,
    B_x: jax.Array,
    B_w_r: jax.Array,
    B_w_gate: jax.Array,
    B_w_up: jax.Array,
    B_w_down: jax.Array,
    c: jax.Array,
    w_mod: jax.Array,
):
    B, S, D = A_x.shape
    _, HKV, SK, dh = A_k_cache.shape
    F = B_w_gate.shape[1]
    W = min(4096, max(256, SK // 4))
    assert B == 1 and dh == DH and A_wq.shape == (D, HQ * DH)
    kernel, scratch = _make_kernel(S, D, HKV, SK, W, F)
    any_spec = pl.BlockSpec(memory_space=pl.ANY)
    return pl.pallas_call(
        kernel,
        out_shape=jax.ShapeDtypeStruct((B, S, D), A_x.dtype),
        in_specs=[any_spec] * 11,
        out_specs=any_spec,
        scratch_shapes=scratch,
        compiler_params=pltpu.CompilerParams(vmem_limit_bytes=120 * 1024 * 1024,
                                             disable_semaphore_checks=True, disable_bounds_checks=True),
    )(A_x, A_k_cache, A_v_cache, A_wq, A_wo, B_w_r, B_w_gate, B_w_up, B_w_down, c, w_mod)
```

```python
import functools

import jax
import jax.numpy as jnp
from jax import lax
import jax.experimental.pallas as pl
import jax.experimental.pallas.tpu as pltpu

f32 = jnp.float32
bf16 = jnp.bfloat16
u32 = jnp.uint32
i32 = jnp.int32

HQ = 32
DH = 128
T0 = 480
TM = 224
TE = 256
L0 = 96
PR = 16
EPS = 1e-05
LOG2E = 1.4426950408889634
PAD = 128
NMLP = 2
FCH = 256
OGAP = 3
M_SA, M_CA1, M_GA, M_SB, M_CB1, M_GB, M_AW, M_C0 = range(8)


def _rb(x):
    return x.astype(bf16).astype(f32)


def _silu(x):
    return x * (1.0 / (1.0 + jnp.exp(-x)))


def _dot(a, b):
    return jnp.dot(a, b, preferred_element_type=f32)


def _mult(i, n, base=0, align=16):
    return base + i * n if isinstance(i, int) else pl.multiple_of(base + i * n, align)


def _make_kernel(S, D, HKV, SK, W, F):
    NM = (S - T0) // TM
    NK = D // 128
    REP = HQ // HKV
    GD = REP * DH
    QSCALE = DH ** (-0.5) * LOG2E
    XQ = 64
    TL = S - NM * TE
    FC = F // NMLP
    OH = TL // NMLP
    assert T0 + NM * TM == S and HKV * XQ >= TM and T0 % L0 == 0 and HKV == 4
    assert all(T0 + t * TM >= (t + 1) * TE for t in range(NM)) and OH % PR == 0

    sem_base, n_in_sems = {}, 0
    for name, n in (("c", 1), ("wr", 1), ("x0", 1), ("x1", HKV), ("xr", 1), ("wma", 2 * NK), ("wq", NK),
                    ("k", HKV), ("v", HKV), ("wo", HKV), ("wmb", HKV), ("wg", NMLP), ("wu", NMLP), ("wd", 1)):
        sem_base[name] = n_in_sems
        n_in_sems += n

    def kernel(x_hbm, k_hbm, v_hbm, wq_hbm, wo_hbm, wr_hbm, wg_hbm, wu_hbm, wd_hbm, c_hbm, wm_hbm,
               out_hbm,
               xb, x0b, ob, hb, kb, vb, wq, wo, wg, wu, wd, wma, wmb, cb, wrb, colb, moda, modp, modb,
               st_ref, acc_ref, qacc, xn_ref, fix, flag, sem_in, sem_out):
        def cp(name, i, src, dst):
            return pltpu.make_async_copy(src, dst, sem_in.at[sem_base[name] + i])

        def cp_x1(g):
            r = pl.ds(_mult(g, XQ, T0), XQ)
            return cp("x1", g, x_hbm.at[0, r], xb.at[r])

        def cp_wma(i, j):
            return cp("wma", 2 * i + j, wm_hbm.at[:, pl.ds(_mult(i, 128, j * D, 128), 128)], wma.at[i, j])

        def cp_wmb(j):
            return cp("wmb", j, wm_hbm.at[:, pl.ds(_mult(j, D, 2 * D, 128), D)], wmb.at[j, :, pl.ds(0, D)])

        def cp_wq(i):
            r = pl.ds(_mult(i, 128), 128)
            return cp("wq", i, wq_hbm.at[r], wq.at[r, pl.ds(0, HQ * DH)])

        def cp_k(g):
            return cp("k", g, k_hbm.at[0, g, pl.ds(SK - W, W)], kb.at[g])

        def cp_v(g):
            return cp("v", g, v_hbm.at[0, g, pl.ds(SK - W, W)], vb.at[g])

        def cp_wo(g):
            return cp("wo", g, wo_hbm.at[pl.ds(_mult(g, GD), GD)], wo.at[g, :, pl.ds(0, D)])

        xr0 = T0 + HKV * XQ
        cp_c = cp("c", 0, c_hbm, cb)
        cp_wr = cp("wr", 0, wr_hbm, wrb)
        cp_x0 = cp("x0", 0, x_hbm.at[0, pl.ds(0, T0)], x0b)
        cp_xr = cp("xr", 0, x_hbm.at[0, pl.ds(xr0, S - xr0)], xb.at[pl.ds(xr0, S - xr0)])
        cp_wg = [cp("wg", j, wg_hbm.at[:, pl.ds(j * FC, FC)], wg.at[j, :, pl.ds(0, FC)]) for j in range(NMLP)]
        cp_wu = [cp("wu", j, wu_hbm.at[:, pl.ds(j * FC, FC)], wu.at[j, :, pl.ds(0, FC)]) for j in range(NMLP)]
        cp_wd = cp("wd", 0, wd_hbm, wd.at[:, pl.ds(0, D)])

        def cp_out(t):
            r = pl.ds(_mult(t, TE), TE)
            return pltpu.make_async_copy(ob.at[r], out_hbm.at[0, r], sem_out.at[t])

        def cp_outl(j):
            r = pl.ds(_mult(j, OH, NM * TE), OH)
            return pltpu.make_async_copy(ob.at[r], out_hbm.at[0, r], sem_out.at[NM + j])

        order = [cp_c, cp_x0, cp_wma(0, 0), cp_wma(0, 1)]
        for i in range(NK):
            order += [cp_wq(i)]
            if i + 1 < NK:
                order += [cp_wma(i + 1, 0), cp_wma(i + 1, 1)]
        for g in range(HKV):
            order += [cp_k(g), cp_v(g), cp_wo(g), cp_wmb(g), cp_x1(g)]
        order += [cp_wr, cp_xr] + cp_wg + cp_wu + [cp_wd]
        assert len(order) == n_in_sems
        for c in order:
            c.start()

        flag[0] = 0

        def tie(x, tok, never):
            if tok is None:
                return x
            return jnp.concatenate([jnp.where(never, tok, x[:, :128]), x[:, 128:]], axis=-1)

        def due_rows(lhs, toks, never):
            if not toks:
                return lhs
            parts = [jnp.where(never, tok, lhs[8 * k:8 * k + 8]) for k, tok in enumerate(toks)]
            return jnp.concatenate(parts + [lhs[8 * len(toks):]], axis=0)

        def ln_plain(x):
            m = jnp.sum(x, axis=-1, keepdims=True) * (1.0 / D)
            xc = x - m
            v = jnp.sum(xc * xc, axis=-1, keepdims=True) * (1.0 / D)
            return xc * lax.rsqrt(v + EPS)

        def lane_bc(v):
            return jnp.broadcast_to(v.reshape(-1, 1), (v.shape[0] * 8, 128))

        def sub_bc(p):
            return jnp.broadcast_to(_rb(jnp.sum(p, axis=0, keepdims=True)), p.shape)

        def h2_of(xc, rinv):
            return (xc * rinv) * modb[M_CB1][None] + modb[M_SB][None]

        def load_stats(row):
            st = st_ref[pl.ds(row, PR), :]
            mb = jnp.concatenate([st[:, 0:128]] * NK, axis=-1).reshape(PR // 8, 8, D)
            rinv = jnp.concatenate([st[:, 128:256]] * NK, axis=-1).reshape(PR // 8, 8, D)
            return mb, rinv

        def tok_of(v):
            return v[0:8] + v[8:16]

        def ln1_piece(xrow, slot, hrow, tok=None, never=None):
            x = tie(xb[pl.ds(xrow, PR), :].astype(f32), tok, never).reshape(PR // 8, 8, D)
            h = (ln_plain(x) * modb[M_CA1][None] + modb[M_SA][None]).reshape(PR, D)
            hb[slot, pl.ds(hrow, PR // 2), :] = pltpu.bitcast(h.astype(bf16), u32)
            return tok_of(h[:, 0:128])

        sub_iota = lax.broadcasted_iota(i32, (8, 128), 0)

        def route_piece(row, best, x1):
            m = jnp.sum(x1, axis=-1, keepdims=True) * (1.0 / D)
            mb = _rb(m)
            xc = x1 - mb
            dm = m - mb
            v = jnp.sum(xc * xc, axis=-1, keepdims=True) * (1.0 / D) - dm * dm
            rs = jnp.sum(xc * modb[M_AW][None], axis=-1, keepdims=True)
            sd = _rb(jnp.sqrt(_rb(_rb(jnp.maximum(v, 0.0)) + EPS)))
            r0 = pl.reciprocal(sd, approx=True)
            rinv = r0 * (2.0 - sd * r0)
            st_ref[pl.ds(row, PR), :] = jnp.concatenate([lane_bc(mb), lane_bc(rinv)], axis=-1)
            rr = lane_bc(rs * rinv).reshape(PR // 8, 8, 128) + modb[M_C0, :, 0:128][None]
            rbf = _rb(rr.reshape(PR, 128))
            for j in range(PR // 8):
                rj = rbf[8 * j:8 * j + 8]
                upd = rj > best[0]
                best[1] = jnp.where(upd, sub_iota + (row + 8 * j), best[1])
                best[0] = jnp.where(upd, rj, best[0])
            return xc, rinv, rbf

        def load_x1(row, tok=None, never=None):
            return tie(xb[pl.ds(row, PR), :].astype(f32), tok, never).reshape(PR // 8, 8, D)

        def epi_piece(row, best, tok=None, never=None):
            x1 = load_x1(row, tok, never)
            xc, rinv, rbf = route_piece(row, best, x1)
            ob[pl.ds(row, PR), :] = (x1 + modb[M_GB][None] * h2_of(xc, rinv)).reshape(PR, D).astype(bf16)
            return tok_of(rbf)

        def out_piece(row, tok, never):
            x1 = load_x1(row)
            mb, rinv = load_stats(row)
            mb = jnp.where(never, jnp.concatenate([tok] * NK, axis=-1).reshape(PR // 8, 8, D), mb)
            o = (x1 + modb[M_GB][None] * h2_of(x1 - mb, rinv)).reshape(PR, D)
            ob[pl.ds(row, PR), :] = o.astype(bf16)
            return o[:, 0:128]

        def matvec(w_at, tok, never):
            y = None if tok is None else jnp.where(never, tok[0:8], 0.0)
            for kg in range(D // 8):
                t = w_at(slice(kg * 8, (kg + 1) * 8)).astype(f32) * colb[kg * 8:(kg + 1) * 8, :]
                y = t if y is None else y + t
            return y

        def moda_piece(i, j, tok=None, never=None):
            y = sub_bc(matvec(lambda r: wma[i, j, r, :], tok, never))
            if j == 1:
                y = _rb(1.0 + y)
            moda[i, j] = y
            return y

        def modb_piece(ch, n, tok=None, never=None):
            y = matvec(lambda r: wmb[ch, r, n * 128:(n + 1) * 128], tok, never)
            modp[ch, :, n * 128:(n + 1) * 128] = y
            return y

        def qk(q, g):
            s = lax.dot_general(q, kb[g], (((1,), (1,)), ((), ())), preferred_element_type=f32)
            m = jnp.max(s, axis=-1, keepdims=True)
            p = jnp.exp2(s - m)
            l = jnp.sum(p, axis=-1, keepdims=True)
            rl = pl.reciprocal(l, approx=True)
            return p, rl * (2.0 - l * rl)

        def pv(prl, g, prev=None, never=None):
            p, rl = prl
            if prev is not None:
                p = jnp.concatenate([jnp.where(never, prev, p[:, 0:DH]), p[:, DH:]], axis=-1)
            return _dot(p.astype(bf16), vb[g]) * rl

        def paced(nsteps, step, pieces, gap, never):
            outs, done = {}, 0
            for n in range(nsteps):
                a = step(n, outs.pop(n, []))
                if n < nsteps - gap:
                    cnt = int(round((n + 1) * len(pieces) / (nsteps - gap))) - done
                    for k in range(cnt):
                        rr = (k * a.shape[0] // cnt) // PR * PR
                        outs.setdefault(n + gap, []).append(pieces[done](a[rr:rr + PR, 0:128], never))
                        done += 1
            assert done == len(pieces)

        def oproj(os_, g, j0, sink, pieces, gap, never):
            def step(n, toks):
                cs = slice(n * 128, (n + 1) * 128)
                og = jnp.concatenate([due_rows(os_[0], toks, never)] + list(os_[1:]), axis=-1)
                a = _dot(og.astype(bf16), wo[g, j0 * DH:(j0 + len(os_)) * DH, cs])
                sink(n, cs, a)
                return a
            paced(NK, step, pieces, gap, never)

        def acc_set(n, cs, a):
            acc_ref[0:a.shape[0], cs] = a

        def acc_add(n, cs, a):
            acc_ref[0:a.shape[0], cs] += a

        def write_x1(r0, x, acc, ga):
            rows = x.shape[0]
            a = acc.reshape(rows // 8, 8, D) * ga[None]
            xb[pl.ds(r0, rows), :] = (x.astype(f32) + a.reshape(rows, D)).astype(bf16)

        def zero(i, c):
            r = pl.ds(_mult(i, PR), PR)
            for g in range(HKV):
                qacc[g, r, :] = jnp.zeros((PR, GD), f32)
            acc_ref[r, :] = jnp.zeros((PR, D), f32)
            return c

        lax.fori_loop(0, T0 // PR, zero, 0)
        modp[0] = jnp.zeros((8, D), f32)
        cp_c.wait()
        sc = _rb(_silu(cb[...].astype(f32)))
        colb[...] = jnp.broadcast_to(sc, (128, D)).T
        cp_x0.wait()

        def ln0(i, c):
            r = pl.ds(_mult(i, L0), L0)
            xn = ln_plain(x0b[r, :].astype(f32))
            for n in range(NK):
                xn_ref[n, r, :] = xn[:, n * 128:(n + 1) * 128]
            return c

        lax.fori_loop(0, T0 // L0, ln0, 0)

        def kstep(i, c):
            @pl.when(i <= 1)
            def _():
                cp_wma(i, 0).wait()
                cp_wma(i, 1).wait()
                moda_piece(i, 0)
                moda_piece(i, 1)

            cp_wq(i).wait()
            ahead = jnp.logical_and(i >= 1, i + 1 < NK)

            @pl.when(ahead)
            def _():
                cp_wma(i + 1, 0).wait()
                cp_wma(i + 1, 1).wait()

            never = flag[0] > 0
            h = (xn_ref[i].reshape(T0 // 8, 8, 128) * moda[i, 1][None] + moda[i, 0][None])
            h = h.reshape(T0, 128)
            nxt = jnp.where(ahead, i + 1, i)
            r = pl.ds(_mult(i, 128), 128)
            nw = 4 * DH

            def step(n, toks):
                a = _dot(due_rows(h, toks, never).astype(bf16), wq[r, n * nw:(n + 1) * nw])
                g, c0 = divmod(n * nw, GD)
                qacc[g, :, c0:c0 + nw] += a
                return a

            paced(HQ * DH // nw, step, [functools.partial(moda_piece, nxt, j) for j in range(2)], 4, never)
            return c

        lax.fori_loop(0, NK, kstep, 0)
        modb[M_SA] = jnp.concatenate([moda[i, 0] for i in range(NK)], axis=-1)
        modb[M_CA1] = jnp.concatenate([moda[i, 1] for i in range(NK)], axis=-1)

        def group0(g, c):
            for d in (cp_k(g), cp_v(g), cp_wo(g), cp_wmb(g), cp_x1(g)):
                d.wait()
            never = flag[0] > 0
            ga = sub_bc(modp[0])

            def q_of(j):
                return (qacc[g, :, j * DH:(j + 1) * DH] * QSCALE).astype(bf16)

            mv = [functools.partial(modb_piece, g, n) for n in range(NK)]
            os_ = []
            prl = qk(q_of(0), g)
            for j in range(REP):
                if j + 1 < REP:
                    nxt = qk(q_of(j + 1), g)
                else:
                    oproj(os_[:REP // 2], g, 0, acc_add, mv[:6], 2, never)
                os_.append(pv(prl, g, os_[-1] if os_ else None, never))
                prl = nxt
            pieces = [functools.partial(ln1_piece, _mult(g, XQ, T0 + i * PR), 0,
                                        _mult(g, XQ // 2, i * PR // 2, 8)) for i in range(XQ // PR)]
            fin = [None] * NK

            def acc_fin(n, cs, a):
                fin[n] = acc_ref[:, cs] + a
                acc_ref[:, cs] = fin[n]

            oproj(os_[REP // 2:], g, REP // 2, acc_fin, pieces + mv[6:], 2, never)
            write_x1(0, x0b[...], jnp.concatenate(fin, axis=-1), ga)
            return c

        lax.fori_loop(0, HKV, group0, 0)

        cp_wr.wait()
        cp_xr.wait()
        wr8 = jnp.broadcast_to(wrb[...].astype(f32).reshape(1, D), (8, D))
        sb8 = sub_bc(modp[1])
        cb8 = _rb(1.0 + sub_bc(modp[2]))
        modb[M_GA] = sub_bc(modp[0])
        modb[M_SB] = sb8
        modb[M_CB1] = cb8
        modb[M_GB] = sub_bc(modp[3])
        modb[M_AW] = cb8 * wr8
        modb[M_C0] = jnp.broadcast_to(jnp.sum(sb8 * wr8, axis=-1, keepdims=True), (8, D))

        def body(t, carry):
            never = flag[0] > 0
            slot = t % 2
            r0 = _mult(t, TM, T0)
            re = _mult(t, TE)
            rn = _mult(jnp.minimum(t + 1, NM - 1), TM, T0)
            best = list(carry)
            pe = [functools.partial(epi_piece, re + i * PR, best) for i in range(TE // PR)]
            pn = [functools.partial(ln1_piece, rn + i * PR, 1 - slot, i * PR // 2) for i in range(TM // PR)]
            pieces = [p for pair in zip(pe, pn) for p in pair] + pe[len(pn):]
            npg = -(-len(pieces) // (HKV - 1))
            hh = pltpu.bitcast(hb[slot, 0:TM // 2, :], bf16)
            fin = [None] * NK

            def qproj(h):
                return (_dot(hh, wq[:, h * DH:(h + 1) * DH]) * QSCALE).astype(bf16)

            def acc_fin(n, cs, a):
                fin[n] = acc_ref[0:TM, cs] + a

            q = qproj(0)
            for g in range(HKV):
                os_ = []
                for j in range(REP):
                    prl = qk(q, g)
                    if g * REP + j + 1 < HQ:
                        q = qproj(g * REP + j + 1)
                    else:
                        oproj(os_[:REP // 2], g, 0, acc_add, [], 0, never)
                    os_.append(pv(prl, g, os_[-1] if os_ else None, never))
                if g + 1 < HKV:
                    oproj(os_, g, 0, acc_set if g == 0 else acc_add, pieces[g * npg:(g + 1) * npg], 3, never)
                else:
                    oproj(os_[REP // 2:], g, REP // 2, acc_fin, [], 0, never)
            write_x1(r0, xb[pl.ds(r0, TM), :], jnp.concatenate(fin, axis=-1), modb[M_GA])
            cp_out(t).start()
            return tuple(best)

        init = (jnp.full((8, 128), -jnp.inf, f32), jnp.zeros((8, 128), i32))
        best = list(lax.fori_loop(0, NM, body, init))

        for c in cp_wg + cp_wu + [cp_wd]:
            c.wait()
        rl = NM * TE
        for i in range(TL // PR):
            route_piece(rl + i * PR, best, load_x1(rl + i * PR))

        bv, bi = best
        rmax = jnp.max(bv, axis=0, keepdims=True)
        imin = jnp.min(jnp.where(bv == rmax, bi, S), axis=0, keepdims=True)
        idx = jnp.minimum(imin[0, 0], S - 1)
        gate = jnp.concatenate([_rb(1.0 / (1.0 + jnp.exp(-rmax)))] * NK, axis=-1)
        s0 = pl.multiple_of(lax.shift_right_logical(idx, 4) * PR, PR)
        x1s = load_x1(s0)
        mbs, rinvs = load_stats(s0)
        h2s = h2_of(x1s - mbs, rinvs)
        lhs = h2s.reshape(PR, D)

        def mlp(jj, y):
            never = flag[0] > 0
            r0 = _mult(jj, OH, rl)
            pend, due, done, act = [], {}, 0, []
            for j in range(2 * (FC // FCH)):
                toks = due.pop(j, [])
                lj = jnp.concatenate(
                    [jnp.where(never, tok, lhs[:, k * 128:(k + 1) * 128]) for k, tok in enumerate(toks)]
                    + [lhs[:, len(toks) * 128:]], axis=-1)
                wref = wu if j % 2 else wg
                res = _dot(lj.astype(bf16), wref[jj, :, (j // 2) * FCH:(j // 2 + 1) * FCH])
                if done < OH // PR:
                    due.setdefault(j + OGAP, []).append(out_piece(r0 + done * PR, res[:, 0:128], never))
                    done += 1
                    if done == OH // PR:
                        cp_outl(jj).start()
                if j % 2:
                    act.append(pend.pop() * _rb(res))
                else:
                    pend.append(_rb(_silu(_rb(res))))
            assert done == OH // PR and not due
            return y + _dot(jnp.concatenate(act, axis=-1).astype(bf16), wd[pl.ds(_mult(jj, FC), FC), 0:D])

        y = _rb(lax.fori_loop(0, NMLP, mlp, jnp.zeros((PR, D), f32)))
        y = _rb(y * gate)
        rows = lax.broadcasted_iota(i32, (PR, D), 0) + s0
        upd = jnp.where(rows == idx, y, 0.0).reshape(PR // 8, 8, D)
        fix[...] = (x1s + modb[M_GB][None] * (h2s + upd)).reshape(PR, D).astype(bf16)
        for t in range(NM):
            cp_out(t).wait()
        for j in range(NMLP):
            cp_outl(j).wait()
        cp_fix = pltpu.make_async_copy(fix, out_hbm.at[0, pl.ds(s0, PR)], sem_out.at[NM + NMLP])
        cp_fix.start()
        cp_fix.wait()

    scratch = [
        pltpu.VMEM((S, D), bf16),
        pltpu.VMEM((T0, D), bf16),
        pltpu.VMEM((S, D), bf16),
        pltpu.VMEM((2, HKV * XQ // 2, D), u32),
        pltpu.VMEM((HKV, W, DH), bf16),
        pltpu.VMEM((HKV, W, DH), bf16),
        pltpu.VMEM((D, HQ * DH + PAD), bf16),
        pltpu.VMEM((HKV, GD, D + PAD), bf16),
        pltpu.VMEM((NMLP, D, FC + PAD), bf16),
        pltpu.VMEM((NMLP, D, FC + PAD), bf16),
        pltpu.VMEM((F, D + PAD), bf16),
        pltpu.VMEM((NK, 2, D, 128), bf16),
        pltpu.VMEM((HKV, D, D + PAD), bf16),
        pltpu.VMEM((1, D), bf16),
        pltpu.VMEM((D,), bf16),
        pltpu.VMEM((D, 128), f32),
        pltpu.VMEM((NK, 2, 8, 128), f32),
        pltpu.VMEM((HKV, 8, D), f32),
        pltpu.VMEM((8, 8, D), f32),
        pltpu.VMEM((S, 256), f32),
        pltpu.VMEM((T0, D), f32),
        pltpu.VMEM((HKV, T0, GD), f32),
        pltpu.VMEM((NK, T0, 128), f32),
        pltpu.VMEM((PR, D), bf16),
        pltpu.SMEM((1,), i32),
        pltpu.SemaphoreType.DMA((n_in_sems,)),
        pltpu.SemaphoreType.DMA((NM + NMLP + 1,)),
    ]
    return kernel, scratch


@jax.jit
def pallas_adaLN_cond__sliding_block_cached__moe_arch_mod__prompt_kernel(
    A_x: jax.Array,
    A_k_cache: jax.Array,
    A_v_cache: jax.Array,
    A_wq: jax.Array,
    A_wo: jax.Array,
    B_x: jax.Array,
    B_w_r: jax.Array,
    B_w_gate: jax.Array,
    B_w_up: jax.Array,
    B_w_down: jax.Array,
    c: jax.Array,
    w_mod: jax.Array,
):
    B, S, D = A_x.shape
    _, HKV, SK, dh = A_k_cache.shape
    F = B_w_gate.shape[1]
    W = min(4096, max(256, SK // 4))
    assert B == 1 and dh == DH and A_wq.shape == (D, HQ * DH)
    kernel, scratch = _make_kernel(S, D, HKV, SK, W, F)
    any_spec = pl.BlockSpec(memory_space=pl.ANY)
    return pl.pallas_call(
        kernel,
        out_shape=jax.ShapeDtypeStruct((B, S, D), A_x.dtype),
        in_specs=[any_spec] * 11,
        out_specs=any_spec,
        scratch_shapes=scratch,
        compiler_params=pltpu.CompilerParams(vmem_limit_bytes=120 * 1024 * 1024,
                                             disable_semaphore_checks=True, disable_bounds_checks=True),
    )(A_x, A_k_cache, A_v_cache, A_wq, A_wo, B_w_r, B_w_gate, B_w_up, B_w_down, c, w_mod)
```

```python
import functools

import jax
import jax.numpy as jnp
from jax import lax
import jax.experimental.pallas as pl
import jax.experimental.pallas.tpu as pltpu

f32 = jnp.float32
bf16 = jnp.bfloat16
u32 = jnp.uint32
i32 = jnp.int32

HQ = 32
DH = 128
T0 = 480
TM = 224
TE = 256
L0 = 96
PR = 16
EPS = 1e-05
LOG2E = 1.4426950408889634
PAD = 128
NMLP = 2
FCH = 256
OGAP = 3
M_SA, M_CA1, M_CB1, M_AW, M_C0 = range(5)
R_GA, R_SB, R_CB, R_GB = range(4)


def _rb(x):
    return x.astype(bf16).astype(f32)


def _silu(x):
    return x * (1.0 / (1.0 + jnp.exp(-x)))


def _dot(a, b):
    return jnp.dot(a, b, preferred_element_type=f32)


def _mult(i, n, base=0, align=16):
    return base + i * n if isinstance(i, int) else pl.multiple_of(base + i * n, align)


def _make_kernel(S, D, HKV, SK, W, F):
    NM = (S - T0) // TM
    NK = D // 128
    REP = HQ // HKV
    GD = REP * DH
    QSCALE = DH ** (-0.5) * LOG2E
    XQ = 64
    TL = S - NM * TE
    FC = F // NMLP
    OH = TL // NMLP
    assert T0 + NM * TM == S and HKV * XQ >= TM and T0 % L0 == 0 and HKV == 4
    assert all(T0 + t * TM >= (t + 1) * TE for t in range(NM)) and OH % PR == 0

    sem_base, n_in_sems = {}, 0
    for name, n in (("c", 1), ("wr", 1), ("x0", 1), ("x1", HKV), ("xr", 1), ("wma", 2 * NK), ("wq", NK),
                    ("k", HKV), ("v", HKV), ("wo", HKV), ("wmb", HKV), ("wg", NMLP), ("wu", NMLP), ("wd", 1)):
        sem_base[name] = n_in_sems
        n_in_sems += n

    def kernel(x_hbm, k_hbm, v_hbm, wq_hbm, wo_hbm, wr_hbm, wg_hbm, wu_hbm, wd_hbm, c_hbm, wm_hbm,
               out_hbm,
               xb, x0b, ob, hb, kb, vb, wq, wo, wg, wu, wd, wma, wmb, cb, wrb, colb, moda, modr, modb,
               st_ref, acc_ref, qacc, xn_ref, fix, flag, sem_in, sem_out):
        def cp(name, i, src, dst):
            return pltpu.make_async_copy(src, dst, sem_in.at[sem_base[name] + i])

        def cp_x1(g):
            r = pl.ds(_mult(g, XQ, T0), XQ)
            return cp("x1", g, x_hbm.at[0, r], xb.at[r])

        def cp_wma(i, j):
            return cp("wma", 2 * i + j, wm_hbm.at[:, pl.ds(_mult(i, 128, j * D, 128), 128)], wma.at[i, j])

        def cp_wmb(j):
            return cp("wmb", j, wm_hbm.at[:, pl.ds(_mult(j, D, 2 * D, 128), D)], wmb.at[j, :, pl.ds(0, D)])

        def cp_wq(i):
            r = pl.ds(_mult(i, 128), 128)
            return cp("wq", i, wq_hbm.at[r], wq.at[r, pl.ds(0, HQ * DH)])

        def cp_k(g):
            return cp("k", g, k_hbm.at[0, g, pl.ds(SK - W, W)], kb.at[g])

        def cp_v(g):
            return cp("v", g, v_hbm.at[0, g, pl.ds(SK - W, W)], vb.at[g])

        def cp_wo(g):
            return cp("wo", g, wo_hbm.at[pl.ds(_mult(g, GD), GD)], wo.at[g, :, pl.ds(0, D)])

        xr0 = T0 + HKV * XQ
        cp_c = cp("c", 0, c_hbm, cb)
        cp_wr = cp("wr", 0, wr_hbm, wrb)
        cp_x0 = cp("x0", 0, x_hbm.at[0, pl.ds(0, T0)], x0b)
        cp_xr = cp("xr", 0, x_hbm.at[0, pl.ds(xr0, S - xr0)], xb.at[pl.ds(xr0, S - xr0)])
        cp_wg = [cp("wg", j, wg_hbm.at[:, pl.ds(j * FC, FC)], wg.at[j, :, pl.ds(0, FC)]) for j in range(NMLP)]
        cp_wu = [cp("wu", j, wu_hbm.at[:, pl.ds(j * FC, FC)], wu.at[j, :, pl.ds(0, FC)]) for j in range(NMLP)]
        cp_wd = cp("wd", 0, wd_hbm, wd.at[:, pl.ds(0, D)])

        def cp_out(t):
            r = pl.ds(_mult(t, TE), TE)
            return pltpu.make_async_copy(ob.at[r], out_hbm.at[0, r], sem_out.at[t])

        def cp_outl(j):
            r = pl.ds(_mult(j, OH, NM * TE), OH)
            return pltpu.make_async_copy(ob.at[r], out_hbm.at[0, r], sem_out.at[NM + j])

        order = [cp_c, cp_x0, cp_wma(0, 0), cp_wma(0, 1)]
        for i in range(NK):
            order += [cp_wq(i)]
            if i + 1 < NK:
                order += [cp_wma(i + 1, 0), cp_wma(i + 1, 1)]
        order += [cp_wr]
        for g in range(HKV):
            order += [cp_k(g), cp_v(g), cp_wo(g), cp_wmb(g), cp_x1(g)]
        order += [cp_xr] + cp_wg + cp_wu + [cp_wd]
        assert len(order) == n_in_sems
        for c in order:
            c.start()

        flag[0] = 0

        def tie(x, tok, never):
            if tok is None:
                return x
            return jnp.concatenate([jnp.where(never, tok, x[:, :128]), x[:, 128:]], axis=-1)

        def due_rows(lhs, toks, never):
            if not toks:
                return lhs
            parts = [jnp.where(never, tok, lhs[8 * k:8 * k + 8]) for k, tok in enumerate(toks)]
            return jnp.concatenate(parts + [lhs[8 * len(toks):]], axis=0)

        def ln_plain(x):
            m = jnp.sum(x, axis=-1, keepdims=True) * (1.0 / D)
            xc = x - m
            v = jnp.sum(xc * xc, axis=-1, keepdims=True) * (1.0 / D)
            return xc * lax.rsqrt(v + EPS)

        def lane_bc(v):
            return jnp.broadcast_to(v.reshape(-1, 1), (v.shape[0] * 8, 128))

        def sub_bc(p):
            return jnp.broadcast_to(_rb(jnp.sum(p, axis=0, keepdims=True)), p.shape)

        def h2_of(xc, rinv):
            return (xc * rinv) * modb[M_CB1][None] + modr[R_SB][None]

        def load_stats(row):
            st = st_ref[pl.ds(row, PR), :]
            mb = jnp.concatenate([st[:, 0:128]] * NK, axis=-1).reshape(PR // 8, 8, D)
            rinv = jnp.concatenate([st[:, 128:256]] * NK, axis=-1).reshape(PR // 8, 8, D)
            return mb, rinv

        def tok_of(v):
            return v[0:8] + v[8:16]

        def ln1_piece(xrow, slot, hrow, tok=None, never=None):
            x = tie(xb[pl.ds(xrow, PR), :].astype(f32), tok, never).reshape(PR // 8, 8, D)
            h = (ln_plain(x) * modb[M_CA1][None] + modb[M_SA][None]).reshape(PR, D)
            hb[slot, pl.ds(hrow, PR // 2), :] = pltpu.bitcast(h.astype(bf16), u32)
            return tok_of(h[:, 0:128])

        sub_iota = lax.broadcasted_iota(i32, (8, 128), 0)

        def route_piece(row, best, x1):
            m = jnp.sum(x1, axis=-1, keepdims=True) * (1.0 / D)
            mb = _rb(m)
            xc = x1 - mb
            dm = m - mb
            v = jnp.sum(xc * xc, axis=-1, keepdims=True) * (1.0 / D) - dm * dm
            rs = jnp.sum(xc * modb[M_AW][None], axis=-1, keepdims=True)
            sd = _rb(jnp.sqrt(_rb(_rb(jnp.maximum(v, 0.0)) + EPS)))
            r0 = pl.reciprocal(sd, approx=True)
            rinv = r0 * (2.0 - sd * r0)
            st_ref[pl.ds(row, PR), :] = jnp.concatenate([lane_bc(mb), lane_bc(rinv)], axis=-1)
            rr = lane_bc(rs * rinv).reshape(PR // 8, 8, 128) + modb[M_C0, :, 0:128][None]
            rbf = _rb(rr.reshape(PR, 128))
            for j in range(PR // 8):
                rj = rbf[8 * j:8 * j + 8]
                upd = rj > best[0]
                best[1] = jnp.where(upd, sub_iota + (row + 8 * j), best[1])
                best[0] = jnp.where(upd, rj, best[0])
            return xc, rinv, rbf

        def load_x1(row, tok=None, never=None):
            return tie(xb[pl.ds(row, PR), :].astype(f32), tok, never).reshape(PR // 8, 8, D)

        def epi_piece(row, best, tok=None, never=None):
            x1 = load_x1(row, tok, never)
            xc, rinv, rbf = route_piece(row, best, x1)
            ob[pl.ds(row, PR), :] = (x1 + modr[R_GB][None] * h2_of(xc, rinv)).reshape(PR, D).astype(bf16)
            return tok_of(rbf)

        def out_piece(row, tok, never):
            x1 = load_x1(row)
            mb, rinv = load_stats(row)
            mb = jnp.where(never, jnp.concatenate([tok] * NK, axis=-1).reshape(PR // 8, 8, D), mb)
            o = (x1 + modr[R_GB][None] * h2_of(x1 - mb, rinv)).reshape(PR, D)
            ob[pl.ds(row, PR), :] = o.astype(bf16)
            return o[:, 0:128]

        def matvec(w_at, tok, never):
            y = None if tok is None else jnp.where(never, tok[0:8], 0.0)
            for kg in range(D // 8):
                t = w_at(slice(kg * 8, (kg + 1) * 8)).astype(f32) * colb[kg * 8:(kg + 1) * 8, :]
                y = t if y is None else y + t
            return y

        def moda_piece(i, j, tok=None, never=None):
            y = sub_bc(matvec(lambda r: wma[i, j, r, :], tok, never))
            if j == 1:
                y = _rb(1.0 + y)
            moda[i, j] = y
            return y

        def modb_piece(ch, n, tok=None, never=None):
            y = sub_bc(matvec(lambda r: wmb[ch, r, n * 128:(n + 1) * 128], tok, never))
            modr[ch, :, n * 128:(n + 1) * 128] = y
            return y

        def qk(q, g):
            s = lax.dot_general(q, kb[g], (((1,), (1,)), ((), ())), preferred_element_type=f32)
            m = jnp.max(s, axis=-1, keepdims=True)
            p = jnp.exp2(s - m)
            l = jnp.sum(p, axis=-1, keepdims=True)
            rl = pl.reciprocal(l, approx=True)
            return p, rl * (2.0 - l * rl)

        def pv(prl, g, prev=None, never=None):
            p, rl = prl
            if prev is not None:
                p = jnp.concatenate([jnp.where(never, prev, p[:, 0:DH]), p[:, DH:]], axis=-1)
            return _dot(p.astype(bf16), vb[g]) * rl

        def paced(nsteps, step, pieces, gap, never):
            outs, done = {}, 0
            for n in range(nsteps):
                a = step(n, outs.pop(n, []))
                if n < nsteps - gap:
                    cnt = int(round((n + 1) * len(pieces) / (nsteps - gap))) - done
                    for k in range(cnt):
                        rr = (k * a.shape[0] // cnt) // PR * PR
                        outs.setdefault(n + gap, []).append(pieces[done](a[rr:rr + PR, 0:128], never))
                        done += 1
            assert done == len(pieces)

        def oproj(os_, g, j0, sink, pieces, gap, never):
            def step(n, toks):
                cs = slice(n * 128, (n + 1) * 128)
                og = jnp.concatenate([due_rows(os_[0], toks, never)] + list(os_[1:]), axis=-1)
                a = _dot(og.astype(bf16), wo[g, j0 * DH:(j0 + len(os_)) * DH, cs])
                sink(n, cs, a)
                return a
            paced(NK, step, pieces, gap, never)

        def acc_set(n, cs, a):
            acc_ref[0:a.shape[0], cs] = a

        def acc_add(n, cs, a):
            acc_ref[0:a.shape[0], cs] += a

        def write_x1(r0, x, acc, ga):
            rows = x.shape[0]
            a = acc.reshape(rows // 8, 8, D) * ga[None]
            xb[pl.ds(r0, rows), :] = (x.astype(f32) + a.reshape(rows, D)).astype(bf16)

        def zero(i, c):
            r = pl.ds(_mult(i, PR), PR)
            for g in range(HKV):
                qacc[g, r, :] = jnp.zeros((PR, GD), f32)
            acc_ref[r, :] = jnp.zeros((PR, D), f32)
            return c

        lax.fori_loop(0, T0 // PR, zero, 0)
        modr[...] = jnp.zeros((HKV, 8, D), f32)
        cp_c.wait()
        sc = _rb(_silu(cb[...].astype(f32)))
        colb[...] = jnp.broadcast_to(sc, (128, D)).T
        cp_x0.wait()

        def ln0(i, c):
            r = pl.ds(_mult(i, L0), L0)
            xn = ln_plain(x0b[r, :].astype(f32))
            for n in range(NK):
                xn_ref[n, r, :] = xn[:, n * 128:(n + 1) * 128]
            return c

        lax.fori_loop(0, T0 // L0, ln0, 0)

        def kstep(i, c):
            @pl.when(i <= 2)
            def _():
                cp_wma(i, 0).wait()
                cp_wma(i, 1).wait()
                moda_piece(i, 0)
                moda_piece(i, 1)

            cp_wq(i).wait()
            ahead = jnp.logical_and(i >= 2, i + 1 < NK)

            @pl.when(ahead)
            def _():
                cp_wma(i + 1, 0).wait()
                cp_wma(i + 1, 1).wait()

            never = flag[0] > 0
            h = (xn_ref[i].reshape(T0 // 8, 8, 128) * moda[i, 1][None] + moda[i, 0][None])
            h = h.reshape(T0, 128)
            nxt = jnp.where(ahead, i + 1, i)
            r = pl.ds(_mult(i, 128), 128)
            nw = 4 * DH

            def step(n, toks):
                a = _dot(due_rows(h, toks, never).astype(bf16), wq[r, n * nw:(n + 1) * nw])
                g, c0 = divmod(n * nw, GD)
                qacc[g, :, c0:c0 + nw] += a
                return a

            paced(HQ * DH // nw, step, [functools.partial(moda_piece, nxt, j) for j in range(2)], 4, never)
            return c

        lax.fori_loop(0, NK, kstep, 0)
        cp_wr.wait()
        modb[M_SA] = jnp.concatenate([moda[i, 0] for i in range(NK)], axis=-1)
        modb[M_CA1] = jnp.concatenate([moda[i, 1] for i in range(NK)], axis=-1)

        def group0(g, c):
            for d in (cp_k(g), cp_v(g), cp_wo(g), cp_wmb(g), cp_x1(g)):
                d.wait()

            @pl.when(g == HKV - 1)
            def _():
                cp_xr.wait()

            never = flag[0] > 0
            ga = modr[R_GA]
            wr8 = jnp.broadcast_to(wrb[...].astype(f32).reshape(1, D), (8, D))
            cb1 = _rb(1.0 + modr[R_CB])
            modb[M_CB1] = cb1
            modb[M_AW] = cb1 * wr8
            modb[M_C0, :, 0:128] = jnp.broadcast_to(jnp.sum(modr[R_SB] * wr8, axis=-1, keepdims=True), (8, 128))

            def q_of(j):
                return (qacc[g, :, j * DH:(j + 1) * DH] * QSCALE).astype(bf16)

            mv = [functools.partial(modb_piece, g, n) for n in range(NK)]
            os_ = []
            prl = qk(q_of(0), g)
            for j in range(REP):
                if j + 1 < REP:
                    nxt = qk(q_of(j + 1), g)
                else:
                    oproj(os_[:REP // 2], g, 0, acc_add, mv[:6], 2, never)
                os_.append(pv(prl, g, os_[-1] if os_ else None, never))
                prl = nxt
            pieces = [functools.partial(ln1_piece, _mult(g, XQ, T0 + i * PR), 0,
                                        _mult(g, XQ // 2, i * PR // 2, 8)) for i in range(XQ // PR)]
            fin = [None] * NK

            def acc_fin(n, cs, a):
                fin[n] = acc_ref[:, cs] + a
                acc_ref[:, cs] = fin[n]

            oproj(os_[REP // 2:], g, REP // 2, acc_fin, pieces + mv[6:], 2, never)
            write_x1(0, x0b[...], jnp.concatenate(fin, axis=-1), ga)
            return c

        lax.fori_loop(0, HKV, group0, 0)

        def body(t, carry):
            never = flag[0] > 0
            slot = t % 2
            r0 = _mult(t, TM, T0, 32)
            re = _mult(t, TE, 0, 32)
            rn = _mult(jnp.minimum(t + 1, NM - 1), TM, T0, 32)
            best = list(carry)
            pe = [functools.partial(epi_piece, re + i * PR, best) for i in range(TE // PR)]
            pn = [functools.partial(ln1_piece, rn + i * PR, 1 - slot, i * PR // 2) for i in range(TM // PR)]
            pieces = [p for pair in zip(pe, pn) for p in pair] + pe[len(pn):]
            npg = -(-len(pieces) // (HKV - 1))
            hh = pltpu.bitcast(hb[slot, 0:TM // 2, :], bf16)
            fin = [None] * NK

            def qproj(h):
                return (_dot(hh, wq[:, h * DH:(h + 1) * DH]) * QSCALE).astype(bf16)

            def acc_fin(n, cs, a):
                fin[n] = acc_ref[0:TM, cs] + a

            q = qproj(0)
            for g in range(HKV):
                os_ = []
                for j in range(REP):
                    prl = qk(q, g)
                    if g * REP + j + 1 < HQ:
                        q = qproj(g * REP + j + 1)
                    else:
                        oproj(os_[:REP // 2], g, 0, acc_add, [], 0, never)
                    os_.append(pv(prl, g, os_[-1] if os_ else None, never))
                if g + 1 < HKV:
                    oproj(os_, g, 0, acc_set if g == 0 else acc_add, pieces[g * npg:(g + 1) * npg], 3, never)
                else:
                    oproj(os_[REP // 2:], g, REP // 2, acc_fin, [], 0, never)
            write_x1(r0, xb[pl.ds(r0, TM), :], jnp.concatenate(fin, axis=-1), modr[R_GA])
            cp_out(t).start()
            return tuple(best)

        init = (jnp.full((8, 128), -jnp.inf, f32), jnp.zeros((8, 128), i32))
        best = list(lax.fori_loop(0, NM, body, init))

        for c in cp_wg + cp_wu + [cp_wd]:
            c.wait()
        rl = NM * TE
        for i in range(TL // PR):
            route_piece(rl + i * PR, best, load_x1(rl + i * PR))

        bv, bi = best
        rmax = jnp.max(bv, axis=0, keepdims=True)
        imin = jnp.min(jnp.where(bv == rmax, bi, S), axis=0, keepdims=True)
        idx = jnp.minimum(imin[0, 0], S - 1)
        gate = jnp.concatenate([_rb(1.0 / (1.0 + jnp.exp(-rmax)))] * NK, axis=-1)
        s0 = pl.multiple_of(lax.shift_right_logical(idx, 4) * PR, PR)
        x1s = load_x1(s0)
        mbs, rinvs = load_stats(s0)
        h2s = h2_of(x1s - mbs, rinvs)
        lhs = h2s.reshape(PR, D)

        def mlp(jj, y):
            never = flag[0] > 0
            r0 = _mult(jj, OH, rl)
            pend, due, done, act = [], {}, 0, []
            for j in range(2 * (FC // FCH)):
                toks = due.pop(j, [])
                lj = jnp.concatenate(
                    [jnp.where(never, tok, lhs[:, k * 128:(k + 1) * 128]) for k, tok in enumerate(toks)]
                    + [lhs[:, len(toks) * 128:]], axis=-1)
                wref = wu if j % 2 else wg
                res = _dot(lj.astype(bf16), wref[jj, :, (j // 2) * FCH:(j // 2 + 1) * FCH])
                if done < OH // PR:
                    due.setdefault(j + OGAP, []).append(out_piece(r0 + done * PR, res[:, 0:128], never))
                    done += 1
                    if done == OH // PR:
                        cp_outl(jj).start()
                if j % 2:
                    act.append(pend.pop() * _rb(res))
                else:
                    pend.append(_rb(_silu(_rb(res))))
            assert done == OH // PR and not due
            return y + _dot(jnp.concatenate(act, axis=-1).astype(bf16), wd[pl.ds(_mult(jj, FC), FC), 0:D])

        y = _rb(lax.fori_loop(0, NMLP, mlp, jnp.zeros((PR, D), f32)))
        y = _rb(y * gate)
        rows = lax.broadcasted_iota(i32, (PR, D), 0) + s0
        upd = jnp.where(rows == idx, y, 0.0).reshape(PR // 8, 8, D)
        fix[...] = (x1s + modr[R_GB][None] * (h2s + upd)).reshape(PR, D).astype(bf16)
        for t in range(NM):
            cp_out(t).wait()
        for j in range(NMLP):
            cp_outl(j).wait()
        cp_fix = pltpu.make_async_copy(fix, out_hbm.at[0, pl.ds(s0, PR)], sem_out.at[NM + NMLP])
        cp_fix.start()
        cp_fix.wait()

    scratch = [
        pltpu.VMEM((S, D), bf16),
        pltpu.VMEM((T0, D), bf16),
        pltpu.VMEM((S, D), bf16),
        pltpu.VMEM((2, HKV * XQ // 2, D), u32),
        pltpu.VMEM((HKV, W, DH), bf16),
        pltpu.VMEM((HKV, W, DH), bf16),
        pltpu.VMEM((D, HQ * DH + PAD), bf16),
        pltpu.VMEM((HKV, GD, D + PAD), bf16),
        pltpu.VMEM((NMLP, D, FC + PAD), bf16),
        pltpu.VMEM((NMLP, D, FC + PAD), bf16),
        pltpu.VMEM((F, D + PAD), bf16),
        pltpu.VMEM((NK, 2, D, 128), bf16),
        pltpu.VMEM((HKV, D, D + PAD), bf16),
        pltpu.VMEM((1, D), bf16),
        pltpu.VMEM((D,), bf16),
        pltpu.VMEM((D, 128), f32),
        pltpu.VMEM((NK, 2, 8, 128), f32),
        pltpu.VMEM((HKV, 8, D), f32),
        pltpu.VMEM((5, 8, D), f32),
        pltpu.VMEM((S, 256), f32),
        pltpu.VMEM((T0, D), f32),
        pltpu.VMEM((HKV, T0, GD), f32),
        pltpu.VMEM((NK, T0, 128), f32),
        pltpu.VMEM((PR, D), bf16),
        pltpu.SMEM((1,), i32),
        pltpu.SemaphoreType.DMA((n_in_sems,)),
        pltpu.SemaphoreType.DMA((NM + NMLP + 1,)),
    ]
    return kernel, scratch


@jax.jit
def pallas_adaLN_cond__sliding_block_cached__moe_arch_mod__prompt_kernel(
    A_x: jax.Array,
    A_k_cache: jax.Array,
    A_v_cache: jax.Array,
    A_wq: jax.Array,
    A_wo: jax.Array,
    B_x: jax.Array,
    B_w_r: jax.Array,
    B_w_gate: jax.Array,
    B_w_up: jax.Array,
    B_w_down: jax.Array,
    c: jax.Array,
    w_mod: jax.Array,
):
    B, S, D = A_x.shape
    _, HKV, SK, dh = A_k_cache.shape
    F = B_w_gate.shape[1]
    W = min(4096, max(256, SK // 4))
    assert B == 1 and dh == DH and A_wq.shape == (D, HQ * DH)
    kernel, scratch = _make_kernel(S, D, HKV, SK, W, F)
    any_spec = pl.BlockSpec(memory_space=pl.ANY)
    return pl.pallas_call(
        kernel,
        out_shape=jax.ShapeDtypeStruct((B, S, D), A_x.dtype),
        in_specs=[any_spec] * 11,
        out_specs=any_spec,
        scratch_shapes=scratch,
        compiler_params=pltpu.CompilerParams(vmem_limit_bytes=120 * 1024 * 1024,
                                             disable_semaphore_checks=True, disable_bounds_checks=True),
    )(A_x, A_k_cache, A_v_cache, A_wq, A_wo, B_w_r, B_w_gate, B_w_up, B_w_down, c, w_mod)
```

```python
import functools

import jax
import jax.numpy as jnp
from jax import lax
import jax.experimental.pallas as pl
import jax.experimental.pallas.tpu as pltpu

f32 = jnp.float32
bf16 = jnp.bfloat16
u32 = jnp.uint32
i32 = jnp.int32

HQ = 32
DH = 128
T0 = 480
TM = 224
TE = 256
L0 = 96
PR = 16
EPS = 1e-05
LOG2E = 1.4426950408889634
PAD = 128
NMLP = 2
FCH = 256
OGAP = 3
M_SA, M_CA1, M_CB1, M_AW, M_C0 = range(5)
R_GA, R_SB, R_CB, R_GB = range(4)


def _rb(x):
    return x.astype(bf16).astype(f32)


def _silu(x):
    return x * (1.0 / (1.0 + jnp.exp(-x)))


def _dot(a, b):
    return jnp.dot(a, b, preferred_element_type=f32)


def _mult(i, n, base=0, align=16):
    return base + i * n if isinstance(i, int) else pl.multiple_of(base + i * n, align)


def _make_kernel(S, D, HKV, SK, W, F):
    NM = (S - T0) // TM
    NK = D // 128
    REP = HQ // HKV
    GD = REP * DH
    QSCALE = DH ** (-0.5) * LOG2E
    XQ = 64
    TL = S - NM * TE
    HN = HQ * DH // 2
    FC = F // NMLP
    OH = TL // NMLP
    assert T0 + NM * TM == S and HKV * XQ >= TM and T0 % L0 == 0 and HKV == 4
    assert all(T0 + t * TM >= (t + 1) * TE for t in range(NM)) and OH % PR == 0

    sem_base, n_in_sems = {}, 0
    for name, n in (("c", 1), ("wr", 1), ("x0", T0 // L0), ("x1", HKV), ("xr", 1), ("wma", 2 * NK), ("wq", NK + 1),
                    ("k", HKV), ("v", HKV), ("wo", HKV), ("wmb", HKV), ("wg", NMLP), ("wu", NMLP), ("wd", 1)):
        sem_base[name] = n_in_sems
        n_in_sems += n

    def kernel(x_hbm, k_hbm, v_hbm, wq_hbm, wo_hbm, wr_hbm, wg_hbm, wu_hbm, wd_hbm, c_hbm, wm_hbm,
               out_hbm,
               xb, x0b, ob, hb, kb, vb, wq, wo, wg, wu, wd, wma, wmb, cb, wrb, colb, moda, modr, modb,
               st_ref, acc_ref, qacc, xn_ref, fix, flag, sem_in, sem_out):
        def cp(name, i, src, dst):
            return pltpu.make_async_copy(src, dst, sem_in.at[sem_base[name] + i])

        def cp_x1(g):
            r = pl.ds(_mult(g, XQ, T0), XQ)
            return cp("x1", g, x_hbm.at[0, r], xb.at[r])

        def cp_wma(i, j):
            return cp("wma", 2 * i + j, wm_hbm.at[:, pl.ds(_mult(i, 128, j * D, 128), 128)], wma.at[i, j])

        def cp_wmb(j):
            return cp("wmb", j, wm_hbm.at[:, pl.ds(_mult(j, D, 2 * D, 128), D)], wmb.at[j, :, pl.ds(0, D)])

        def cp_wq(i):
            r = pl.ds(_mult(i, 128), 128)
            return cp("wq", i + 1, wq_hbm.at[r], wq.at[r, pl.ds(0, HQ * DH)])

        def cp_wq0(p):
            c = pl.ds(_mult(p, HN, 0, 128), HN)
            return cp("wq", p, wq_hbm.at[pl.ds(0, 128), c], wq.at[pl.ds(0, 128), c])

        def cp_x0(i):
            r = pl.ds(_mult(i, L0), L0)
            return cp("x0", i, x_hbm.at[0, r], x0b.at[r])

        def cp_k(g):
            return cp("k", g, k_hbm.at[0, g, pl.ds(SK - W, W)], kb.at[g])

        def cp_v(g):
            return cp("v", g, v_hbm.at[0, g, pl.ds(SK - W, W)], vb.at[g])

        def cp_wo(g):
            return cp("wo", g, wo_hbm.at[pl.ds(_mult(g, GD), GD)], wo.at[g, :, pl.ds(0, D)])

        xr0 = T0 + HKV * XQ
        cp_c = cp("c", 0, c_hbm, cb)
        cp_wr = cp("wr", 0, wr_hbm, wrb)
        cp_xr = cp("xr", 0, x_hbm.at[0, pl.ds(xr0, S - xr0)], xb.at[pl.ds(xr0, S - xr0)])
        cp_wg = [cp("wg", j, wg_hbm.at[:, pl.ds(j * FC, FC)], wg.at[j, :, pl.ds(0, FC)]) for j in range(NMLP)]
        cp_wu = [cp("wu", j, wu_hbm.at[:, pl.ds(j * FC, FC)], wu.at[j, :, pl.ds(0, FC)]) for j in range(NMLP)]
        cp_wd = cp("wd", 0, wd_hbm, wd.at[:, pl.ds(0, D)])

        def cp_out(t):
            r = pl.ds(_mult(t, TE), TE)
            return pltpu.make_async_copy(ob.at[r], out_hbm.at[0, r], sem_out.at[t])

        def cp_outl(j):
            r = pl.ds(_mult(j, OH, NM * TE), OH)
            return pltpu.make_async_copy(ob.at[r], out_hbm.at[0, r], sem_out.at[NM + j])

        order = [cp_c] + [cp_x0(i) for i in range(T0 // L0)] + [cp_wma(0, 0), cp_wma(0, 1)]
        for i in range(NK):
            order += [cp_wq(i)] if i else [cp_wq0(0), cp_wq0(1)]
            if i + 1 < NK:
                order += [cp_wma(i + 1, 0), cp_wma(i + 1, 1)]
        order += [cp_wr]
        for g in range(HKV):
            order += [cp_k(g), cp_v(g), cp_wo(g), cp_wmb(g), cp_x1(g)]
        order += [cp_xr] + cp_wg + cp_wu + [cp_wd]
        assert len(order) == n_in_sems
        for c in order:
            c.start()

        flag[0] = 0

        def tie(x, tok, never):
            if tok is None:
                return x
            return jnp.concatenate([jnp.where(never, tok, x[:, :128]), x[:, 128:]], axis=-1)

        def due_rows(lhs, toks, never):
            if not toks:
                return lhs
            parts = [jnp.where(never, tok, lhs[8 * k:8 * k + 8]) for k, tok in enumerate(toks)]
            return jnp.concatenate(parts + [lhs[8 * len(toks):]], axis=0)

        def ln_plain(x):
            m = jnp.sum(x, axis=-1, keepdims=True) * (1.0 / D)
            xc = x - m
            v = jnp.sum(xc * xc, axis=-1, keepdims=True) * (1.0 / D)
            return xc * lax.rsqrt(v + EPS)

        def lane_bc(v):
            return jnp.broadcast_to(v.reshape(-1, 1), (v.shape[0] * 8, 128))

        def sub_bc(p):
            return jnp.broadcast_to(_rb(jnp.sum(p, axis=0, keepdims=True)), p.shape)

        def h2_of(xc, rinv):
            return (xc * rinv) * modb[M_CB1][None] + modr[R_SB][None]

        def load_stats(row):
            st = st_ref[pl.ds(row, PR), :]
            mb = jnp.concatenate([st[:, 0:128]] * NK, axis=-1).reshape(PR // 8, 8, D)
            rinv = jnp.concatenate([st[:, 128:256]] * NK, axis=-1).reshape(PR // 8, 8, D)
            return mb, rinv

        def tok_of(v):
            return v[0:8] + v[8:16]

        def ln1_piece(xrow, slot, hrow, tok=None, never=None):
            x = tie(xb[pl.ds(xrow, PR), :].astype(f32), tok, never).reshape(PR // 8, 8, D)
            h = (ln_plain(x) * modb[M_CA1][None] + modb[M_SA][None]).reshape(PR, D)
            hb[slot, pl.ds(hrow, PR // 2), :] = pltpu.bitcast(h.astype(bf16), u32)
            return tok_of(h[:, 0:128])

        sub_iota = lax.broadcasted_iota(i32, (8, 128), 0)

        def route_piece(row, best, x1):
            m = jnp.sum(x1, axis=-1, keepdims=True) * (1.0 / D)
            mb = _rb(m)
            xc = x1 - mb
            dm = m - mb
            v = jnp.sum(xc * xc, axis=-1, keepdims=True) * (1.0 / D) - dm * dm
            rs = jnp.sum(xc * modb[M_AW][None], axis=-1, keepdims=True)
            sd = _rb(jnp.sqrt(_rb(_rb(jnp.maximum(v, 0.0)) + EPS)))
            r0 = pl.reciprocal(sd, approx=True)
            rinv = r0 * (2.0 - sd * r0)
            st_ref[pl.ds(row, PR), :] = jnp.concatenate([lane_bc(mb), lane_bc(rinv)], axis=-1)
            rr = lane_bc(rs * rinv).reshape(PR // 8, 8, 128) + modb[M_C0, :, 0:128][None]
            rbf = _rb(rr.reshape(PR, 128))
            for j in range(PR // 8):
                rj = rbf[8 * j:8 * j + 8]
                upd = rj > best[0]
                best[1] = jnp.where(upd, sub_iota + (row + 8 * j), best[1])
                best[0] = jnp.where(upd, rj, best[0])
            return xc, rinv, rbf

        def load_x1(row, tok=None, never=None):
            return tie(xb[pl.ds(row, PR), :].astype(f32), tok, never).reshape(PR // 8, 8, D)

        def epi_piece(row, best, tok=None, never=None):
            x1 = load_x1(row, tok, never)
            xc, rinv, rbf = route_piece(row, best, x1)
            ob[pl.ds(row, PR), :] = (x1 + modr[R_GB][None] * h2_of(xc, rinv)).reshape(PR, D).astype(bf16)
            return tok_of(rbf)

        def out_piece(row, tok, never):
            x1 = load_x1(row)
            mb, rinv = load_stats(row)
            mb = jnp.where(never, jnp.concatenate([tok] * NK, axis=-1).reshape(PR // 8, 8, D), mb)
            o = (x1 + modr[R_GB][None] * h2_of(x1 - mb, rinv)).reshape(PR, D)
            ob[pl.ds(row, PR), :] = o.astype(bf16)
            return o[:, 0:128]

        def matvec(w_at, tok, never):
            ys = [None, None] if tok is None else [jnp.where(never, tok[0:8], 0.0)]
            for kg in range(D // 8):
                t = w_at(slice(kg * 8, (kg + 1) * 8)).astype(f32) * colb[kg * 8:(kg + 1) * 8, :]
                k = kg % len(ys)
                ys[k] = t if ys[k] is None else ys[k] + t
            return sum(ys[1:], ys[0])

        def moda_piece(i, j, tok=None, never=None):
            y = sub_bc(matvec(lambda r: wma[i, j, r, :], tok, never))
            if j == 1:
                y = _rb(1.0 + y)
            moda[i, j] = y
            return y

        def modb_piece(ch, n, tok=None, never=None):
            y = sub_bc(matvec(lambda r: wmb[ch, r, n * 128:(n + 1) * 128], tok, never))
            modr[ch, :, n * 128:(n + 1) * 128] = y
            return y

        def qk(q, g):
            s = lax.dot_general(q, kb[g], (((1,), (1,)), ((), ())), preferred_element_type=f32)
            m = jnp.max(s, axis=-1, keepdims=True)
            p = jnp.exp2(s - m)
            l = jnp.sum(p, axis=-1, keepdims=True)
            rl = pl.reciprocal(l, approx=True)
            return p, rl * (2.0 - l * rl)

        def pv(prl, g, prev=None, never=None):
            p, rl = prl
            if prev is not None:
                p = jnp.concatenate([jnp.where(never, prev, p[:, 0:DH]), p[:, DH:]], axis=-1)
            return _dot(p.astype(bf16), vb[g]) * rl

        def paced(nsteps, step, pieces, gap, never):
            outs, done = {}, 0
            for n in range(nsteps):
                a = step(n, outs.pop(n, []))
                if n < nsteps - gap:
                    cnt = int(round((n + 1) * len(pieces) / (nsteps - gap))) - done
                    for k in range(cnt):
                        rr = (k * a.shape[0] // cnt) // PR * PR
                        outs.setdefault(n + gap, []).append(pieces[done](a[rr:rr + PR, 0:128], never))
                        done += 1
            assert done == len(pieces)

        def oproj(os_, g, j0, sink, pieces, gap, never):
            def step(n, toks):
                cs = slice(n * 128, (n + 1) * 128)
                og = jnp.concatenate([due_rows(os_[0], toks, never)] + list(os_[1:]), axis=-1)
                a = _dot(og.astype(bf16), wo[g, j0 * DH:(j0 + len(os_)) * DH, cs])
                sink(n, cs, a)
                return a
            paced(NK, step, pieces, gap, never)

        def acc_set(n, cs, a):
            acc_ref[0:a.shape[0], cs] = a

        def acc_add(n, cs, a):
            acc_ref[0:a.shape[0], cs] += a

        def write_x1(r0, x, acc, ga):
            rows = x.shape[0]
            a = acc.reshape(rows // 8, 8, D) * ga[None]
            xb[pl.ds(r0, rows), :] = (x.astype(f32) + a.reshape(rows, D)).astype(bf16)

        def zero(i, c):
            acc_ref[pl.ds(_mult(i, L0), L0), :] = jnp.zeros((L0, D), f32)
            return c

        lax.fori_loop(0, T0 // L0, zero, 0)
        modr[...] = jnp.zeros((HKV, 8, D), f32)
        cp_c.wait()
        sc = _rb(_silu(cb[...].astype(f32)))
        colb[...] = jnp.broadcast_to(sc, (128, D)).T

        def ln0(i, c):
            cp_x0(i).wait()
            r = pl.ds(_mult(i, L0), L0)
            xn = ln_plain(x0b[r, :].astype(f32))
            for n in range(NK):
                xn_ref[n, r, :] = xn[:, n * 128:(n + 1) * 128]
            return c

        lax.fori_loop(0, T0 // L0, ln0, 0)

        nw = 4 * DH

        def moda_now(i):
            cp_wma(i, 0).wait()
            cp_wma(i, 1).wait()
            moda_piece(i, 0)
            moda_piece(i, 1)

        def h_of(i):
            h = xn_ref[i].reshape(T0 // 8, 8, 128) * moda[i, 1][None] + moda[i, 0][None]
            return h.reshape(T0, 128)

        moda_now(0)

        def kfirst(p, c):
            cp_wq0(p).wait()

            @pl.when(p == 1)
            def _():
                cp_wma(1, 0).wait()
                cp_wma(1, 1).wait()

            never = flag[0] > 0
            h = h_of(0)

            def step(n, toks):
                cols = pl.ds(_mult(p, HN, n * nw, 128), nw)
                a = _dot(due_rows(h, toks, never).astype(bf16), wq[0:128, cols])
                g, c0 = divmod(n * nw, GD)
                qacc[p * (HKV // 2) + g, :, c0:c0 + nw] = a
                return a

            paced(HN // nw, step, [functools.partial(moda_piece, p, j) for j in range(2)], 2, never)
            return c

        lax.fori_loop(0, 2, kfirst, 0)

        def kstep(i, c):
            @pl.when(i == 2)
            def _():
                moda_now(i)

            cp_wq(i).wait()
            ahead = jnp.logical_and(i >= 2, i + 1 < NK)

            @pl.when(ahead)
            def _():
                cp_wma(i + 1, 0).wait()
                cp_wma(i + 1, 1).wait()

            never = flag[0] > 0
            h = h_of(i)
            nxt = jnp.where(ahead, i + 1, i)
            r = pl.ds(_mult(i, 128), 128)

            def step(n, toks):
                a = _dot(due_rows(h, toks, never).astype(bf16), wq[r, n * nw:(n + 1) * nw])
                g, c0 = divmod(n * nw, GD)
                qacc[g, :, c0:c0 + nw] += a
                return a

            paced(HQ * DH // nw, step, [functools.partial(moda_piece, nxt, j) for j in range(2)], 4, never)
            return c

        lax.fori_loop(1, NK, kstep, 0)
        cp_wr.wait()
        modb[M_SA] = jnp.concatenate([moda[i, 0] for i in range(NK)], axis=-1)
        modb[M_CA1] = jnp.concatenate([moda[i, 1] for i in range(NK)], axis=-1)

        def group0(g, c):
            for d in (cp_k(g), cp_v(g), cp_wo(g), cp_wmb(g), cp_x1(g)):
                d.wait()

            @pl.when(g == HKV - 1)
            def _():
                cp_xr.wait()

            never = flag[0] > 0
            ga = modr[R_GA]
            wr8 = jnp.broadcast_to(wrb[...].astype(f32).reshape(1, D), (8, D))
            cb1 = _rb(1.0 + modr[R_CB])
            modb[M_CB1] = cb1
            modb[M_AW] = cb1 * wr8
            modb[M_C0, :, 0:128] = jnp.broadcast_to(jnp.sum(modr[R_SB] * wr8, axis=-1, keepdims=True), (8, 128))

            def q_of(j):
                return (qacc[g, :, j * DH:(j + 1) * DH] * QSCALE).astype(bf16)

            mv = [functools.partial(modb_piece, g, n) for n in range(NK)]
            os_ = []
            prl = qk(q_of(0), g)
            for j in range(REP):
                if j + 1 < REP:
                    nxt = qk(q_of(j + 1), g)
                else:
                    oproj(os_[:REP // 2], g, 0, acc_add, mv[:6], 2, never)
                os_.append(pv(prl, g, os_[-1] if os_ else None, never))
                prl = nxt
            pieces = [functools.partial(ln1_piece, _mult(g, XQ, T0 + i * PR), 0,
                                        _mult(g, XQ // 2, i * PR // 2, 8)) for i in range(XQ // PR)]
            fin = [None] * NK

            def acc_fin(n, cs, a):
                fin[n] = acc_ref[:, cs] + a
                acc_ref[:, cs] = fin[n]

            oproj(os_[REP // 2:], g, REP // 2, acc_fin, pieces + mv[6:], 2, never)
            write_x1(0, x0b[...], jnp.concatenate(fin, axis=-1), ga)
            return c

        lax.fori_loop(0, HKV, group0, 0)

        def body(t, carry):
            never = flag[0] > 0
            slot = t % 2
            r0 = _mult(t, TM, T0, 32)
            re = _mult(t, TE, 0, 32)
            rn = _mult(jnp.minimum(t + 1, NM - 1), TM, T0, 32)
            best = list(carry)
            pe = [functools.partial(epi_piece, re + i * PR, best) for i in range(TE // PR)]
            pn = [functools.partial(ln1_piece, rn + i * PR, 1 - slot, i * PR // 2) for i in range(TM // PR)]
            pieces = [p for pair in zip(pe, pn) for p in pair] + pe[len(pn):]
            npg = -(-len(pieces) // (HKV - 1))
            hh = pltpu.bitcast(hb[slot, 0:TM // 2, :], bf16)
            fin = [None] * NK

            def qproj(h):
                return (_dot(hh, wq[:, h * DH:(h + 1) * DH]) * QSCALE).astype(bf16)

            def acc_fin(n, cs, a):
                fin[n] = acc_ref[0:TM, cs] + a

            q = qproj(0)
            for g in range(HKV):
                os_ = []
                for j in range(REP):
                    prl = qk(q, g)
                    if g * REP + j + 1 < HQ:
                        q = qproj(g * REP + j + 1)
                    else:
                        oproj(os_[:REP // 2], g, 0, acc_add, [], 0, never)
                    os_.append(pv(prl, g, os_[-1] if os_ else None, never))
                if g + 1 < HKV:
                    oproj(os_, g, 0, acc_set if g == 0 else acc_add, pieces[g * npg:(g + 1) * npg], 3, never)
                else:
                    oproj(os_[REP // 2:], g, REP // 2, acc_fin, [], 0, never)
            write_x1(r0, xb[pl.ds(r0, TM), :], jnp.concatenate(fin, axis=-1), modr[R_GA])
            cp_out(t).start()
            return tuple(best)

        init = (jnp.full((8, 128), -jnp.inf, f32), jnp.zeros((8, 128), i32))
        best = list(lax.fori_loop(0, NM, body, init))

        for c in cp_wg + cp_wu + [cp_wd]:
            c.wait()
        rl = NM * TE
        for i in range(TL // PR):
            route_piece(rl + i * PR, best, load_x1(rl + i * PR))

        bv, bi = best
        rmax = jnp.max(bv, axis=0, keepdims=True)
        imin = jnp.min(jnp.where(bv == rmax, bi, S), axis=0, keepdims=True)
        idx = jnp.minimum(imin[0, 0], S - 1)
        gate = jnp.concatenate([_rb(1.0 / (1.0 + jnp.exp(-rmax)))] * NK, axis=-1)
        s0 = pl.multiple_of(lax.shift_right_logical(idx, 4) * PR, PR)
        x1s = load_x1(s0)
        mbs, rinvs = load_stats(s0)
        h2s = h2_of(x1s - mbs, rinvs)
        lhs = h2s.reshape(PR, D)

        def mlp(jj, y):
            never = flag[0] > 0
            r0 = _mult(jj, OH, rl)
            pend, due, done, act = [], {}, 0, []
            for j in range(2 * (FC // FCH)):
                toks = due.pop(j, [])
                lj = jnp.concatenate(
                    [jnp.where(never, tok, lhs[:, k * 128:(k + 1) * 128]) for k, tok in enumerate(toks)]
                    + [lhs[:, len(toks) * 128:]], axis=-1)
                wref = wu if j % 2 else wg
                res = _dot(lj.astype(bf16), wref[jj, :, (j // 2) * FCH:(j // 2 + 1) * FCH])
                if done < OH // PR:
                    due.setdefault(j + OGAP, []).append(out_piece(r0 + done * PR, res[:, 0:128], never))
                    done += 1
                    if done == OH // PR:
                        cp_outl(jj).start()
                if j % 2:
                    act.append(pend.pop() * _rb(res))
                else:
                    pend.append(_rb(_silu(_rb(res))))
            assert done == OH // PR and not due
            return y + _dot(jnp.concatenate(act, axis=-1).astype(bf16), wd[pl.ds(_mult(jj, FC), FC), 0:D])

        y = _rb(lax.fori_loop(0, NMLP, mlp, jnp.zeros((PR, D), f32)))
        y = _rb(y * gate)
        rows = lax.broadcasted_iota(i32, (PR, D), 0) + s0
        upd = jnp.where(rows == idx, y, 0.0).reshape(PR // 8, 8, D)
        fix[...] = (x1s + modr[R_GB][None] * (h2s + upd)).reshape(PR, D).astype(bf16)
        for t in range(NM):
            cp_out(t).wait()
        for j in range(NMLP):
            cp_outl(j).wait()
        cp_fix = pltpu.make_async_copy(fix, out_hbm.at[0, pl.ds(s0, PR)], sem_out.at[NM + NMLP])
        cp_fix.start()
        cp_fix.wait()

    scratch = [
        pltpu.VMEM((S, D), bf16),
        pltpu.VMEM((T0, D), bf16),
        pltpu.VMEM((S, D), bf16),
        pltpu.VMEM((2, HKV * XQ // 2, D), u32),
        pltpu.VMEM((HKV, W, DH), bf16),
        pltpu.VMEM((HKV, W, DH), bf16),
        pltpu.VMEM((D, HQ * DH + PAD), bf16),
        pltpu.VMEM((HKV, GD, D + PAD), bf16),
        pltpu.VMEM((NMLP, D, FC + PAD), bf16),
        pltpu.VMEM((NMLP, D, FC + PAD), bf16),
        pltpu.VMEM((F, D + PAD), bf16),
        pltpu.VMEM((NK, 2, D, 128), bf16),
        pltpu.VMEM((HKV, D, D + PAD), bf16),
        pltpu.VMEM((1, D), bf16),
        pltpu.VMEM((D,), bf16),
        pltpu.VMEM((D, 128), f32),
        pltpu.VMEM((NK, 2, 8, 128), f32),
        pltpu.VMEM((HKV, 8, D), f32),
        pltpu.VMEM((5, 8, D), f32),
        pltpu.VMEM((S, 256), f32),
        pltpu.VMEM((T0, D), f32),
        pltpu.VMEM((HKV, T0, GD), f32),
        pltpu.VMEM((NK, T0, 128), f32),
        pltpu.VMEM((PR, D), bf16),
        pltpu.SMEM((1,), i32),
        pltpu.SemaphoreType.DMA((n_in_sems,)),
        pltpu.SemaphoreType.DMA((NM + NMLP + 1,)),
    ]
    return kernel, scratch


@jax.jit
def pallas_adaLN_cond__sliding_block_cached__moe_arch_mod__prompt_kernel(
    A_x: jax.Array,
    A_k_cache: jax.Array,
    A_v_cache: jax.Array,
    A_wq: jax.Array,
    A_wo: jax.Array,
    B_x: jax.Array,
    B_w_r: jax.Array,
    B_w_gate: jax.Array,
    B_w_up: jax.Array,
    B_w_down: jax.Array,
    c: jax.Array,
    w_mod: jax.Array,
):
    B, S, D = A_x.shape
    _, HKV, SK, dh = A_k_cache.shape
    F = B_w_gate.shape[1]
    W = min(4096, max(256, SK // 4))
    assert B == 1 and dh == DH and A_wq.shape == (D, HQ * DH)
    kernel, scratch = _make_kernel(S, D, HKV, SK, W, F)
    any_spec = pl.BlockSpec(memory_space=pl.ANY)
    return pl.pallas_call(
        kernel,
        out_shape=jax.ShapeDtypeStruct((B, S, D), A_x.dtype),
        in_specs=[any_spec] * 11,
        out_specs=any_spec,
        scratch_shapes=scratch,
        compiler_params=pltpu.CompilerParams(vmem_limit_bytes=120 * 1024 * 1024,
                                             disable_semaphore_checks=True, disable_bounds_checks=True),
    )(A_x, A_k_cache, A_v_cache, A_wq, A_wo, B_w_r, B_w_gate, B_w_up, B_w_down, c, w_mod)
```

```python
import functools

import jax
import jax.numpy as jnp
from jax import lax
import jax.experimental.pallas as pl
import jax.experimental.pallas.tpu as pltpu

f32 = jnp.float32
bf16 = jnp.bfloat16
u32 = jnp.uint32
i32 = jnp.int32

HQ = 32
DH = 128
T0 = 480
TM = 224
TE = 256
L0 = 96
PR = 16
EPS = 1e-05
LOG2E = 1.4426950408889634
PAD = 128
NMLP = 2
FCH = 256
OGAP = 3
M_SA, M_CA1, M_CB1, M_AW, M_C0 = range(5)
R_GA, R_SB, R_CB, R_GB = range(4)


def _rb(x):
    return x.astype(bf16).astype(f32)


def _silu(x):
    return x * (1.0 / (1.0 + jnp.exp(-x)))


def _dot(a, b):
    return jnp.dot(a, b, preferred_element_type=f32)


def _mult(i, n, base=0, align=16):
    return base + i * n if isinstance(i, int) else pl.multiple_of(base + i * n, align)


def _make_kernel(S, D, HKV, SK, W, F):
    NM = (S - T0) // TM
    NK = D // 128
    REP = HQ // HKV
    GD = REP * DH
    QSCALE = DH ** (-0.5) * LOG2E
    XQ = 64
    TL = S - NM * TE
    HN = HQ * DH // 2
    FC = F // NMLP
    OH = TL // NMLP
    assert T0 + NM * TM == S and HKV * XQ >= TM and T0 % L0 == 0 and HKV == 4
    assert all(T0 + t * TM >= (t + 1) * TE for t in range(NM)) and OH % PR == 0

    sem_base, n_in_sems = {}, 0
    for name, n in (("c", 1), ("wr", 1), ("x0", T0 // L0), ("x1", HKV), ("xr", 1), ("wma", 2 * NK), ("wq", NK + 1),
                    ("k", HKV), ("v", HKV), ("wo", HKV), ("wmb", HKV), ("wg", NMLP), ("wu", NMLP), ("wd", 1)):
        sem_base[name] = n_in_sems
        n_in_sems += n

    def kernel(x_hbm, k_hbm, v_hbm, wq_hbm, wo_hbm, wr_hbm, wg_hbm, wu_hbm, wd_hbm, c_hbm, wm_hbm,
               out_hbm,
               xb, x0b, ob, hb, kb, vb, wq, wo, wg, wu, wd, wma, wmb, cb, wrb, colb, moda, modr, modb,
               st_ref, acc_ref, qacc, xn_ref, fix, flag, sem_in, sem_out):
        def cp(name, i, src, dst):
            return pltpu.make_async_copy(src, dst, sem_in.at[sem_base[name] + i])

        def cp_x1(g):
            r = pl.ds(_mult(g, XQ, T0), XQ)
            return cp("x1", g, x_hbm.at[0, r], xb.at[r])

        def cp_wma(i, j):
            return cp("wma", 2 * i + j, wm_hbm.at[:, pl.ds(_mult(i, 128, j * D, 128), 128)], wma.at[i, j])

        def cp_wmb(j):
            return cp("wmb", j, wm_hbm.at[:, pl.ds(_mult(j, D, 2 * D, 128), D)], wmb.at[j, :, pl.ds(0, D)])

        def cp_wq(i):
            r = pl.ds(_mult(i, 128), 128)
            return cp("wq", i + 1, wq_hbm.at[r], wq.at[r, pl.ds(0, HQ * DH)])

        def cp_wq0(p):
            c = pl.ds(_mult(p, HN, 0, 128), HN)
            return cp("wq", p, wq_hbm.at[pl.ds(0, 128), c], wq.at[pl.ds(0, 128), c])

        def cp_x0(i):
            r = pl.ds(_mult(i, L0), L0)
            return cp("x0", i, x_hbm.at[0, r], x0b.at[r])

        def cp_k(g):
            return cp("k", g, k_hbm.at[0, g, pl.ds(SK - W, W)], kb.at[g])

        def cp_v(g):
            return cp("v", g, v_hbm.at[0, g, pl.ds(SK - W, W)], vb.at[g])

        def cp_wo(g):
            return cp("wo", g, wo_hbm.at[pl.ds(_mult(g, GD), GD)], wo.at[g, :, pl.ds(0, D)])

        xr0 = T0 + HKV * XQ
        cp_c = cp("c", 0, c_hbm, cb)
        cp_wr = cp("wr", 0, wr_hbm, wrb)
        cp_xr = cp("xr", 0, x_hbm.at[0, pl.ds(xr0, S - xr0)], xb.at[pl.ds(xr0, S - xr0)])
        cp_wg = [cp("wg", j, wg_hbm.at[:, pl.ds(j * FC, FC)], wg.at[j, :, pl.ds(0, FC)]) for j in range(NMLP)]
        cp_wu = [cp("wu", j, wu_hbm.at[:, pl.ds(j * FC, FC)], wu.at[j, :, pl.ds(0, FC)]) for j in range(NMLP)]
        cp_wd = cp("wd", 0, wd_hbm, wd.at[:, pl.ds(0, D)])

        def cp_out(t):
            r = pl.ds(_mult(t, TE), TE)
            return pltpu.make_async_copy(ob.at[r], out_hbm.at[0, r], sem_out.at[t])

        def cp_outl(j):
            r = pl.ds(_mult(j, OH, NM * TE), OH)
            return pltpu.make_async_copy(ob.at[r], out_hbm.at[0, r], sem_out.at[NM + j])

        def wma_pair(i):
            return [cp_wma(i, 0), cp_wma(i, 1)] if i < NK else []

        order = [cp_c] + [cp_x0(i) for i in range(T0 // L0)] + wma_pair(0)
        order += [cp_wq0(0)] + wma_pair(1) + [cp_wq0(1), cp_wq(1)] + wma_pair(2)
        for i in range(2, NK):
            order += wma_pair(i + 1) + [cp_wq(i)]
        order += [cp_wr]
        for g in range(HKV):
            order += [cp_k(g), cp_v(g), cp_wo(g), cp_wmb(g), cp_x1(g)]
        order += [cp_xr] + cp_wg + cp_wu + [cp_wd]
        assert len(order) == n_in_sems
        for c in order:
            c.start()

        flag[0] = 0

        def tie(x, tok, never):
            if tok is None:
                return x
            return jnp.concatenate([jnp.where(never, tok, x[:, :128]), x[:, 128:]], axis=-1)

        def due_rows(lhs, toks, never):
            if not toks:
                return lhs
            parts = [jnp.where(never, tok, lhs[8 * k:8 * k + 8]) for k, tok in enumerate(toks)]
            return jnp.concatenate(parts + [lhs[8 * len(toks):]], axis=0)

        def ln_plain(x):
            m = jnp.sum(x, axis=-1, keepdims=True) * (1.0 / D)
            xc = x - m
            v = jnp.sum(xc * xc, axis=-1, keepdims=True) * (1.0 / D)
            return xc * lax.rsqrt(v + EPS)

        def lane_bc(v):
            return jnp.broadcast_to(v.reshape(-1, 1), (v.shape[0] * 8, 128))

        def sub_bc(p):
            return jnp.broadcast_to(_rb(jnp.sum(p, axis=0, keepdims=True)), p.shape)

        def h2_of(xc, rinv):
            return (xc * rinv) * modb[M_CB1][None] + modr[R_SB][None]

        def load_stats(row):
            st = st_ref[pl.ds(row, PR), :]
            mb = jnp.concatenate([st[:, 0:128]] * NK, axis=-1).reshape(PR // 8, 8, D)
            rinv = jnp.concatenate([st[:, 128:256]] * NK, axis=-1).reshape(PR // 8, 8, D)
            return mb, rinv

        def tok_of(v):
            return v[0:8] + v[8:16]

        def ln1_piece(xrow, slot, hrow, tok=None, never=None):
            x = tie(xb[pl.ds(xrow, PR), :].astype(f32), tok, never).reshape(PR // 8, 8, D)
            h = (ln_plain(x) * modb[M_CA1][None] + modb[M_SA][None]).reshape(PR, D)
            hb[slot, pl.ds(hrow, PR // 2), :] = pltpu.bitcast(h.astype(bf16), u32)
            return tok_of(h[:, 0:128])

        sub_iota = lax.broadcasted_iota(i32, (8, 128), 0)

        def route_piece(row, best, x1):
            m = jnp.sum(x1, axis=-1, keepdims=True) * (1.0 / D)
            mb = _rb(m)
            xc = x1 - mb
            dm = m - mb
            v = jnp.sum(xc * xc, axis=-1, keepdims=True) * (1.0 / D) - dm * dm
            rs = jnp.sum(xc * modb[M_AW][None], axis=-1, keepdims=True)
            sd = _rb(jnp.sqrt(_rb(_rb(jnp.maximum(v, 0.0)) + EPS)))
            r0 = pl.reciprocal(sd, approx=True)
            rinv = r0 * (2.0 - sd * r0)
            st_ref[pl.ds(row, PR), :] = jnp.concatenate([lane_bc(mb), lane_bc(rinv)], axis=-1)
            rr = lane_bc(rs * rinv).reshape(PR // 8, 8, 128) + modb[M_C0, :, 0:128][None]
            rbf = _rb(rr.reshape(PR, 128))
            for j in range(PR // 8):
                rj = rbf[8 * j:8 * j + 8]
                upd = rj > best[0]
                best[1] = jnp.where(upd, sub_iota + (row + 8 * j), best[1])
                best[0] = jnp.where(upd, rj, best[0])
            return xc, rinv, rbf

        def load_x1(row, tok=None, never=None):
            return tie(xb[pl.ds(row, PR), :].astype(f32), tok, never).reshape(PR // 8, 8, D)

        def epi_piece(row, best, tok=None, never=None):
            x1 = load_x1(row, tok, never)
            xc, rinv, rbf = route_piece(row, best, x1)
            ob[pl.ds(row, PR), :] = (x1 + modr[R_GB][None] * h2_of(xc, rinv)).reshape(PR, D).astype(bf16)
            return tok_of(rbf)

        def out_piece(row, tok, never):
            x1 = load_x1(row)
            mb, rinv = load_stats(row)
            mb = jnp.where(never, jnp.concatenate([tok] * NK, axis=-1).reshape(PR // 8, 8, D), mb)
            o = (x1 + modr[R_GB][None] * h2_of(x1 - mb, rinv)).reshape(PR, D)
            ob[pl.ds(row, PR), :] = o.astype(bf16)
            return o[:, 0:128]

        def matvec(w_at, tok, never):
            ys = [None, None] if tok is None else [jnp.where(never, tok[0:8], 0.0)]
            for kg in range(D // 8):
                t = w_at(slice(kg * 8, (kg + 1) * 8)).astype(f32) * colb[kg * 8:(kg + 1) * 8, :]
                k = kg % len(ys)
                ys[k] = t if ys[k] is None else ys[k] + t
            return sum(ys[1:], ys[0])

        def moda_piece(i, j, tok=None, never=None):
            y = sub_bc(matvec(lambda r: wma[i, j, r, :], tok, never))
            if j == 1:
                y = _rb(1.0 + y)
            moda[i, j] = y
            return y

        def modb_piece(ch, n, tok=None, never=None):
            y = sub_bc(matvec(lambda r: wmb[ch, r, n * 128:(n + 1) * 128], tok, never))
            modr[ch, :, n * 128:(n + 1) * 128] = y
            return y

        def qk(q, g):
            s = lax.dot_general(q, kb[g], (((1,), (1,)), ((), ())), preferred_element_type=f32)
            m = jnp.max(s, axis=-1, keepdims=True)
            p = jnp.exp2(s - m)
            l = jnp.sum(p, axis=-1, keepdims=True)
            rl = pl.reciprocal(l, approx=True)
            return p, rl * (2.0 - l * rl)

        def pv(prl, g, prev=None, never=None):
            p, rl = prl
            if prev is not None:
                p = jnp.concatenate([jnp.where(never, prev, p[:, 0:DH]), p[:, DH:]], axis=-1)
            return _dot(p.astype(bf16), vb[g]) * rl

        def paced(nsteps, step, pieces, gap, never):
            outs, done = {}, 0
            for n in range(nsteps):
                a = step(n, outs.pop(n, []))
                if n < nsteps - gap:
                    cnt = int(round((n + 1) * len(pieces) / (nsteps - gap))) - done
                    for k in range(cnt):
                        rr = (k * a.shape[0] // cnt) // PR * PR
                        outs.setdefault(n + gap, []).append(pieces[done](a[rr:rr + PR, 0:128], never))
                        done += 1
            assert done == len(pieces)

        def oproj(os_, g, j0, sink, pieces, gap, never):
            def step(n, toks):
                cs = slice(n * 128, (n + 1) * 128)
                og = jnp.concatenate([due_rows(os_[0], toks, never)] + list(os_[1:]), axis=-1)
                a = _dot(og.astype(bf16), wo[g, j0 * DH:(j0 + len(os_)) * DH, cs])
                sink(n, cs, a)
                return a
            paced(NK, step, pieces, gap, never)

        def acc_set(n, cs, a):
            acc_ref[0:a.shape[0], cs] = a

        def acc_add(n, cs, a):
            acc_ref[0:a.shape[0], cs] += a

        def write_x1(r0, x, acc, ga):
            rows = x.shape[0]
            a = acc.reshape(rows // 8, 8, D) * ga[None]
            xb[pl.ds(r0, rows), :] = (x.astype(f32) + a.reshape(rows, D)).astype(bf16)

        def zero(i, c):
            acc_ref[pl.ds(_mult(i, L0), L0), :] = jnp.zeros((L0, D), f32)
            return c

        lax.fori_loop(0, T0 // L0, zero, 0)
        modr[...] = jnp.zeros((HKV, 8, D), f32)
        cp_c.wait()
        sc = _rb(_silu(cb[...].astype(f32)))
        colb[...] = jnp.broadcast_to(sc, (128, D)).T

        def ln0(i, c):
            cp_x0(i).wait()
            r = pl.ds(_mult(i, L0), L0)
            xn = ln_plain(x0b[r, :].astype(f32))
            for n in range(NK):
                xn_ref[n, r, :] = xn[:, n * 128:(n + 1) * 128]
            return c

        lax.fori_loop(0, T0 // L0, ln0, 0)

        nw = 4 * DH

        def moda_now(i):
            cp_wma(i, 0).wait()
            cp_wma(i, 1).wait()
            moda_piece(i, 0)
            moda_piece(i, 1)

        def h_of(i):
            h = xn_ref[i].reshape(T0 // 8, 8, 128) * moda[i, 1][None] + moda[i, 0][None]
            return h.reshape(T0, 128)

        moda_now(0)

        def kfirst(p, c):
            cp_wq0(p).wait()

            @pl.when(p == 1)
            def _():
                cp_wma(1, 0).wait()
                cp_wma(1, 1).wait()

            never = flag[0] > 0
            h = h_of(0)

            def step(n, toks):
                cols = pl.ds(_mult(p, HN, n * nw, 128), nw)
                a = _dot(due_rows(h, toks, never).astype(bf16), wq[0:128, cols])
                g, c0 = divmod(n * nw, GD)
                qacc[p * (HKV // 2) + g, :, c0:c0 + nw] = a
                return a

            paced(HN // nw, step, [functools.partial(moda_piece, p, j) for j in range(2)], 2, never)
            return c

        lax.fori_loop(0, 2, kfirst, 0)

        def kstep(i, c):
            @pl.when(i == 2)
            def _():
                moda_now(i)

            cp_wq(i).wait()
            ahead = jnp.logical_and(i >= 2, i + 1 < NK)

            @pl.when(ahead)
            def _():
                cp_wma(i + 1, 0).wait()
                cp_wma(i + 1, 1).wait()

            never = flag[0] > 0
            h = h_of(i)
            nxt = jnp.where(ahead, i + 1, i)
            r = pl.ds(_mult(i, 128), 128)

            def step(n, toks):
                a = _dot(due_rows(h, toks, never).astype(bf16), wq[r, n * nw:(n + 1) * nw])
                g, c0 = divmod(n * nw, GD)
                qacc[g, :, c0:c0 + nw] += a
                return a

            paced(HQ * DH // nw, step, [functools.partial(moda_piece, nxt, j) for j in range(2)], 4, never)
            return c

        lax.fori_loop(1, NK, kstep, 0)
        cp_wr.wait()
        modb[M_SA] = jnp.concatenate([moda[i, 0] for i in range(NK)], axis=-1)
        modb[M_CA1] = jnp.concatenate([moda[i, 1] for i in range(NK)], axis=-1)

        def group0(g, c):
            for d in (cp_k(g), cp_v(g), cp_wo(g), cp_wmb(g), cp_x1(g)):
                d.wait()

            @pl.when(g == HKV - 1)
            def _():
                cp_xr.wait()

            never = flag[0] > 0
            ga = modr[R_GA]
            wr8 = jnp.broadcast_to(wrb[...].astype(f32).reshape(1, D), (8, D))
            cb1 = _rb(1.0 + modr[R_CB])
            modb[M_CB1] = cb1
            modb[M_AW] = cb1 * wr8
            modb[M_C0, :, 0:128] = jnp.broadcast_to(jnp.sum(modr[R_SB] * wr8, axis=-1, keepdims=True), (8, 128))

            def q_of(j):
                return (qacc[g, :, j * DH:(j + 1) * DH] * QSCALE).astype(bf16)

            mv = [functools.partial(modb_piece, g, n) for n in range(NK)]
            os_ = []
            prl = qk(q_of(0), g)
            for j in range(REP):
                if j + 1 < REP:
                    nxt = qk(q_of(j + 1), g)
                else:
                    oproj(os_[:REP // 2], g, 0, acc_add, mv[:6], 2, never)
                os_.append(pv(prl, g, os_[-1] if os_ else None, never))
                prl = nxt
            pieces = [functools.partial(ln1_piece, _mult(g, XQ, T0 + i * PR), 0,
                                        _mult(g, XQ // 2, i * PR // 2, 8)) for i in range(XQ // PR)]
            fin = [None] * NK

            def acc_fin(n, cs, a):
                fin[n] = acc_ref[:, cs] + a
                acc_ref[:, cs] = fin[n]

            oproj(os_[REP // 2:], g, REP // 2, acc_fin, pieces + mv[6:], 2, never)
            write_x1(0, x0b[...], jnp.concatenate(fin, axis=-1), ga)
            return c

        lax.fori_loop(0, HKV, group0, 0)

        def body(t, carry):
            never = flag[0] > 0
            slot = t % 2
            r0 = _mult(t, TM, T0, 32)
            re = _mult(t, TE, 0, 32)
            rn = _mult(jnp.minimum(t + 1, NM - 1), TM, T0, 32)
            best = list(carry)
            pe = [functools.partial(epi_piece, re + i * PR, best) for i in range(TE // PR)]
            pn = [functools.partial(ln1_piece, rn + i * PR, 1 - slot, i * PR // 2) for i in range(TM // PR)]
            pieces = [p for pair in zip(pe, pn) for p in pair] + pe[len(pn):]
            npg = -(-len(pieces) // (HKV - 1))
            hh = pltpu.bitcast(hb[slot, 0:TM // 2, :], bf16)
            fin = [None] * NK

            def qproj(h):
                return (_dot(hh, wq[:, h * DH:(h + 1) * DH]) * QSCALE).astype(bf16)

            def acc_fin(n, cs, a):
                fin[n] = acc_ref[0:TM, cs] + a

            q = qproj(0)
            for g in range(HKV):
                os_ = []
                for j in range(REP):
                    prl = qk(q, g)
                    if g * REP + j + 1 < HQ:
                        q = qproj(g * REP + j + 1)
                    else:
                        oproj(os_[:REP // 2], g, 0, acc_add, [], 0, never)
                    os_.append(pv(prl, g, os_[-1] if os_ else None, never))
                if g + 1 < HKV:
                    oproj(os_, g, 0, acc_set if g == 0 else acc_add, pieces[g * npg:(g + 1) * npg], 3, never)
                else:
                    oproj(os_[REP // 2:], g, REP // 2, acc_fin, [], 0, never)
            write_x1(r0, xb[pl.ds(r0, TM), :], jnp.concatenate(fin, axis=-1), modr[R_GA])
            cp_out(t).start()
            return tuple(best)

        init = (jnp.full((8, 128), -jnp.inf, f32), jnp.zeros((8, 128), i32))
        best = list(lax.fori_loop(0, NM, body, init))

        for c in cp_wg + cp_wu + [cp_wd]:
            c.wait()
        rl = NM * TE
        for i in range(TL // PR):
            route_piece(rl + i * PR, best, load_x1(rl + i * PR))

        bv, bi = best
        rmax = jnp.max(bv, axis=0, keepdims=True)
        imin = jnp.min(jnp.where(bv == rmax, bi, S), axis=0, keepdims=True)
        idx = jnp.minimum(imin[0, 0], S - 1)
        gate = jnp.concatenate([_rb(1.0 / (1.0 + jnp.exp(-rmax)))] * NK, axis=-1)
        s0 = pl.multiple_of(lax.shift_right_logical(idx, 4) * PR, PR)
        x1s = load_x1(s0)
        mbs, rinvs = load_stats(s0)
        h2s = h2_of(x1s - mbs, rinvs)
        lhs = h2s.reshape(PR, D)

        def mlp(jj, y):
            never = flag[0] > 0
            r0 = _mult(jj, OH, rl)
            pend, due, done, act = [], {}, 0, []
            for j in range(2 * (FC // FCH)):
                toks = due.pop(j, [])
                lj = jnp.concatenate(
                    [jnp.where(never, tok, lhs[:, k * 128:(k + 1) * 128]) for k, tok in enumerate(toks)]
                    + [lhs[:, len(toks) * 128:]], axis=-1)
                wref = wu if j % 2 else wg
                res = _dot(lj.astype(bf16), wref[jj, :, (j // 2) * FCH:(j // 2 + 1) * FCH])
                if done < OH // PR:
                    due.setdefault(j + OGAP, []).append(out_piece(r0 + done * PR, res[:, 0:128], never))
                    done += 1
                    if done == OH // PR:
                        cp_outl(jj).start()
                if j % 2:
                    act.append(pend.pop() * _rb(res))
                else:
                    pend.append(_rb(_silu(_rb(res))))
            assert done == OH // PR and not due
            return y + _dot(jnp.concatenate(act, axis=-1).astype(bf16), wd[pl.ds(_mult(jj, FC), FC), 0:D])

        y = _rb(lax.fori_loop(0, NMLP, mlp, jnp.zeros((PR, D), f32)))
        y = _rb(y * gate)
        rows = lax.broadcasted_iota(i32, (PR, D), 0) + s0
        upd = jnp.where(rows == idx, y, 0.0).reshape(PR // 8, 8, D)
        fix[...] = (x1s + modr[R_GB][None] * (h2s + upd)).reshape(PR, D).astype(bf16)
        for t in range(NM):
            cp_out(t).wait()
        for j in range(NMLP):
            cp_outl(j).wait()
        cp_fix = pltpu.make_async_copy(fix, out_hbm.at[0, pl.ds(s0, PR)], sem_out.at[NM + NMLP])
        cp_fix.start()
        cp_fix.wait()

    scratch = [
        pltpu.VMEM((S, D), bf16),
        pltpu.VMEM((T0, D), bf16),
        pltpu.VMEM((S, D), bf16),
        pltpu.VMEM((2, HKV * XQ // 2, D), u32),
        pltpu.VMEM((HKV, W, DH), bf16),
        pltpu.VMEM((HKV, W, DH), bf16),
        pltpu.VMEM((D, HQ * DH + PAD), bf16),
        pltpu.VMEM((HKV, GD, D + PAD), bf16),
        pltpu.VMEM((NMLP, D, FC + PAD), bf16),
        pltpu.VMEM((NMLP, D, FC + PAD), bf16),
        pltpu.VMEM((F, D + PAD), bf16),
        pltpu.VMEM((NK, 2, D, 128), bf16),
        pltpu.VMEM((HKV, D, D + PAD), bf16),
        pltpu.VMEM((1, D), bf16),
        pltpu.VMEM((D,), bf16),
        pltpu.VMEM((D, 128), f32),
        pltpu.VMEM((NK, 2, 8, 128), f32),
        pltpu.VMEM((HKV, 8, D), f32),
        pltpu.VMEM((5, 8, D), f32),
        pltpu.VMEM((S, 256), f32),
        pltpu.VMEM((T0, D), f32),
        pltpu.VMEM((HKV, T0, GD), f32),
        pltpu.VMEM((NK, T0, 128), f32),
        pltpu.VMEM((PR, D), bf16),
        pltpu.SMEM((1,), i32),
        pltpu.SemaphoreType.DMA((n_in_sems,)),
        pltpu.SemaphoreType.DMA((NM + NMLP + 1,)),
    ]
    return kernel, scratch


@jax.jit
def pallas_adaLN_cond__sliding_block_cached__moe_arch_mod__prompt_kernel(
    A_x: jax.Array,
    A_k_cache: jax.Array,
    A_v_cache: jax.Array,
    A_wq: jax.Array,
    A_wo: jax.Array,
    B_x: jax.Array,
    B_w_r: jax.Array,
    B_w_gate: jax.Array,
    B_w_up: jax.Array,
    B_w_down: jax.Array,
    c: jax.Array,
    w_mod: jax.Array,
):
    B, S, D = A_x.shape
    _, HKV, SK, dh = A_k_cache.shape
    F = B_w_gate.shape[1]
    W = min(4096, max(256, SK // 4))
    assert B == 1 and dh == DH and A_wq.shape == (D, HQ * DH)
    kernel, scratch = _make_kernel(S, D, HKV, SK, W, F)
    any_spec = pl.BlockSpec(memory_space=pl.ANY)
    return pl.pallas_call(
        kernel,
        out_shape=jax.ShapeDtypeStruct((B, S, D), A_x.dtype),
        in_specs=[any_spec] * 11,
        out_specs=any_spec,
        scratch_shapes=scratch,
        compiler_params=pltpu.CompilerParams(vmem_limit_bytes=120 * 1024 * 1024,
                                             disable_semaphore_checks=True, disable_bounds_checks=True),
    )(A_x, A_k_cache, A_v_cache, A_wq, A_wo, B_w_r, B_w_gate, B_w_up, B_w_down, c, w_mod)
```

```python
import functools

import jax
import jax.numpy as jnp
from jax import lax
import jax.experimental.pallas as pl
import jax.experimental.pallas.tpu as pltpu

f32 = jnp.float32
bf16 = jnp.bfloat16
u32 = jnp.uint32
i32 = jnp.int32

HQ = 32
DH = 128
T0 = 480
TM = 224
TE = 256
L0 = 96
PR = 16
EPS = 1e-05
LOG2E = 1.4426950408889634
PAD = 128
NMLP = 2
FCH = 256
OGAP = 3
M_SA, M_CA1, M_CB1, M_AW, M_C0 = range(5)
R_GA, R_SB, R_CB, R_GB = range(4)


def _rb(x):
    return x.astype(bf16).astype(f32)


def _silu(x):
    return x * (1.0 / (1.0 + jnp.exp(-x)))


def _dot(a, b):
    return jnp.dot(a, b, preferred_element_type=f32)


def _mult(i, n, base=0, align=16):
    return base + i * n if isinstance(i, int) else pl.multiple_of(base + i * n, align)


def _make_kernel(S, D, HKV, SK, W, F):
    NM = (S - T0) // TM
    NK = D // 128
    REP = HQ // HKV
    GD = REP * DH
    QSCALE = DH ** (-0.5) * LOG2E
    XQ = 64
    TL = S - NM * TE
    HN = HQ * DH // 2
    FC = F // NMLP
    OH = TL // NMLP
    assert T0 + NM * TM == S and HKV * XQ >= TM and T0 % L0 == 0 and HKV == 4
    assert all(T0 + t * TM >= (t + 1) * TE for t in range(NM)) and OH % PR == 0

    sem_base, n_in_sems = {}, 0
    for name, n in (("c", 1), ("wr", 1), ("x0", T0 // L0), ("x1", HKV), ("xr", 1), ("wma", 2 * NK), ("wq", NK + 1),
                    ("k", HKV), ("v", HKV), ("wo", HKV), ("wmb", HKV), ("wg", NMLP), ("wu", NMLP), ("wd", 1)):
        sem_base[name] = n_in_sems
        n_in_sems += n

    def kernel(x_hbm, k_hbm, v_hbm, wq_hbm, wo_hbm, wr_hbm, wg_hbm, wu_hbm, wd_hbm, c_hbm, wm_hbm,
               out_hbm,
               xb, x0b, ob, hb, kb, vb, wq, wo, wg, wu, wd, wma, wmb, colb, moda, modr, modb,
               st_ref, acc_ref, qacc, xn_ref, fix, cb, wrb, flag, sem_in, sem_out):
        def cp(name, i, src, dst):
            return pltpu.make_async_copy(src, dst, sem_in.at[sem_base[name] + i])

        def cp_x1(g):
            r = pl.ds(_mult(g, XQ, T0), XQ)
            return cp("x1", g, x_hbm.at[0, r], xb.at[r])

        def cp_wma(i, j):
            return cp("wma", 2 * i + j, wm_hbm.at[:, pl.ds(_mult(i, 128, j * D, 128), 128)], wma.at[i, j])

        def cp_wmb(j):
            return cp("wmb", j, wm_hbm.at[:, pl.ds(_mult(j, D, 2 * D, 128), D)], wmb.at[j, :, pl.ds(0, D)])

        def cp_wq(i):
            r = pl.ds(_mult(i, 128), 128)
            return cp("wq", i + 1, wq_hbm.at[r], wq.at[r, pl.ds(0, HQ * DH)])

        def cp_wq0(p):
            c = pl.ds(_mult(p, HN, 0, 128), HN)
            return cp("wq", p, wq_hbm.at[pl.ds(0, 128), c], wq.at[pl.ds(0, 128), c])

        def cp_x0(i):
            r = pl.ds(_mult(i, L0), L0)
            return cp("x0", i, x_hbm.at[0, r], x0b.at[r])

        def cp_k(g):
            return cp("k", g, k_hbm.at[0, g, pl.ds(SK - W, W)], kb.at[g])

        def cp_v(g):
            return cp("v", g, v_hbm.at[0, g, pl.ds(SK - W, W)], vb.at[g])

        def cp_wo(g):
            return cp("wo", g, wo_hbm.at[pl.ds(_mult(g, GD), GD)], wo.at[g, :, pl.ds(0, D)])

        xr0 = T0 + HKV * XQ
        cp_c = cp("c", 0, c_hbm, cb)
        cp_wr = cp("wr", 0, wr_hbm, wrb.at[pl.ds(0, D)])
        cp_xr = cp("xr", 0, x_hbm.at[0, pl.ds(xr0, S - xr0)], xb.at[pl.ds(xr0, S - xr0)])
        cp_wg = [cp("wg", j, wg_hbm.at[:, pl.ds(j * FC, FC)], wg.at[j, :, pl.ds(0, FC)]) for j in range(NMLP)]
        cp_wu = [cp("wu", j, wu_hbm.at[:, pl.ds(j * FC, FC)], wu.at[j, :, pl.ds(0, FC)]) for j in range(NMLP)]
        cp_wd = cp("wd", 0, wd_hbm, wd.at[:, pl.ds(0, D)])

        def cp_out(t):
            r = pl.ds(_mult(t, TE), TE)
            return pltpu.make_async_copy(ob.at[r], out_hbm.at[0, r], sem_out.at[t])

        def cp_outl(j):
            r = pl.ds(_mult(j, OH, NM * TE), OH)
            return pltpu.make_async_copy(ob.at[r], out_hbm.at[0, r], sem_out.at[NM + j])

        def wma_pair(i):
            return [cp_wma(i, 0), cp_wma(i, 1)] if i < NK else []

        order = [cp_c] + [cp_x0(i) for i in range(T0 // L0)] + wma_pair(0)
        order += [cp_wq0(0)] + wma_pair(1) + [cp_wq0(1), cp_wq(1)] + wma_pair(2)
        for i in range(2, NK):
            order += wma_pair(i + 1) + [cp_wq(i)]
        order += [cp_wr]
        for g in range(HKV):
            order += [cp_k(g), cp_v(g), cp_wo(g), cp_wmb(g), cp_x1(g)]
        order += [cp_xr] + cp_wg + cp_wu + [cp_wd]
        assert len(order) == n_in_sems
        for c in order:
            c.start()

        flag[0] = 0

        def tie(x, tok, never):
            if tok is None:
                return x
            return jnp.concatenate([jnp.where(never, tok, x[:, :128]), x[:, 128:]], axis=-1)

        def due_rows(lhs, toks, never):
            if not toks:
                return lhs
            parts = [jnp.where(never, tok, lhs[8 * k:8 * k + 8]) for k, tok in enumerate(toks)]
            return jnp.concatenate(parts + [lhs[8 * len(toks):]], axis=0)

        def ln_plain(x):
            m = jnp.sum(x, axis=-1, keepdims=True) * (1.0 / D)
            xc = x - m
            v = jnp.sum(xc * xc, axis=-1, keepdims=True) * (1.0 / D)
            return xc * lax.rsqrt(v + EPS)

        def lane_bc(v):
            return jnp.broadcast_to(v.reshape(-1, 1), (v.shape[0] * 8, 128))

        def sub_bc(p):
            return jnp.broadcast_to(_rb(jnp.sum(p, axis=0, keepdims=True)), p.shape)

        def h2_of(xc, rinv):
            return (xc * rinv) * modb[M_CB1][None] + modr[R_SB][None]

        def load_stats(row):
            st = st_ref[pl.ds(row, PR), :]
            mb = jnp.concatenate([st[:, 0:128]] * NK, axis=-1).reshape(PR // 8, 8, D)
            rinv = jnp.concatenate([st[:, 128:256]] * NK, axis=-1).reshape(PR // 8, 8, D)
            return mb, rinv

        def tok_of(v):
            return v[0:8] + v[8:16]

        def ln1_piece(xrow, slot, hrow, tok=None, never=None):
            x = tie(xb[pl.ds(xrow, PR), :].astype(f32), tok, never).reshape(PR // 8, 8, D)
            h = (ln_plain(x) * modb[M_CA1][None] + modb[M_SA][None]).reshape(PR, D)
            hb[slot, pl.ds(hrow, PR // 2), :] = pltpu.bitcast(h.astype(bf16), u32)
            return tok_of(h[:, 0:128])

        sub_iota = lax.broadcasted_iota(i32, (8, 128), 0)

        def route_piece(row, best, x1):
            m = jnp.sum(x1, axis=-1, keepdims=True) * (1.0 / D)
            mb = _rb(m)
            xc = x1 - mb
            dm = m - mb
            v = jnp.sum(xc * xc, axis=-1, keepdims=True) * (1.0 / D) - dm * dm
            rs = jnp.sum(xc * modb[M_AW][None], axis=-1, keepdims=True)
            sd = _rb(jnp.sqrt(_rb(_rb(jnp.maximum(v, 0.0)) + EPS)))
            r0 = pl.reciprocal(sd, approx=True)
            rinv = r0 * (2.0 - sd * r0)
            st_ref[pl.ds(row, PR), :] = jnp.concatenate([lane_bc(mb), lane_bc(rinv)], axis=-1)
            rr = lane_bc(rs * rinv).reshape(PR // 8, 8, 128) + modb[M_C0, :, 0:128][None]
            rbf = _rb(rr.reshape(PR, 128))
            for j in range(PR // 8):
                rj = rbf[8 * j:8 * j + 8]
                upd = rj > best[0]
                best[1] = jnp.where(upd, sub_iota + (row + 8 * j), best[1])
                best[0] = jnp.where(upd, rj, best[0])
            return xc, rinv, rbf

        def load_x1(row, tok=None, never=None):
            return tie(xb[pl.ds(row, PR), :].astype(f32), tok, never).reshape(PR // 8, 8, D)

        def epi_piece(row, best, tok=None, never=None):
            x1 = load_x1(row, tok, never)
            xc, rinv, rbf = route_piece(row, best, x1)
            ob[pl.ds(row, PR), :] = (x1 + modr[R_GB][None] * h2_of(xc, rinv)).reshape(PR, D).astype(bf16)
            return tok_of(rbf)

        def out_piece(row, tok, never):
            x1 = load_x1(row)
            mb, rinv = load_stats(row)
            mb = jnp.where(never, jnp.concatenate([tok] * NK, axis=-1).reshape(PR // 8, 8, D), mb)
            o = (x1 + modr[R_GB][None] * h2_of(x1 - mb, rinv)).reshape(PR, D)
            ob[pl.ds(row, PR), :] = o.astype(bf16)
            return o[:, 0:128]

        def matvec(w_at, tok, never):
            ys = [None, None] if tok is None else [jnp.where(never, tok[0:8], 0.0)]
            for kg in range(D // 8):
                t = w_at(slice(kg * 8, (kg + 1) * 8)).astype(f32) * colb[kg * 8:(kg + 1) * 8, :]
                k = kg % len(ys)
                ys[k] = t if ys[k] is None else ys[k] + t
            return sum(ys[1:], ys[0])

        def moda_piece(i, j, tok=None, never=None):
            y = sub_bc(matvec(lambda r: wma[i, j, r, :], tok, never))
            if j == 1:
                y = _rb(1.0 + y)
            moda[i, j] = y
            return y

        def modb_piece(ch, n, tok=None, never=None):
            y = sub_bc(matvec(lambda r: wmb[ch, r, n * 128:(n + 1) * 128], tok, never))
            modr[ch, :, n * 128:(n + 1) * 128] = y
            return y

        def qk(q, g):
            s = lax.dot_general(q, kb[g], (((1,), (1,)), ((), ())), preferred_element_type=f32)
            m = jnp.max(s, axis=-1, keepdims=True)
            p = jnp.exp2(s - m)
            l = jnp.sum(p, axis=-1, keepdims=True)
            rl = pl.reciprocal(l, approx=True)
            return p, rl * (2.0 - l * rl)

        def pv(prl, g, prev=None, never=None):
            p, rl = prl
            if prev is not None:
                p = jnp.concatenate([jnp.where(never, prev, p[:, 0:DH]), p[:, DH:]], axis=-1)
            return _dot(p.astype(bf16), vb[g]) * rl

        def paced(nsteps, step, pieces, gap, never):
            outs, done = {}, 0
            for n in range(nsteps):
                a = step(n, outs.pop(n, []))
                if n < nsteps - gap:
                    cnt = int(round((n + 1) * len(pieces) / (nsteps - gap))) - done
                    for k in range(cnt):
                        rr = (k * a.shape[0] // cnt) // PR * PR
                        outs.setdefault(n + gap, []).append(pieces[done](a[rr:rr + PR, 0:128], never))
                        done += 1
            assert done == len(pieces)

        def oproj(os_, g, j0, sink, pieces, gap, never):
            def step(n, toks):
                cs = slice(n * 128, (n + 1) * 128)
                og = jnp.concatenate([due_rows(os_[0], toks, never)] + list(os_[1:]), axis=-1)
                a = _dot(og.astype(bf16), wo[g, j0 * DH:(j0 + len(os_)) * DH, cs])
                sink(n, cs, a)
                return a
            paced(NK, step, pieces, gap, never)

        def acc_set(n, cs, a):
            acc_ref[0:a.shape[0], cs] = a

        def acc_add(n, cs, a):
            acc_ref[0:a.shape[0], cs] += a

        def write_x1(r0, x, acc, ga):
            rows = x.shape[0]
            a = acc.reshape(rows // 8, 8, D) * ga[None]
            xb[pl.ds(r0, rows), :] = (x.astype(f32) + a.reshape(rows, D)).astype(bf16)

        def zero(i, c):
            acc_ref[pl.ds(_mult(i, L0), L0), :] = jnp.zeros((L0, D), f32)
            return c

        lax.fori_loop(0, T0 // L0, zero, 0)
        modr[...] = jnp.zeros((HKV, 8, D), f32)
        cp_c.wait()
        sc = _rb(_silu(cb[...].astype(f32)))
        colb[...] = jnp.broadcast_to(sc, (128, D)).T

        def ln0(i, c):
            cp_x0(i).wait()
            r = pl.ds(_mult(i, L0), L0)
            xn = ln_plain(x0b[r, :].astype(f32))
            for n in range(NK):
                xn_ref[n, r, :] = xn[:, n * 128:(n + 1) * 128]
            return c

        lax.fori_loop(0, T0 // L0, ln0, 0)

        nw = 4 * DH

        def moda_now(i):
            cp_wma(i, 0).wait()
            cp_wma(i, 1).wait()
            moda_piece(i, 0)
            moda_piece(i, 1)

        def h_of(i):
            h = xn_ref[i].reshape(T0 // 8, 8, 128) * moda[i, 1][None] + moda[i, 0][None]
            return h.reshape(T0, 128)

        moda_now(0)

        def kfirst(p, c):
            cp_wq0(p).wait()

            @pl.when(p == 1)
            def _():
                cp_wma(1, 0).wait()
                cp_wma(1, 1).wait()

            never = flag[0] > 0
            h = h_of(0)

            def step(n, toks):
                cols = pl.ds(_mult(p, HN, n * nw, 128), nw)
                a = _dot(due_rows(h, toks, never).astype(bf16), wq[0:128, cols])
                g, c0 = divmod(n * nw, GD)
                qacc[p * (HKV // 2) + g, :, c0:c0 + nw] = a
                return a

            paced(HN // nw, step, [functools.partial(moda_piece, p, j) for j in range(2)], 2, never)
            return c

        lax.fori_loop(0, 2, kfirst, 0)

        def kstep(i, c):
            @pl.when(i == 2)
            def _():
                moda_now(i)

            cp_wq(i).wait()
            ahead = jnp.logical_and(i >= 2, i + 1 < NK)

            @pl.when(ahead)
            def _():
                cp_wma(i + 1, 0).wait()
                cp_wma(i + 1, 1).wait()

            never = flag[0] > 0
            h = h_of(i)
            nxt = jnp.where(ahead, i + 1, i)
            r = pl.ds(_mult(i, 128), 128)

            def step(n, toks):
                a = _dot(due_rows(h, toks, never).astype(bf16), wq[r, n * nw:(n + 1) * nw])
                g, c0 = divmod(n * nw, GD)
                qacc[g, :, c0:c0 + nw] += a
                return a

            paced(HQ * DH // nw, step, [functools.partial(moda_piece, nxt, j) for j in range(2)], 4, never)
            return c

        lax.fori_loop(1, NK, kstep, 0)
        cp_wr.wait()
        modb[M_SA] = jnp.concatenate([moda[i, 0] for i in range(NK)], axis=-1)
        modb[M_CA1] = jnp.concatenate([moda[i, 1] for i in range(NK)], axis=-1)

        def group0(g, c):
            for d in (cp_k(g), cp_v(g), cp_wo(g), cp_wmb(g), cp_x1(g)):
                d.wait()

            @pl.when(g == HKV - 1)
            def _():
                cp_xr.wait()

            never = flag[0] > 0
            ga = modr[R_GA]
            wr8 = jnp.broadcast_to(wrb[0:D].astype(f32).reshape(1, D), (8, D))
            cb1 = _rb(1.0 + modr[R_CB])
            modb[M_CB1] = cb1
            modb[M_AW] = cb1 * wr8
            modb[M_C0, :, 0:128] = jnp.broadcast_to(jnp.sum(modr[R_SB] * wr8, axis=-1, keepdims=True), (8, 128))

            def q_of(j):
                return (qacc[g, :, j * DH:(j + 1) * DH] * QSCALE).astype(bf16)

            mv = [functools.partial(modb_piece, g, n) for n in range(NK)]
            os_ = []
            prl = qk(q_of(0), g)
            for j in range(REP):
                if j + 1 < REP:
                    nxt = qk(q_of(j + 1), g)
                else:
                    oproj(os_[:REP // 2], g, 0, acc_add, mv[:6], 2, never)
                os_.append(pv(prl, g, os_[-1] if os_ else None, never))
                prl = nxt
            pieces = [functools.partial(ln1_piece, _mult(g, XQ, T0 + i * PR), 0,
                                        _mult(g, XQ // 2, i * PR // 2, 8)) for i in range(XQ // PR)]
            fin = [None] * NK

            def acc_fin(n, cs, a):
                fin[n] = acc_ref[:, cs] + a
                acc_ref[:, cs] = fin[n]

            oproj(os_[REP // 2:], g, REP // 2, acc_fin, pieces + mv[6:], 2, never)
            write_x1(0, x0b[...], jnp.concatenate(fin, axis=-1), ga)
            return c

        lax.fori_loop(0, HKV, group0, 0)

        def body(t, carry):
            never = flag[0] > 0
            slot = t % 2
            r0 = _mult(t, TM, T0, 32)
            re = _mult(t, TE, 0, 32)
            rn = _mult(jnp.minimum(t + 1, NM - 1), TM, T0, 32)
            best = list(carry)
            pe = [functools.partial(epi_piece, re + i * PR, best) for i in range(TE // PR)]
            pn = [functools.partial(ln1_piece, rn + i * PR, 1 - slot, i * PR // 2) for i in range(TM // PR)]
            pieces = [p for pair in zip(pe, pn) for p in pair] + pe[len(pn):]
            npg = -(-len(pieces) // (HKV - 1))
            hh = pltpu.bitcast(hb[slot, 0:TM // 2, :], bf16)
            fin = [None] * NK

            def qproj(h):
                return (_dot(hh, wq[:, h * DH:(h + 1) * DH]) * QSCALE).astype(bf16)

            def acc_fin(n, cs, a):
                fin[n] = acc_ref[0:TM, cs] + a

            q = qproj(0)
            for g in range(HKV):
                os_ = []
                for j in range(REP):
                    prl = qk(q, g)
                    if g * REP + j + 1 < HQ:
                        q = qproj(g * REP + j + 1)
                    else:
                        oproj(os_[:REP // 2], g, 0, acc_add, [], 0, never)
                    os_.append(pv(prl, g, os_[-1] if os_ else None, never))
                if g + 1 < HKV:
                    oproj(os_, g, 0, acc_set if g == 0 else acc_add, pieces[g * npg:(g + 1) * npg], 3, never)
                else:
                    oproj(os_[REP // 2:], g, REP // 2, acc_fin, [], 0, never)
            write_x1(r0, xb[pl.ds(r0, TM), :], jnp.concatenate(fin, axis=-1), modr[R_GA])
            cp_out(t).start()
            return tuple(best)

        init = (jnp.full((8, 128), -jnp.inf, f32), jnp.zeros((8, 128), i32))
        best = list(lax.fori_loop(0, NM, body, init))

        for c in cp_wg + cp_wu + [cp_wd]:
            c.wait()
        rl = NM * TE
        for i in range(TL // PR):
            route_piece(rl + i * PR, best, load_x1(rl + i * PR))

        bv, bi = best
        rmax = jnp.max(bv, axis=0, keepdims=True)
        imin = jnp.min(jnp.where(bv == rmax, bi, S), axis=0, keepdims=True)
        idx = jnp.minimum(imin[0, 0], S - 1)
        gate = jnp.concatenate([_rb(1.0 / (1.0 + jnp.exp(-rmax)))] * NK, axis=-1)
        s0 = pl.multiple_of(lax.shift_right_logical(idx, 4) * PR, PR)
        x1s = load_x1(s0)
        mbs, rinvs = load_stats(s0)
        h2s = h2_of(x1s - mbs, rinvs)
        lhs = h2s.reshape(PR, D)

        def mlp(jj, y):
            never = flag[0] > 0
            r0 = _mult(jj, OH, rl)
            pend, due, done, act = [], {}, 0, []
            for j in range(2 * (FC // FCH)):
                toks = due.pop(j, [])
                lj = jnp.concatenate(
                    [jnp.where(never, tok, lhs[:, k * 128:(k + 1) * 128]) for k, tok in enumerate(toks)]
                    + [lhs[:, len(toks) * 128:]], axis=-1)
                wref = wu if j % 2 else wg
                res = _dot(lj.astype(bf16), wref[jj, :, (j // 2) * FCH:(j // 2 + 1) * FCH])
                if done < OH // PR:
                    due.setdefault(j + OGAP, []).append(out_piece(r0 + done * PR, res[:, 0:128], never))
                    done += 1
                    if done == OH // PR:
                        cp_outl(jj).start()
                if j % 2:
                    act.append(pend.pop() * _rb(res))
                else:
                    pend.append(_rb(_silu(_rb(res))))
            assert done == OH // PR and not due
            return y + _dot(jnp.concatenate(act, axis=-1).astype(bf16), wd[pl.ds(_mult(jj, FC), FC), 0:D])

        y = _rb(lax.fori_loop(0, NMLP, mlp, jnp.zeros((PR, D), f32)))
        y = _rb(y * gate)
        rows = lax.broadcasted_iota(i32, (PR, D), 0) + s0
        upd = jnp.where(rows == idx, y, 0.0).reshape(PR // 8, 8, D)
        fix[...] = (x1s + modr[R_GB][None] * (h2s + upd)).reshape(PR, D).astype(bf16)
        for t in range(NM):
            cp_out(t).wait()
        for j in range(NMLP):
            cp_outl(j).wait()
        cp_fix = pltpu.make_async_copy(fix, out_hbm.at[0, pl.ds(s0, PR)], sem_out.at[NM + NMLP])
        cp_fix.start()
        cp_fix.wait()

    scratch = [
        pltpu.VMEM((S, D), bf16),
        pltpu.VMEM((T0, D), bf16),
        pltpu.VMEM((S, D), bf16),
        pltpu.VMEM((2, HKV * XQ // 2, D), u32),
        pltpu.VMEM((HKV, W, DH), bf16),
        pltpu.VMEM((HKV, W, DH), bf16),
        pltpu.VMEM((D, HQ * DH + PAD), bf16),
        pltpu.VMEM((HKV, GD, D + PAD), bf16),
        pltpu.VMEM((NMLP, D, FC + PAD), bf16),
        pltpu.VMEM((NMLP, D, FC + PAD), bf16),
        pltpu.VMEM((F, D + PAD), bf16),
        pltpu.VMEM((NK, 2, D, 128), bf16),
        pltpu.VMEM((HKV, D, D + PAD), bf16),
        pltpu.VMEM((D, 128), f32),
        pltpu.VMEM((NK, 2, 8, 128), f32),
        pltpu.VMEM((HKV, 8, D), f32),
        pltpu.VMEM((5, 8, D), f32),
        pltpu.VMEM((S, 256), f32),
        pltpu.VMEM((T0, D), f32),
        pltpu.VMEM((HKV, T0, GD), f32),
        pltpu.VMEM((NK, T0, 128), f32),
        pltpu.VMEM((PR, D), bf16),
        pltpu.VMEM((1, D), bf16),
        pltpu.VMEM((6 * D,), bf16),
        pltpu.SMEM((1,), i32),
        pltpu.SemaphoreType.DMA((n_in_sems,)),
        pltpu.SemaphoreType.DMA((NM + NMLP + 1,)),
    ]
    return kernel, scratch


@jax.jit
def pallas_adaLN_cond__sliding_block_cached__moe_arch_mod__prompt_kernel(
    A_x: jax.Array,
    A_k_cache: jax.Array,
    A_v_cache: jax.Array,
    A_wq: jax.Array,
    A_wo: jax.Array,
    B_x: jax.Array,
    B_w_r: jax.Array,
    B_w_gate: jax.Array,
    B_w_up: jax.Array,
    B_w_down: jax.Array,
    c: jax.Array,
    w_mod: jax.Array,
):
    B, S, D = A_x.shape
    _, HKV, SK, dh = A_k_cache.shape
    F = B_w_gate.shape[1]
    W = min(4096, max(256, SK // 4))
    assert B == 1 and dh == DH and A_wq.shape == (D, HQ * DH)
    kernel, scratch = _make_kernel(S, D, HKV, SK, W, F)
    any_spec = pl.BlockSpec(memory_space=pl.ANY)
    return pl.pallas_call(
        kernel,
        out_shape=jax.ShapeDtypeStruct((B, S, D), A_x.dtype),
        in_specs=[any_spec] * 11,
        out_specs=any_spec,
        scratch_shapes=scratch,
        compiler_params=pltpu.CompilerParams(vmem_limit_bytes=120 * 1024 * 1024,
                                             disable_semaphore_checks=True, disable_bounds_checks=True),
    )(A_x, A_k_cache, A_v_cache, A_wq, A_wo, B_w_r, B_w_gate, B_w_up, B_w_down, c, w_mod)
```

```python
import functools

import jax
import jax.numpy as jnp
from jax import lax
import jax.experimental.pallas as pl
import jax.experimental.pallas.tpu as pltpu

f32 = jnp.float32
bf16 = jnp.bfloat16
u32 = jnp.uint32
i32 = jnp.int32

HQ = 32
DH = 128
T0 = 480
TM = 224
TE = 256
L0 = 96
PR = 16
EPS = 1e-05
LOG2E = 1.4426950408889634
PAD = 128
NMLP = 2
FCH = 256
OGAP = 3
M_SA, M_CA1, M_CB1, M_AW, M_C0 = range(5)
R_GA, R_SB, R_CB, R_GB = range(4)


def _rb(x):
    return x.astype(bf16).astype(f32)


def _silu(x):
    return x * (1.0 / (1.0 + jnp.exp(-x)))


def _dot(a, b):
    return jnp.dot(a, b, preferred_element_type=f32)


def _mult(i, n, base=0, align=16):
    return base + i * n if isinstance(i, int) else pl.multiple_of(base + i * n, align)


def _make_kernel(S, D, HKV, SK, W, F):
    NM = (S - T0) // TM
    NK = D // 128
    REP = HQ // HKV
    GD = REP * DH
    QSCALE = DH ** (-0.5) * LOG2E
    XQ = 64
    TL = S - NM * TE
    HN = HQ * DH // 2
    FC = F // NMLP
    OH = TL // NMLP
    assert T0 + NM * TM == S and HKV * XQ >= TM and T0 % L0 == 0 and HKV == 4
    assert all(T0 + t * TM >= (t + 1) * TE for t in range(NM)) and OH % PR == 0

    sem_base, n_in_sems = {}, 0
    for name, n in (("c", 1), ("wr", 1), ("x0", T0 // L0), ("x1", HKV), ("xr", 1), ("wma", 2 * NK), ("wq", NK + 1),
                    ("k", HKV), ("v", HKV), ("wo", HKV), ("wmb", HKV), ("wg", NMLP), ("wu", NMLP), ("wd", 1)):
        sem_base[name] = n_in_sems
        n_in_sems += n

    def kernel(x_hbm, k_hbm, v_hbm, wq_hbm, wo_hbm, wr_hbm, wg_hbm, wu_hbm, wd_hbm, c_hbm, wm_hbm,
               out_hbm,
               xb, x0b, ob, hb, kb, vb, wq, wo, wg, wu, wd, wma, wmb, colb, moda, modr, modb,
               st_ref, acc_ref, qacc, xn_ref, fix, cb, wrb, flag, sem_in, sem_out):
        def cp(name, i, src, dst):
            return pltpu.make_async_copy(src, dst, sem_in.at[sem_base[name] + i])

        def cp_x1(g):
            r = pl.ds(_mult(g, XQ, T0), XQ)
            return cp("x1", g, x_hbm.at[0, r], xb.at[r])

        def cp_wma(i, j):
            return cp("wma", 2 * i + j, wm_hbm.at[:, pl.ds(_mult(i, 128, j * D, 128), 128)], wma.at[i, j])

        def cp_wmb(j):
            return cp("wmb", j, wm_hbm.at[:, pl.ds(_mult(j, D, 2 * D, 128), D)], wmb.at[j, :, pl.ds(0, D)])

        def cp_wq(i):
            r = pl.ds(_mult(i, 128), 128)
            return cp("wq", i + 1, wq_hbm.at[r], wq.at[r, pl.ds(0, HQ * DH)])

        def cp_wq0(p):
            c = pl.ds(_mult(p, HN, 0, 128), HN)
            return cp("wq", p, wq_hbm.at[pl.ds(0, 128), c], wq.at[pl.ds(0, 128), c])

        def cp_x0(i):
            r = pl.ds(_mult(i, L0), L0)
            return cp("x0", i, x_hbm.at[0, r], x0b.at[r])

        def cp_k(g):
            return cp("k", g, k_hbm.at[0, g, pl.ds(SK - W, W)], kb.at[g])

        def cp_v(g):
            return cp("v", g, v_hbm.at[0, g, pl.ds(SK - W, W)], vb.at[g])

        def cp_wo(g):
            return cp("wo", g, wo_hbm.at[pl.ds(_mult(g, GD), GD)], wo.at[g, :, pl.ds(0, D)])

        xr0 = T0 + HKV * XQ
        cp_c = cp("c", 0, c_hbm, cb)
        cp_wr = cp("wr", 0, wr_hbm, wrb.at[pl.ds(0, D)])
        cp_xr = cp("xr", 0, x_hbm.at[0, pl.ds(xr0, S - xr0)], xb.at[pl.ds(xr0, S - xr0)])
        cp_wg = [cp("wg", j, wg_hbm.at[:, pl.ds(j * FC, FC)], wg.at[j, :, pl.ds(0, FC)]) for j in range(NMLP)]
        cp_wu = [cp("wu", j, wu_hbm.at[:, pl.ds(j * FC, FC)], wu.at[j, :, pl.ds(0, FC)]) for j in range(NMLP)]
        cp_wd = cp("wd", 0, wd_hbm, wd.at[:, pl.ds(0, D)])

        def cp_out(t):
            r = pl.ds(_mult(t, TE), TE)
            return pltpu.make_async_copy(ob.at[r], out_hbm.at[0, r], sem_out.at[t])

        def cp_outl(j):
            r = pl.ds(_mult(j, OH, NM * TE), OH)
            return pltpu.make_async_copy(ob.at[r], out_hbm.at[0, r], sem_out.at[NM + j])

        def wma_pair(i):
            return [cp_wma(i, 0), cp_wma(i, 1)] if i < NK else []

        order = [cp_c] + [cp_x0(i) for i in range(T0 // L0)] + wma_pair(0)
        order += [cp_wq0(0)] + wma_pair(1) + [cp_wq0(1), cp_wq(1)] + wma_pair(2)
        for i in range(2, NK):
            order += wma_pair(i + 1) + [cp_wq(i)]
        order += [cp_wr]
        for g in range(HKV):
            order += [cp_k(g), cp_v(g), cp_wo(g), cp_wmb(g), cp_x1(g)]
        order += [cp_xr] + cp_wg + cp_wu + [cp_wd]
        assert len(order) == n_in_sems
        for c in order:
            c.start()

        flag[0] = 0

        def tie(x, tok, never):
            if tok is None:
                return x
            return jnp.concatenate([jnp.where(never, tok, x[:, :128]), x[:, 128:]], axis=-1)

        def due_rows(lhs, toks, never):
            if not toks:
                return lhs
            parts = [jnp.where(never, tok, lhs[8 * k:8 * k + 8]) for k, tok in enumerate(toks)]
            return jnp.concatenate(parts + [lhs[8 * len(toks):]], axis=0)

        def ln_plain(x):
            m = jnp.sum(x, axis=-1, keepdims=True) * (1.0 / D)
            xc = x - m
            v = jnp.sum(xc * xc, axis=-1, keepdims=True) * (1.0 / D)
            return xc * lax.rsqrt(v + EPS)

        def lane_bc(v):
            return jnp.broadcast_to(v.reshape(-1, 1), (v.shape[0] * 8, 128))

        def sub_bc(p):
            return jnp.broadcast_to(_rb(jnp.sum(p, axis=0, keepdims=True)), p.shape)

        def h2_of(xc, rinv):
            return (xc * rinv) * modb[M_CB1][None] + modr[R_SB][None]

        def load_stats(row):
            st = st_ref[pl.ds(row, PR), :]
            mb = jnp.concatenate([st[:, 0:128]] * NK, axis=-1).reshape(PR // 8, 8, D)
            rinv = jnp.concatenate([st[:, 128:256]] * NK, axis=-1).reshape(PR // 8, 8, D)
            return mb, rinv

        def tok_of(v):
            return v[0:8] + v[8:16]

        def ln1_piece(xrow, hrow, tok=None, never=None):
            x = tie(xb[pl.ds(xrow, PR), :].astype(f32), tok, never).reshape(PR // 8, 8, D)
            h = (ln_plain(x) * modb[M_CA1][None] + modb[M_SA][None]).reshape(PR, D)
            hb[pl.ds(hrow, PR // 2), :] = pltpu.bitcast(h.astype(bf16), u32)
            return tok_of(h[:, 0:128])

        sub_iota = lax.broadcasted_iota(i32, (8, 128), 0)

        def route_piece(row, best, x1):
            m = jnp.sum(x1, axis=-1, keepdims=True) * (1.0 / D)
            mb = _rb(m)
            xc = x1 - mb
            dm = m - mb
            v = jnp.sum(xc * xc, axis=-1, keepdims=True) * (1.0 / D) - dm * dm
            rs = jnp.sum(xc * modb[M_AW][None], axis=-1, keepdims=True)
            sd = _rb(jnp.sqrt(_rb(_rb(jnp.maximum(v, 0.0)) + EPS)))
            r0 = pl.reciprocal(sd, approx=True)
            rinv = r0 * (2.0 - sd * r0)
            st_ref[pl.ds(row, PR), :] = jnp.concatenate([lane_bc(mb), lane_bc(rinv)], axis=-1)
            rr = lane_bc(rs * rinv).reshape(PR // 8, 8, 128) + modb[M_C0, :, 0:128][None]
            rbf = _rb(rr.reshape(PR, 128))
            for j in range(PR // 8):
                rj = rbf[8 * j:8 * j + 8]
                upd = rj > best[0]
                best[1] = jnp.where(upd, sub_iota + (row + 8 * j), best[1])
                best[0] = jnp.where(upd, rj, best[0])
            return xc, rinv, rbf

        def load_x1(row, tok=None, never=None):
            return tie(xb[pl.ds(row, PR), :].astype(f32), tok, never).reshape(PR // 8, 8, D)

        def epi_piece(row, best, tok=None, never=None):
            x1 = load_x1(row, tok, never)
            xc, rinv, rbf = route_piece(row, best, x1)
            ob[pl.ds(row, PR), :] = (x1 + modr[R_GB][None] * h2_of(xc, rinv)).reshape(PR, D).astype(bf16)
            return tok_of(rbf)

        def out_piece(row, tok, never):
            x1 = load_x1(row)
            mb, rinv = load_stats(row)
            mb = jnp.where(never, jnp.concatenate([tok] * NK, axis=-1).reshape(PR // 8, 8, D), mb)
            o = (x1 + modr[R_GB][None] * h2_of(x1 - mb, rinv)).reshape(PR, D)
            ob[pl.ds(row, PR), :] = o.astype(bf16)
            return o[:, 0:128]

        def matvec(w_at, tok, never):
            ys = [None, None] if tok is None else [jnp.where(never, tok[0:8], 0.0)]
            for kg in range(D // 8):
                t = w_at(slice(kg * 8, (kg + 1) * 8)).astype(f32) * colb[kg * 8:(kg + 1) * 8, :]
                k = kg % len(ys)
                ys[k] = t if ys[k] is None else ys[k] + t
            return sum(ys[1:], ys[0])

        def moda_piece(i, j, tok=None, never=None):
            y = sub_bc(matvec(lambda r: wma[i, j, r, :], tok, never))
            if j == 1:
                y = _rb(1.0 + y)
            moda[i, j] = y
            return y

        def modb_piece(ch, n, tok=None, never=None):
            y = sub_bc(matvec(lambda r: wmb[ch, r, n * 128:(n + 1) * 128], tok, never))
            modr[ch, :, n * 128:(n + 1) * 128] = y
            return y

        def qk(q, g):
            s = lax.dot_general(q, kb[g], (((1,), (1,)), ((), ())), preferred_element_type=f32)
            m = jnp.max(s, axis=-1, keepdims=True)
            p = jnp.exp2(s - m)
            l = jnp.sum(p, axis=-1, keepdims=True)
            rl = pl.reciprocal(l, approx=True)
            return p, rl * (2.0 - l * rl)

        def pv(prl, g, prev=None, never=None):
            p, rl = prl
            if prev is not None:
                p = jnp.concatenate([jnp.where(never, prev, p[:, 0:DH]), p[:, DH:]], axis=-1)
            return _dot(p.astype(bf16), vb[g]) * rl

        def paced(nsteps, step, pieces, gap, never):
            outs, done = {}, 0
            for n in range(nsteps):
                a = step(n, outs.pop(n, []))
                if n < nsteps - gap:
                    cnt = int(round((n + 1) * len(pieces) / (nsteps - gap))) - done
                    for k in range(cnt):
                        rr = (k * a.shape[0] // cnt) // PR * PR
                        outs.setdefault(n + gap, []).append(pieces[done](a[rr:rr + PR, 0:128], never))
                        done += 1
            assert done == len(pieces)

        def oproj(os_, g, j0, sink, pieces, gap, never):
            def step(n, toks):
                cs = slice(n * 128, (n + 1) * 128)
                og = jnp.concatenate([due_rows(os_[0], toks, never)] + list(os_[1:]), axis=-1)
                a = _dot(og.astype(bf16), wo[g, j0 * DH:(j0 + len(os_)) * DH, cs])
                sink(n, cs, a)
                return a
            paced(NK, step, pieces, gap, never)

        def acc_set(n, cs, a):
            acc_ref[0:a.shape[0], cs] = a

        def acc_add(n, cs, a):
            acc_ref[0:a.shape[0], cs] += a

        def write_x1(r0, x, acc, ga):
            rows = x.shape[0]
            a = acc.reshape(rows // 8, 8, D) * ga[None]
            xb[pl.ds(r0, rows), :] = (x.astype(f32) + a.reshape(rows, D)).astype(bf16)

        def zero(i, c):
            acc_ref[pl.ds(_mult(i, L0), L0), :] = jnp.zeros((L0, D), f32)
            return c

        lax.fori_loop(0, T0 // L0, zero, 0)
        modr[...] = jnp.zeros((HKV, 8, D), f32)
        cp_c.wait()
        sc = _rb(_silu(cb[...].astype(f32)))
        colb[...] = jnp.broadcast_to(sc, (128, D)).T

        def ln0(i, c):
            cp_x0(i).wait()
            r = pl.ds(_mult(i, L0), L0)
            xn = ln_plain(x0b[r, :].astype(f32))
            for n in range(NK):
                xn_ref[n, r, :] = xn[:, n * 128:(n + 1) * 128]
            return c

        lax.fori_loop(0, T0 // L0, ln0, 0)

        nw = 4 * DH

        def moda_now(i):
            cp_wma(i, 0).wait()
            cp_wma(i, 1).wait()
            moda_piece(i, 0)
            moda_piece(i, 1)

        def h_of(i):
            h = xn_ref[i].reshape(T0 // 8, 8, 128) * moda[i, 1][None] + moda[i, 0][None]
            return h.reshape(T0, 128)

        moda_now(0)

        def kfirst(p, c):
            cp_wq0(p).wait()

            @pl.when(p == 1)
            def _():
                cp_wma(1, 0).wait()
                cp_wma(1, 1).wait()

            never = flag[0] > 0
            h = h_of(0)

            def step(n, toks):
                cols = pl.ds(_mult(p, HN, n * nw, 128), nw)
                a = _dot(due_rows(h, toks, never).astype(bf16), wq[0:128, cols])
                g, c0 = divmod(n * nw, GD)
                qacc[p * (HKV // 2) + g, :, c0:c0 + nw] = a
                return a

            paced(HN // nw, step, [functools.partial(moda_piece, p, j) for j in range(2)], 2, never)
            return c

        lax.fori_loop(0, 2, kfirst, 0)

        def kstep(i, c):
            @pl.when(i == 2)
            def _():
                moda_now(i)

            cp_wq(i).wait()
            ahead = jnp.logical_and(i >= 2, i + 1 < NK)

            @pl.when(ahead)
            def _():
                cp_wma(i + 1, 0).wait()
                cp_wma(i + 1, 1).wait()

            never = flag[0] > 0
            h = h_of(i)
            nxt = jnp.where(ahead, i + 1, i)
            r = pl.ds(_mult(i, 128), 128)

            def step(n, toks):
                a = _dot(due_rows(h, toks, never).astype(bf16), wq[r, n * nw:(n + 1) * nw])
                g, c0 = divmod(n * nw, GD)
                qacc[g, :, c0:c0 + nw] += a
                return a

            paced(HQ * DH // nw, step, [functools.partial(moda_piece, nxt, j) for j in range(2)], 4, never)
            return c

        lax.fori_loop(1, NK, kstep, 0)
        cp_wr.wait()
        modb[M_SA] = jnp.concatenate([moda[i, 0] for i in range(NK)], axis=-1)
        modb[M_CA1] = jnp.concatenate([moda[i, 1] for i in range(NK)], axis=-1)

        def group0(g, c):
            for d in (cp_k(g), cp_v(g), cp_wo(g), cp_wmb(g), cp_x1(g)):
                d.wait()

            @pl.when(g == HKV - 1)
            def _():
                cp_xr.wait()

            never = flag[0] > 0
            ga = modr[R_GA]
            wr8 = jnp.broadcast_to(wrb[0:D].astype(f32).reshape(1, D), (8, D))
            cb1 = _rb(1.0 + modr[R_CB])
            modb[M_CB1] = cb1
            modb[M_AW] = cb1 * wr8
            modb[M_C0, :, 0:128] = jnp.broadcast_to(jnp.sum(modr[R_SB] * wr8, axis=-1, keepdims=True), (8, 128))

            def q_of(j):
                return (qacc[g, :, j * DH:(j + 1) * DH] * QSCALE).astype(bf16)

            mv = [functools.partial(modb_piece, g, n) for n in range(NK)]
            os_ = []
            prl = qk(q_of(0), g)
            for j in range(REP):
                if j + 1 < REP:
                    nxt = qk(q_of(j + 1), g)
                else:
                    oproj(os_[:REP // 2], g, 0, acc_add, mv[:6], 2, never)
                os_.append(pv(prl, g, os_[-1] if os_ else None, never))
                prl = nxt
            pieces = [functools.partial(ln1_piece, _mult(g, XQ, T0 + i * PR),
                                        _mult(g, XQ // 2, i * PR // 2, 8)) for i in range(XQ // PR)]
            fin = [None] * NK

            def acc_fin(n, cs, a):
                fin[n] = acc_ref[:, cs] + a
                acc_ref[:, cs] = fin[n]

            oproj(os_[REP // 2:], g, REP // 2, acc_fin, pieces + mv[6:], 2, never)
            write_x1(0, x0b[...], jnp.concatenate(fin, axis=-1), ga)
            return c

        lax.fori_loop(0, HKV, group0, 0)

        def body(t, carry):
            never = flag[0] > 0
            r0 = _mult(t, TM, T0, 32)
            re = _mult(t, TE, 0, 32)
            rn = _mult(jnp.minimum(t + 1, NM - 1), TM, T0, 32)
            best = list(carry)
            pe = [functools.partial(epi_piece, re + i * PR, best) for i in range(TE // PR)]
            pn = [functools.partial(ln1_piece, rn + i * PR, i * PR // 2) for i in range(TM // PR)]
            pieces = [p for pair in zip(pe, pn) for p in pair] + pe[len(pn):]
            npg = -(-len(pieces) // (HKV - 1))
            hh = pltpu.bitcast(hb[0:TM // 2, :], bf16)
            fin = [None] * NK

            def qproj(h):
                return (_dot(hh, wq[:, h * DH:(h + 1) * DH]) * QSCALE).astype(bf16)

            def acc_fin(n, cs, a):
                fin[n] = acc_ref[0:TM, cs] + a

            q = qproj(0)
            for g in range(HKV):
                os_ = []
                for j in range(REP):
                    prl = qk(q, g)
                    if g * REP + j + 1 < HQ:
                        q = qproj(g * REP + j + 1)
                    else:
                        oproj(os_[:REP // 2], g, 0, acc_add, [], 0, never)
                    os_.append(pv(prl, g, os_[-1] if os_ else None, never))
                if g + 1 < HKV:
                    oproj(os_, g, 0, acc_set if g == 0 else acc_add, pieces[g * npg:(g + 1) * npg], 3, never)
                else:
                    oproj(os_[REP // 2:], g, REP // 2, acc_fin, [], 0, never)
            write_x1(r0, xb[pl.ds(r0, TM), :], jnp.concatenate(fin, axis=-1), modr[R_GA])
            cp_out(t).start()
            return tuple(best)

        init = (jnp.full((8, 128), -jnp.inf, f32), jnp.zeros((8, 128), i32))
        best = list(lax.fori_loop(0, NM, body, init))

        for c in cp_wg + cp_wu + [cp_wd]:
            c.wait()
        rl = NM * TE
        for i in range(TL // PR):
            route_piece(rl + i * PR, best, load_x1(rl + i * PR))

        bv, bi = best
        rmax = jnp.max(bv, axis=0, keepdims=True)
        imin = jnp.min(jnp.where(bv == rmax, bi, S), axis=0, keepdims=True)
        idx = jnp.minimum(imin[0, 0], S - 1)
        gate = jnp.concatenate([_rb(1.0 / (1.0 + jnp.exp(-rmax)))] * NK, axis=-1)
        s0 = pl.multiple_of(lax.shift_right_logical(idx, 4) * PR, PR)
        x1s = load_x1(s0)
        mbs, rinvs = load_stats(s0)
        h2s = h2_of(x1s - mbs, rinvs)
        lhs = h2s.reshape(PR, D)

        def mlp(jj, y):
            never = flag[0] > 0
            r0 = _mult(jj, OH, rl)
            pend, due, done, act = [], {}, 0, []
            for j in range(2 * (FC // FCH)):
                toks = due.pop(j, [])
                lj = jnp.concatenate(
                    [jnp.where(never, tok, lhs[:, k * 128:(k + 1) * 128]) for k, tok in enumerate(toks)]
                    + [lhs[:, len(toks) * 128:]], axis=-1)
                wref = wu if j % 2 else wg
                res = _dot(lj.astype(bf16), wref[jj, :, (j // 2) * FCH:(j // 2 + 1) * FCH])
                if done < OH // PR:
                    due.setdefault(j + OGAP, []).append(out_piece(r0 + done * PR, res[:, 0:128], never))
                    done += 1
                    if done == OH // PR:
                        cp_outl(jj).start()
                if j % 2:
                    act.append(pend.pop() * _rb(res))
                else:
                    pend.append(_rb(_silu(_rb(res))))
            assert done == OH // PR and not due
            return y + _dot(jnp.concatenate(act, axis=-1).astype(bf16), wd[pl.ds(_mult(jj, FC), FC), 0:D])

        y = _rb(lax.fori_loop(0, NMLP, mlp, jnp.zeros((PR, D), f32)))
        y = _rb(y * gate)
        rows = lax.broadcasted_iota(i32, (PR, D), 0) + s0
        upd = jnp.where(rows == idx, y, 0.0).reshape(PR // 8, 8, D)
        fix[...] = (x1s + modr[R_GB][None] * (h2s + upd)).reshape(PR, D).astype(bf16)
        for t in range(NM):
            cp_out(t).wait()
        for j in range(NMLP):
            cp_outl(j).wait()
        cp_fix = pltpu.make_async_copy(fix, out_hbm.at[0, pl.ds(s0, PR)], sem_out.at[NM + NMLP])
        cp_fix.start()
        cp_fix.wait()

    scratch = [
        pltpu.VMEM((S, D), bf16),
        pltpu.VMEM((T0, D), bf16),
        pltpu.VMEM((S, D), bf16),
        pltpu.VMEM((HKV * XQ // 2, D), u32),
        pltpu.VMEM((HKV, W, DH), bf16),
        pltpu.VMEM((HKV, W, DH), bf16),
        pltpu.VMEM((D, HQ * DH + PAD), bf16),
        pltpu.VMEM((HKV, GD, D + PAD), bf16),
        pltpu.VMEM((NMLP, D, FC + PAD), bf16),
        pltpu.VMEM((NMLP, D, FC + PAD), bf16),
        pltpu.VMEM((F, D + PAD), bf16),
        pltpu.VMEM((NK, 2, D, 128), bf16),
        pltpu.VMEM((HKV, D, D + PAD), bf16),
        pltpu.VMEM((D, 128), f32),
        pltpu.VMEM((NK, 2, 8, 128), f32),
        pltpu.VMEM((HKV, 8, D), f32),
        pltpu.VMEM((5, 8, D), f32),
        pltpu.VMEM((S, 256), f32),
        pltpu.VMEM((T0, D), f32),
        pltpu.VMEM((HKV, T0, GD), f32),
        pltpu.VMEM((NK, T0, 128), f32),
        pltpu.VMEM((PR, D), bf16),
        pltpu.VMEM((1, D), bf16),
        pltpu.VMEM((6 * D,), bf16),
        pltpu.SMEM((1,), i32),
        pltpu.SemaphoreType.DMA((n_in_sems,)),
        pltpu.SemaphoreType.DMA((NM + NMLP + 1,)),
    ]
    return kernel, scratch


@jax.jit
def pallas_adaLN_cond__sliding_block_cached__moe_arch_mod__prompt_kernel(
    A_x: jax.Array,
    A_k_cache: jax.Array,
    A_v_cache: jax.Array,
    A_wq: jax.Array,
    A_wo: jax.Array,
    B_x: jax.Array,
    B_w_r: jax.Array,
    B_w_gate: jax.Array,
    B_w_up: jax.Array,
    B_w_down: jax.Array,
    c: jax.Array,
    w_mod: jax.Array,
):
    B, S, D = A_x.shape
    _, HKV, SK, dh = A_k_cache.shape
    F = B_w_gate.shape[1]
    W = min(4096, max(256, SK // 4))
    assert B == 1 and dh == DH and A_wq.shape == (D, HQ * DH)
    kernel, scratch = _make_kernel(S, D, HKV, SK, W, F)
    any_spec = pl.BlockSpec(memory_space=pl.ANY)
    return pl.pallas_call(
        kernel,
        out_shape=jax.ShapeDtypeStruct((B, S, D), A_x.dtype),
        in_specs=[any_spec] * 11,
        out_specs=any_spec,
        scratch_shapes=scratch,
        compiler_params=pltpu.CompilerParams(vmem_limit_bytes=120 * 1024 * 1024,
                                             disable_semaphore_checks=True, disable_bounds_checks=True),
    )(A_x, A_k_cache, A_v_cache, A_wq, A_wo, B_w_r, B_w_gate, B_w_up, B_w_down, c, w_mod)
```

```python
import functools

import jax
import jax.numpy as jnp
from jax import lax
import jax.experimental.pallas as pl
import jax.experimental.pallas.tpu as pltpu

f32 = jnp.float32
bf16 = jnp.bfloat16
u32 = jnp.uint32
i32 = jnp.int32

HQ = 32
DH = 128
T0 = 480
TM = 224
TE = 256
L0 = 96
PR = 16
EPS = 1e-05
LOG2E = 1.4426950408889634
PAD = 128
NMLP = 2
FCH = 256
OGAP = 3
M_SA, M_CA1, M_CB1, M_AW, M_C0 = range(5)
R_GA, R_SB, R_CB, R_GB = range(4)


def _rb(x):
    return x.astype(bf16).astype(f32)


def _silu(x):
    return x * (1.0 / (1.0 + jnp.exp(-x)))


def _dot(a, b):
    return jnp.dot(a, b, preferred_element_type=f32)


def _mult(i, n, base=0, align=16):
    return base + i * n if isinstance(i, int) else pl.multiple_of(base + i * n, align)


def _make_kernel(S, D, HKV, SK, W, F):
    NM = (S - T0) // TM
    NK = D // 128
    REP = HQ // HKV
    GD = REP * DH
    QSCALE = DH ** (-0.5) * LOG2E
    XQ = 64
    TL = S - NM * TE
    HN = HQ * DH // 2
    FC = F // NMLP
    OH = TL // NMLP
    assert T0 + NM * TM == S and HKV * XQ >= TM and T0 % L0 == 0 and HKV == 4
    assert all(T0 + t * TM >= (t + 1) * TE for t in range(NM)) and OH % PR == 0

    sem_base, n_in_sems = {}, 0
    for name, n in (("c", 1), ("wr", 1), ("x0", T0 // L0), ("x1", HKV), ("xr", 1), ("wma", 2 * NK), ("wq", NK + 1),
                    ("k", HKV), ("v", HKV), ("wo", HKV), ("wmb", HKV), ("wg", NMLP), ("wu", NMLP), ("wd", 1)):
        sem_base[name] = n_in_sems
        n_in_sems += n

    def kernel(x_hbm, k_hbm, v_hbm, wq_hbm, wo_hbm, wr_hbm, wg_hbm, wu_hbm, wd_hbm, c_hbm, wm_hbm,
               out_hbm,
               xb, x0b, ob, hb, kb, vb, wq, wo, wg, wu, wd, wma, wmb, colb, moda, modr, modb,
               st_ref, sh_ref, ps_ref, acc_ref, qacc, xn_ref, fix, cb, wrb, flag, sem_in, sem_out):
        def cp(name, i, src, dst):
            return pltpu.make_async_copy(src, dst, sem_in.at[sem_base[name] + i])

        def cp_x1(g):
            r = pl.ds(_mult(g, XQ, T0), XQ)
            return cp("x1", g, x_hbm.at[0, r], xb.at[r])

        def cp_wma(i, j):
            return cp("wma", 2 * i + j, wm_hbm.at[:, pl.ds(_mult(i, 128, j * D, 128), 128)], wma.at[i, j])

        def cp_wmb(j):
            return cp("wmb", j, wm_hbm.at[:, pl.ds(_mult(j, D, 2 * D, 128), D)], wmb.at[j, :, pl.ds(0, D)])

        def cp_wq(i):
            r = pl.ds(_mult(i, 128), 128)
            return cp("wq", i + 1, wq_hbm.at[r], wq.at[r, pl.ds(0, HQ * DH)])

        def cp_wq0(p):
            c = pl.ds(_mult(p, HN, 0, 128), HN)
            return cp("wq", p, wq_hbm.at[pl.ds(0, 128), c], wq.at[pl.ds(0, 128), c])

        def cp_x0(i):
            r = pl.ds(_mult(i, L0), L0)
            return cp("x0", i, x_hbm.at[0, r], x0b.at[r])

        def cp_k(g):
            return cp("k", g, k_hbm.at[0, g, pl.ds(SK - W, W)], kb.at[g])

        def cp_v(g):
            return cp("v", g, v_hbm.at[0, g, pl.ds(SK - W, W)], vb.at[g])

        def cp_wo(g):
            return cp("wo", g, wo_hbm.at[pl.ds(_mult(g, GD), GD)], wo.at[g, :, pl.ds(0, D)])

        xr0 = T0 + HKV * XQ
        cp_c = cp("c", 0, c_hbm, cb)
        cp_wr = cp("wr", 0, wr_hbm, wrb.at[pl.ds(0, D)])
        cp_xr = cp("xr", 0, x_hbm.at[0, pl.ds(xr0, S - xr0)], xb.at[pl.ds(xr0, S - xr0)])
        cp_wg = [cp("wg", j, wg_hbm.at[:, pl.ds(j * FC, FC)], wg.at[j, :, pl.ds(0, FC)]) for j in range(NMLP)]
        cp_wu = [cp("wu", j, wu_hbm.at[:, pl.ds(j * FC, FC)], wu.at[j, :, pl.ds(0, FC)]) for j in range(NMLP)]
        cp_wd = cp("wd", 0, wd_hbm, wd.at[:, pl.ds(0, D)])

        def cp_out(t):
            r = pl.ds(_mult(t, TE), TE)
            return pltpu.make_async_copy(ob.at[r], out_hbm.at[0, r], sem_out.at[t])

        def cp_outl(j):
            r = pl.ds(_mult(j, OH, NM * TE), OH)
            return pltpu.make_async_copy(ob.at[r], out_hbm.at[0, r], sem_out.at[NM + j])

        def wma_pair(i):
            return [cp_wma(i, 0), cp_wma(i, 1)] if i < NK else []

        order = [cp_c] + [cp_x0(i) for i in range(T0 // L0)] + wma_pair(0)
        order += [cp_wq0(0)] + wma_pair(1) + [cp_wq0(1), cp_wq(1)] + wma_pair(2)
        for i in range(2, NK):
            order += wma_pair(i + 1) + [cp_wq(i)]
        order += [cp_wr]
        for g in range(HKV):
            order += [cp_k(g), cp_v(g), cp_wo(g), cp_wmb(g), cp_x1(g)]
        order += [cp_xr] + cp_wg + cp_wu + [cp_wd]
        assert len(order) == n_in_sems
        for c in order:
            c.start()

        flag[0] = 0

        def tie(x, tok, never):
            if tok is None:
                return x
            return jnp.concatenate([jnp.where(never, tok, x[:, :128]), x[:, 128:]], axis=-1)

        def due_rows(lhs, toks, never):
            if not toks:
                return lhs
            parts = [jnp.where(never, tok, lhs[8 * k:8 * k + 8]) for k, tok in enumerate(toks)]
            return jnp.concatenate(parts + [lhs[8 * len(toks):]], axis=0)

        def ln_plain(x):
            m = jnp.sum(x, axis=-1, keepdims=True) * (1.0 / D)
            xc = x - m
            v = jnp.sum(xc * xc, axis=-1, keepdims=True) * (1.0 / D)
            return xc * lax.rsqrt(v + EPS), m

        def lane_bc(v):
            return jnp.broadcast_to(v.reshape(-1, 1), (v.shape[0] * 8, 128))

        def sub_bc(p):
            return jnp.broadcast_to(_rb(jnp.sum(p, axis=0, keepdims=True)), p.shape)

        def h2_of(xc, rinv):
            return (xc * rinv) * modb[M_CB1][None] + modr[R_SB][None]

        def load_stats(row):
            st = st_ref[pl.ds(row, PR), :]
            mb = jnp.concatenate([st[:, 0:128]] * NK, axis=-1).reshape(PR // 8, 8, D)
            rinv = jnp.concatenate([st[:, 128:256]] * NK, axis=-1).reshape(PR // 8, 8, D)
            return mb, rinv

        def tok_of(v):
            return v[0:8] + v[8:16]

        def ln1_piece(xrow, hrow, tok=None, never=None):
            x = tie(xb[pl.ds(xrow, PR), :].astype(f32), tok, never).reshape(PR // 8, 8, D)
            xn, m = ln_plain(x)
            if isinstance(hrow, int):
                sh_ref[2 * hrow:2 * hrow + PR, :] = lane_bc(m)
            h = (xn * modb[M_CA1][None] + modb[M_SA][None]).reshape(PR, D)
            hb[pl.ds(hrow, PR // 2), :] = pltpu.bitcast(h.astype(bf16), u32)
            return tok_of(h[:, 0:128])

        sub_iota = lax.broadcasted_iota(i32, (8, 128), 0)

        def route(row, best, mb, v, rs):
            sd = _rb(jnp.sqrt(_rb(_rb(jnp.maximum(v, 0.0)) + EPS)))
            r0 = pl.reciprocal(sd, approx=True)
            rinv = r0 * (2.0 - sd * r0)
            st_ref[pl.ds(row, PR), :] = jnp.concatenate([mb, rinv], axis=-1)
            rr = (rs * rinv).reshape(PR // 8, 8, 128) + modb[M_C0, :, 0:128][None]
            rbf = _rb(rr.reshape(PR, 128))
            for j in range(PR // 8):
                rj = rbf[8 * j:8 * j + 8]
                upd = rj > best[0]
                best[1] = jnp.where(upd, sub_iota + (row + 8 * j), best[1])
                best[0] = jnp.where(upd, rj, best[0])
            return rinv, rbf

        def route_piece(row, best, x1):
            m = jnp.sum(x1, axis=-1, keepdims=True) * (1.0 / D)
            mb = _rb(m)
            xc = x1 - mb
            dm = m - mb
            v = jnp.sum(xc * xc, axis=-1, keepdims=True) * (1.0 / D) - dm * dm
            rs = jnp.sum(xc * modb[M_AW][None], axis=-1, keepdims=True)
            rinv, rbf = route(row, best, lane_bc(mb), lane_bc(v), lane_bc(rs))
            return xc, jnp.concatenate([rinv] * NK, axis=-1).reshape(PR // 8, 8, D), rbf

        def route_sums(row, best, prow):
            def lane_sum(k):
                t = jnp.sum(ps_ref[prow:prow + PR, k * 128:(k + 1) * 128], axis=-1, keepdims=True)
                return jnp.broadcast_to(t, (PR, 128))
            sh = sh_ref[prow:prow + PR, :]
            d = lane_sum(0) * (1.0 / D)
            mb = _rb(sh + d)
            saw = jnp.concatenate([modb[M_C0, :, 128:256]] * (PR // 8), axis=0)
            route(row, best, mb, lane_sum(1) * (1.0 / D) - d * d, lane_sum(2) + (sh - mb) * saw)

        def load_x1(row, tok=None, never=None):
            return tie(xb[pl.ds(row, PR), :].astype(f32), tok, never).reshape(PR // 8, 8, D)

        def epi_piece(row, best, tok=None, never=None):
            x1 = load_x1(row, tok, never)
            xc, rinv, rbf = route_piece(row, best, x1)
            ob[pl.ds(row, PR), :] = (x1 + modr[R_GB][None] * h2_of(xc, rinv)).reshape(PR, D).astype(bf16)
            return tok_of(rbf)

        def out_piece(row, tok, never):
            x1 = load_x1(row)
            mb, rinv = load_stats(row)
            mb = jnp.where(never, jnp.concatenate([tok] * NK, axis=-1).reshape(PR // 8, 8, D), mb)
            o = (x1 + modr[R_GB][None] * h2_of(x1 - mb, rinv)).reshape(PR, D)
            ob[pl.ds(row, PR), :] = o.astype(bf16)
            return o[:, 0:128]

        def matvec(w_at, tok, never):
            ys = [None, None] if tok is None else [jnp.where(never, tok[0:8], 0.0)]
            for kg in range(D // 8):
                t = w_at(slice(kg * 8, (kg + 1) * 8)).astype(f32) * colb[kg * 8:(kg + 1) * 8, :]
                k = kg % len(ys)
                ys[k] = t if ys[k] is None else ys[k] + t
            return sum(ys[1:], ys[0])

        def moda_piece(i, j, tok=None, never=None):
            y = sub_bc(matvec(lambda r: wma[i, j, r, :], tok, never))
            if j == 1:
                y = _rb(1.0 + y)
            moda[i, j] = y
            return y

        def modb_piece(ch, n, tok=None, never=None):
            y = sub_bc(matvec(lambda r: wmb[ch, r, n * 128:(n + 1) * 128], tok, never))
            modr[ch, :, n * 128:(n + 1) * 128] = y
            return y

        def qk(q, g):
            s = lax.dot_general(q, kb[g], (((1,), (1,)), ((), ())), preferred_element_type=f32)
            m = jnp.max(s, axis=-1, keepdims=True)
            p = jnp.exp2(s - m)
            l = jnp.sum(p, axis=-1, keepdims=True)
            rl = pl.reciprocal(l, approx=True)
            return p, rl * (2.0 - l * rl)

        def pv(prl, g, prev=None, never=None):
            p, rl = prl
            if prev is not None:
                p = jnp.concatenate([jnp.where(never, prev, p[:, 0:DH]), p[:, DH:]], axis=-1)
            return _dot(p.astype(bf16), vb[g]) * rl

        def paced(nsteps, step, pieces, gap, never):
            outs, done = {}, 0
            for n in range(nsteps):
                a = step(n, outs.pop(n, []))
                if n < nsteps - gap:
                    cnt = int(round((n + 1) * len(pieces) / (nsteps - gap))) - done
                    for k in range(cnt):
                        rr = (k * a.shape[0] // cnt) // PR * PR
                        outs.setdefault(n + gap, []).append(pieces[done](a[rr:rr + PR, 0:128], never))
                        done += 1
            assert done == len(pieces)

        def oproj(os_, g, j0, sink, pieces, gap, never):
            def step(n, toks):
                cs = slice(n * 128, (n + 1) * 128)
                og = jnp.concatenate([due_rows(os_[0], toks, never)] + list(os_[1:]), axis=-1)
                a = _dot(og.astype(bf16), wo[g, j0 * DH:(j0 + len(os_)) * DH, cs])
                sink(n, cs, a)
                return a
            paced(NK, step, pieces, gap, never)

        def acc_set(n, cs, a):
            acc_ref[0:a.shape[0], cs] = a

        def acc_add(n, cs, a):
            acc_ref[0:a.shape[0], cs] += a

        def write_x1(r0, x, acc, ga, with_sums=False):
            rows = x.shape[0]
            a = acc.reshape(rows // 8, 8, D) * ga[None]
            x1 = (x.astype(f32) + a.reshape(rows, D)).astype(bf16)
            xb[pl.ds(r0, rows), :] = x1
            if with_sums:
                x1 = x1.astype(f32)
                sh = sh_ref[0:rows, :]
                sums = None
                for n in range(NK):
                    cs = slice(n * 128, (n + 1) * 128)
                    y = x1[:, cs] - sh
                    ya = (y.reshape(rows // 8, 8, 128) * modb[M_AW, :, cs][None]).reshape(rows, 128)
                    t = jnp.concatenate([y, y * y, ya], axis=-1)
                    sums = t if sums is None else sums + t
                ps_ref[0:rows, :] = sums

        def zero(i, c):
            acc_ref[pl.ds(_mult(i, L0), L0), :] = jnp.zeros((L0, D), f32)
            return c

        lax.fori_loop(0, T0 // L0, zero, 0)
        modr[...] = jnp.zeros((HKV, 8, D), f32)
        cp_c.wait()
        sc = _rb(_silu(cb[...].astype(f32)))
        colb[...] = jnp.broadcast_to(sc, (128, D)).T

        def ln0(i, c):
            cp_x0(i).wait()
            r = pl.ds(_mult(i, L0), L0)
            xn, _ = ln_plain(x0b[r, :].astype(f32))
            for n in range(NK):
                xn_ref[n, r, :] = xn[:, n * 128:(n + 1) * 128]
            return c

        lax.fori_loop(0, T0 // L0, ln0, 0)

        nw = 4 * DH

        def moda_now(i):
            cp_wma(i, 0).wait()
            cp_wma(i, 1).wait()
            moda_piece(i, 0)
            moda_piece(i, 1)

        def h_of(i):
            h = xn_ref[i].reshape(T0 // 8, 8, 128) * moda[i, 1][None] + moda[i, 0][None]
            return h.reshape(T0, 128)

        moda_now(0)

        def kfirst(p, c):
            cp_wq0(p).wait()

            @pl.when(p == 1)
            def _():
                cp_wma(1, 0).wait()
                cp_wma(1, 1).wait()

            never = flag[0] > 0
            h = h_of(0)

            def step(n, toks):
                cols = pl.ds(_mult(p, HN, n * nw, 128), nw)
                a = _dot(due_rows(h, toks, never).astype(bf16), wq[0:128, cols])
                g, c0 = divmod(n * nw, GD)
                qacc[p * (HKV // 2) + g, :, c0:c0 + nw] = a
                return a

            paced(HN // nw, step, [functools.partial(moda_piece, p, j) for j in range(2)], 2, never)
            return c

        lax.fori_loop(0, 2, kfirst, 0)

        def kstep(i, c):
            @pl.when(i == 2)
            def _():
                moda_now(i)

            cp_wq(i).wait()
            ahead = jnp.logical_and(i >= 2, i + 1 < NK)

            @pl.when(ahead)
            def _():
                cp_wma(i + 1, 0).wait()
                cp_wma(i + 1, 1).wait()

            never = flag[0] > 0
            h = h_of(i)
            nxt = jnp.where(ahead, i + 1, i)
            r = pl.ds(_mult(i, 128), 128)

            def step(n, toks):
                a = _dot(due_rows(h, toks, never).astype(bf16), wq[r, n * nw:(n + 1) * nw])
                g, c0 = divmod(n * nw, GD)
                qacc[g, :, c0:c0 + nw] += a
                return a

            paced(HQ * DH // nw, step, [functools.partial(moda_piece, nxt, j) for j in range(2)], 4, never)
            return c

        lax.fori_loop(1, NK, kstep, 0)
        cp_wr.wait()
        modb[M_SA] = jnp.concatenate([moda[i, 0] for i in range(NK)], axis=-1)
        modb[M_CA1] = jnp.concatenate([moda[i, 1] for i in range(NK)], axis=-1)

        def group0(g, c):
            for d in (cp_k(g), cp_v(g), cp_wo(g), cp_wmb(g), cp_x1(g)):
                d.wait()

            @pl.when(g == HKV - 1)
            def _():
                cp_xr.wait()

            never = flag[0] > 0
            ga = modr[R_GA]
            wr8 = jnp.broadcast_to(wrb[0:D].astype(f32).reshape(1, D), (8, D))
            cb1 = _rb(1.0 + modr[R_CB])
            modb[M_CB1] = cb1
            modb[M_AW] = cb1 * wr8
            modb[M_C0, :, 0:256] = jnp.concatenate(
                [jnp.broadcast_to(jnp.sum(v * wr8, axis=-1, keepdims=True), (8, 128)) for v in (modr[R_SB], cb1)],
                axis=-1)

            def q_of(j):
                return (qacc[g, :, j * DH:(j + 1) * DH] * QSCALE).astype(bf16)

            mv = [functools.partial(modb_piece, g, n) for n in range(NK)]
            os_ = []
            prl = qk(q_of(0), g)
            for j in range(REP):
                if j + 1 < REP:
                    nxt = qk(q_of(j + 1), g)
                else:
                    oproj(os_[:REP // 2], g, 0, acc_add, mv[:6], 2, never)
                os_.append(pv(prl, g, os_[-1] if os_ else None, never))
                prl = nxt
            pieces = [functools.partial(ln1_piece, _mult(g, XQ, T0 + i * PR),
                                        _mult(g, XQ // 2, i * PR // 2, 8)) for i in range(XQ // PR)]
            fin = [None] * NK

            def acc_fin(n, cs, a):
                fin[n] = acc_ref[:, cs] + a
                acc_ref[:, cs] = fin[n]

            oproj(os_[REP // 2:], g, REP // 2, acc_fin, pieces + mv[6:], 2, never)
            write_x1(0, x0b[...], jnp.concatenate(fin, axis=-1), ga)
            return c

        lax.fori_loop(0, HKV, group0, 0)

        def body(t, carry):
            never = flag[0] > 0
            r0 = _mult(t, TM, T0, 32)
            re = _mult(t, TE, 0, 32)
            rn = _mult(jnp.minimum(t + 1, NM - 1), TM, T0, 32)
            best = list(carry)
            pe = [functools.partial(epi_piece, re + i * PR, best) for i in range(TE // PR)]
            pn = [functools.partial(ln1_piece, rn + i * PR, i * PR // 2) for i in range(TM // PR)]
            pieces = [p for pair in zip(pe, pn) for p in pair] + pe[len(pn):]
            npg = -(-len(pieces) // (HKV - 1))
            hh = pltpu.bitcast(hb[0:TM // 2, :], bf16)
            fin = [None] * NK

            def qproj(h):
                return (_dot(hh, wq[:, h * DH:(h + 1) * DH]) * QSCALE).astype(bf16)

            def acc_fin(n, cs, a):
                fin[n] = acc_ref[0:TM, cs] + a

            q = qproj(0)
            for g in range(HKV):
                os_ = []
                for j in range(REP):
                    prl = qk(q, g)
                    if g * REP + j + 1 < HQ:
                        q = qproj(g * REP + j + 1)
                    else:
                        oproj(os_[:REP // 2], g, 0, acc_add, [], 0, never)
                    os_.append(pv(prl, g, os_[-1] if os_ else None, never))
                if g + 1 < HKV:
                    oproj(os_, g, 0, acc_set if g == 0 else acc_add, pieces[g * npg:(g + 1) * npg], 3, never)
                else:
                    oproj(os_[REP // 2:], g, REP // 2, acc_fin, [], 0, never)
            write_x1(r0, xb[pl.ds(r0, TM), :], jnp.concatenate(fin, axis=-1), modr[R_GA], True)
            cp_out(t).start()
            return tuple(best)

        init = (jnp.full((8, 128), -jnp.inf, f32), jnp.zeros((8, 128), i32))
        best = list(lax.fori_loop(0, NM, body, init))

        for c in cp_wg + cp_wu + [cp_wd]:
            c.wait()
        rl = NM * TE
        for row in range(rl, S, PR):
            if row < S - TM:
                route_piece(row, best, load_x1(row))
            else:
                route_sums(row, best, row - (S - TM))

        bv, bi = best
        rmax = jnp.max(bv, axis=0, keepdims=True)
        imin = jnp.min(jnp.where(bv == rmax, bi, S), axis=0, keepdims=True)
        idx = jnp.clip(imin[0, 0], 0, S - 1)
        gate = jnp.concatenate([_rb(1.0 / (1.0 + jnp.exp(-rmax)))] * NK, axis=-1)
        s0 = pl.multiple_of(lax.shift_right_logical(idx, 4) * PR, PR)
        x1s = load_x1(s0)
        mbs, rinvs = load_stats(s0)
        h2s = h2_of(x1s - mbs, rinvs)
        lhs = h2s.reshape(PR, D)

        def mlp(jj, y):
            never = flag[0] > 0
            r0 = _mult(jj, OH, rl)
            pend, due, done, act = [], {}, 0, []
            for j in range(2 * (FC // FCH)):
                toks = due.pop(j, [])
                lj = jnp.concatenate(
                    [jnp.where(never, tok, lhs[:, k * 128:(k + 1) * 128]) for k, tok in enumerate(toks)]
                    + [lhs[:, len(toks) * 128:]], axis=-1)
                wref = wu if j % 2 else wg
                res = _dot(lj.astype(bf16), wref[jj, :, (j // 2) * FCH:(j // 2 + 1) * FCH])
                if done < OH // PR:
                    due.setdefault(j + OGAP, []).append(out_piece(r0 + done * PR, res[:, 0:128], never))
                    done += 1
                    if done == OH // PR:
                        cp_outl(jj).start()
                if j % 2:
                    act.append(pend.pop() * _rb(res))
                else:
                    pend.append(_rb(_silu(_rb(res))))
            assert done == OH // PR and not due
            return y + _dot(jnp.concatenate(act, axis=-1).astype(bf16), wd[pl.ds(_mult(jj, FC), FC), 0:D])

        y = _rb(lax.fori_loop(0, NMLP, mlp, jnp.zeros((PR, D), f32)))
        y = _rb(y * gate)
        rows = lax.broadcasted_iota(i32, (PR, D), 0) + s0
        upd = jnp.where(rows == idx, y, 0.0).reshape(PR // 8, 8, D)
        fix[...] = (x1s + modr[R_GB][None] * (h2s + upd)).reshape(PR, D).astype(bf16)
        for t in range(NM):
            cp_out(t).wait()
        for j in range(NMLP):
            cp_outl(j).wait()
        cp_fix = pltpu.make_async_copy(fix, out_hbm.at[0, pl.ds(s0, PR)], sem_out.at[NM + NMLP])
        cp_fix.start()
        cp_fix.wait()

    scratch = [
        pltpu.VMEM((S, D), bf16),
        pltpu.VMEM((T0, D), bf16),
        pltpu.VMEM((S, D), bf16),
        pltpu.VMEM((HKV * XQ // 2, D), u32),
        pltpu.VMEM((HKV, W, DH), bf16),
        pltpu.VMEM((HKV, W, DH), bf16),
        pltpu.VMEM((D, HQ * DH + PAD), bf16),
        pltpu.VMEM((HKV, GD, D + PAD), bf16),
        pltpu.VMEM((NMLP, D, FC + PAD), bf16),
        pltpu.VMEM((NMLP, D, FC + PAD), bf16),
        pltpu.VMEM((F, D + PAD), bf16),
        pltpu.VMEM((NK, 2, D, 128), bf16),
        pltpu.VMEM((HKV, D, D + PAD), bf16),
        pltpu.VMEM((D, 128), f32),
        pltpu.VMEM((NK, 2, 8, 128), f32),
        pltpu.VMEM((HKV, 8, D), f32),
        pltpu.VMEM((5, 8, D), f32),
        pltpu.VMEM((S, 256), f32),
        pltpu.VMEM((HKV * XQ, 128), f32),
        pltpu.VMEM((HKV * XQ, 384), f32),
        pltpu.VMEM((T0, D), f32),
        pltpu.VMEM((HKV, T0, GD), f32),
        pltpu.VMEM((NK, T0, 128), f32),
        pltpu.VMEM((PR, D), bf16),
        pltpu.VMEM((1, D), bf16),
        pltpu.VMEM((6 * D,), bf16),
        pltpu.SMEM((1,), i32),
        pltpu.SemaphoreType.DMA((n_in_sems,)),
        pltpu.SemaphoreType.DMA((NM + NMLP + 1,)),
    ]
    return kernel, scratch


@jax.jit
def pallas_adaLN_cond__sliding_block_cached__moe_arch_mod__prompt_kernel(
    A_x: jax.Array,
    A_k_cache: jax.Array,
    A_v_cache: jax.Array,
    A_wq: jax.Array,
    A_wo: jax.Array,
    B_x: jax.Array,
    B_w_r: jax.Array,
    B_w_gate: jax.Array,
    B_w_up: jax.Array,
    B_w_down: jax.Array,
    c: jax.Array,
    w_mod: jax.Array,
):
    B, S, D = A_x.shape
    _, HKV, SK, dh = A_k_cache.shape
    F = B_w_gate.shape[1]
    W = min(4096, max(256, SK // 4))
    assert B == 1 and dh == DH and A_wq.shape == (D, HQ * DH)
    kernel, scratch = _make_kernel(S, D, HKV, SK, W, F)
    any_spec = pl.BlockSpec(memory_space=pl.ANY)
    return pl.pallas_call(
        kernel,
        out_shape=jax.ShapeDtypeStruct((B, S, D), A_x.dtype),
        in_specs=[any_spec] * 11,
        out_specs=any_spec,
        scratch_shapes=scratch,
        compiler_params=pltpu.CompilerParams(vmem_limit_bytes=100 * 1024 * 1024,
                                             disable_semaphore_checks=True, disable_bounds_checks=True),
    )(A_x, A_k_cache, A_v_cache, A_wq, A_wo, B_w_r, B_w_gate, B_w_up, B_w_down, c, w_mod)
```
